```python
import jax
import jax.numpy as jnp

def _softmax(x, axis=-1):
    return jax.nn.softmax(x, axis=axis)
def _gelu(x):
    return jax.nn.gelu(x, approximate=True)
def _silu(x):
    return jax.nn.silu(x)
def _sigmoid(x):
    return jax.nn.sigmoid(x)
def _layernorm(x, axis=-1, eps=1e-5):
    m = jnp.mean(x, axis=axis, keepdims=True)
    v = jnp.var(x, axis=axis, keepdims=True)
    return (x - m) / jnp.sqrt(v + eps)
def _scatter_add(tgt, idx, src, axis=0):
    return tgt.at[idx].add(src)
def _segment_sum(src, seg, n):
    return jax.ops.segment_sum(src, seg, n)
class _Rng:
    def __init__(self, key):
        self._k = key
    def _next(self):
        self._k, sub = jax.random.split(self._k)
        return sub
    def normal(self, shape):
        return jax.random.normal(self._next(), shape, dtype=jnp.bfloat16)
    def randint(self, lo, hi, shape):
        return jax.random.randint(self._next(), shape, lo, hi, dtype=jnp.int32)
    def uniform(self, shape, lo=0.0, hi=1.0):
        return jax.random.uniform(self._next(), shape, jnp.bfloat16, lo, hi)
    def permutation(self, n):
        return jax.random.permutation(self._next(), n)


kernel_name = 'gated_mix__compressed_kv_cla__moe_arch_mod__prompt'

def setup_inputs():
    _rng = _Rng(jax.random.key(int.from_bytes(__import__("os").urandom(4), "little")))
    _w = (lambda a: (lambda t: t.astype(jnp.bfloat16) if jnp.issubdtype(t.dtype, jnp.floating) else t)(jnp.asarray(a)))
    def _A_setup():
        B, H, Sq, Sk, D, M = 1, 16, 2048, 2048, 256, 448
        Dc = 4 * D
        return {
            "x": _w((lambda *s: _rng.normal(s) * 0.05)(B, Sq, M)),
            "c_kv": _w((lambda *s: _rng.normal(s) * 0.05)(B, Sk, Dc)),
            "w_q": _w((lambda *s: _rng.normal(s) * 0.05)(M, H, D) * (M ** -0.5)),
            "w_uk": _w((lambda *s: _rng.normal(s) * 0.05)(Dc, H, D) * (Dc ** -0.5)),
            "w_uv": _w((lambda *s: _rng.normal(s) * 0.05)(Dc, H, D) * (Dc ** -0.5)),
            "w_o": _w((lambda *s: _rng.normal(s) * 0.05)(H, D, M) * ((H * D) ** -0.5)),
        }
    _A_in = _A_setup()

    def _B_setup():
        B, S, D, F, C = 1, 2048, 448, 1792, 2
        return {
            "x": _w((lambda *s: _rng.normal(s) * 0.05)(B, S, D)),
            "w_r": _w((lambda *s: _rng.normal(s) * 0.05)(D)),
            "w_gate": _w((lambda *s: _rng.normal(s) * 0.05)(D, F)),
            "w_up": _w((lambda *s: _rng.normal(s) * 0.05)(D, F)),
            "w_down": _w((lambda *s: _rng.normal(s) * 0.05)(F, D)),
        }
    _B_in = _B_setup()

    return {
        "A_x": _A_in["x"],
        "A_c_kv": _A_in["c_kv"],
        "A_w_q": _A_in["w_q"],
        "A_w_uk": _A_in["w_uk"],
        "A_w_uv": _A_in["w_uv"],
        "A_w_o": _A_in["w_o"],
        "B_x": _B_in["x"],
        "B_w_r": _B_in["w_r"],
        "B_w_gate": _B_in["w_gate"],
        "B_w_up": _B_in["w_up"],
        "B_w_down": _B_in["w_down"],
        "gate_w": _w((lambda *s: _rng.normal(s) * 0.05)(448)),
    }

def reference(A_x, A_c_kv, A_w_q, A_w_uk, A_w_uv, A_w_o, B_x, B_w_r, B_w_gate, B_w_up, B_w_down, gate_w):
    def _A_ref(x, c_kv, w_q, w_uk, w_uv, w_o):
        B, Sq, M = x.shape[0], x.shape[1], x.shape[2]
        Sk = c_kv.shape[1]
        H, D = w_q.shape[1], w_q.shape[2]
        q = jnp.einsum("bqm,mhd->bhqd", x, w_q)
        k = jnp.einsum("bkc,chd->bhkd", c_kv, w_uk)
        v = jnp.einsum("bkc,chd->bhkd", c_kv, w_uv)
        scores = jnp.einsum("bhqd,bhkd->bhqk", q, k) * (D ** -0.5)
        off = Sk - Sq
        qi = jnp.arange(Sq)[:, None]
        kj = jnp.arange(Sk)[None, :]
        cmask = kj <= (qi + off)
        scores = jnp.where(cmask[None, None], scores, -1e9)
        p = _softmax(scores, axis=-1)
        ctx = jnp.einsum("bhqk,bhkd->bhqd", p, v)
        return jnp.einsum("bhqd,hdm->bqm", ctx, w_o)

    def _B_ref(x, w_r, w_gate, w_up, w_down):
        B, S, D = x.shape
        C = 2
        r = x @ w_r
        idx = jnp.argsort(-r, axis=-1)[:, :C]
        idx_e = jnp.repeat(idx.reshape(B, C, 1), D, axis=2)
        x_sel = jnp.take_along_axis(x, idx_e, axis=1)
        g = _silu(x_sel @ w_gate)
        u = x_sel @ w_up
        y = (g * u) @ w_down
        r_sel = _sigmoid(jnp.take_along_axis(r, idx, axis=1))
        y = y * r_sel.reshape(B, C, 1)
        b_off = (jnp.arange(B) * S).reshape(B, 1)
        flat_idx = (idx + b_off).reshape(B * C)
        zero = (x * 0.0).reshape(B * S, D)
        upd = _scatter_add(zero, flat_idx, y.reshape(B * C, D), axis=0)
        return x + upd.reshape(B, S, D)

    x = A_x
    g = _sigmoid((x * gate_w).sum(-1, keepdims=True))
    a = _A_ref(x, A_c_kv, A_w_q, A_w_uk, A_w_uv, A_w_o)
    b = _B_ref(x, B_w_r, B_w_gate, B_w_up, B_w_down)
    return g * a + (1 - g) * b
```

```python
import math

import jax
import jax.numpy as jnp
from jax import lax
import jax.experimental.pallas as pl
import jax.experimental.pallas.tpu as pltpu

S, M, C, H, D, F = 2048, 448, 1024, 16, 256, 1792
TQ = 128
NQ = S // TQ
PB = 512
NPB = S // PB
OB = 512
NOB = S // OB

BF, F32, U32, I32 = jnp.bfloat16, jnp.float32, jnp.uint32, jnp.int32
NN = (((1,), (0,)), ((), ()))
NT = (((1,), (1,)), ((), ()))
LOG2E = math.log2(math.e)
QSCALE = (D ** -0.5) * LOG2E
NEG = -1e9 * LOG2E

SEM_WK, SEM_WV, SEM_WQ, SEM_WO = 0, 2, 4, 6
SEM_CKV, SEM_XT = 8, 8 + NPB
SEM_MISC = 8 + 2 * NPB
SEM_OUT = SEM_MISC + 5
NSEM = SEM_OUT + NOB


def _dot(a, b, dn):
    return lax.dot_general(a, b, dn, preferred_element_type=F32)


def _recip(l):
    r = pl.reciprocal(l, approx=True)
    return r * (2.0 - l * r)


def _sigmoid(z):
    return 1.0 / (1.0 + jnp.exp(-z))


def _task_order():
    npb, nob = PB // TQ, OB // TQ
    t = [("P", 0), ("QK", 0)]
    for j in range(NQ + 1):
        if j < NQ:
            t.append(("SM", j))
        if j >= 1:
            t.append(("PV", j - 1))
        if j + 1 < NQ:
            if (j + 1) % npb == 0:
                t.append(("P", (j + 1) // npb))
            t.append(("QK", j + 1))
        if j >= 2 and (j - 1) % nob == 0:
            t.append(("O", (j - 2) // nob))
    t.append(("O", NOB - 1))
    out, seen = [], set()
    for e in t:
        if e not in seen:
            seen.add(e)
            out.append(e)
    return out


def _kernel(xT_hbm, ckv_hbm, wq_hbm, wk_hbm, wv_hbm, wo_hbm, wr_hbm, wg_hbm,
            wu_hbm, wd_hbm, gw_hbm, out_hbm,
            xT_s, x_s, ckv_s, wq32, wk32, wv32, wo_s, q_s, k_s, v_s, ctx_s, acc,
            wr_s, gw_s, wg_s, wu_s, wd_s, out_s, sem):
    wq_u, wk_u, wv_u = (r.bitcast(U32) for r in (wq_hbm, wk_hbm, wv_hbm))

    def cp(src, dst, s):
        return pltpu.make_async_copy(src, dst, sem.at[s])

    def cp_wk(p, slot): return cp(wk_u.at[:, p, :], wk32.at[slot], SEM_WK + slot)
    def cp_wv(p, slot): return cp(wv_u.at[:, p, :], wv32.at[slot], SEM_WV + slot)
    def cp_wq(p, slot): return cp(wq_u.at[:, p, :], wq32.at[slot], SEM_WQ + slot)
    def cp_wo(h, slot): return cp(wo_hbm.at[h], wo_s.at[slot], SEM_WO + slot)

    def cp_ckv(i):
        r = pl.ds(PB * i, PB)
        return cp(ckv_hbm.at[r, :], ckv_s.at[r, :], SEM_CKV + i)

    def cp_xt(i):
        r = pl.ds(PB * i, PB)
        return cp(xT_hbm.at[:, r], xT_s.at[:, r], SEM_XT + i)

    misc = [cp(wr_hbm, wr_s, SEM_MISC), cp(gw_hbm, gw_s, SEM_MISC + 1),
            cp(wg_hbm, wg_s, SEM_MISC + 2), cp(wu_hbm, wu_s, SEM_MISC + 3),
            cp(wd_hbm, wd_s, SEM_MISC + 4)]

    def cp_out(i):
        r = pl.ds(OB * i, OB)
        return cp(out_s.at[:, r], out_hbm.at[:, r], SEM_OUT + i)

    row = lax.broadcasted_iota(I32, (TQ, TQ), 0)
    col = lax.broadcasted_iota(I32, (TQ, TQ), 1)
    tri = col <= row

    def branch_b_route():
        r16 = lax.broadcasted_iota(I32, (16, M), 0)
        wr = wr_s[...].astype(F32).reshape(1, M)
        gw = gw_s[...].astype(F32).reshape(1, M)
        lhs = jnp.where(r16 == 0, wr, jnp.where(r16 == 1, gw, 0.0)).astype(BF)
        rg = _dot(lhs, xT_s[...], NN)
        r = rg[0:1, :].astype(BF).astype(F32)
        gate = _sigmoid(rg[1:2, :])
        lane = lax.broadcasted_iota(I32, (1, S), 1)
        m1 = jnp.max(r, axis=1, keepdims=True)
        i1 = jnp.min(jnp.where(r == m1, lane, S - 1), axis=1, keepdims=True)
        r2 = jnp.where(lane == i1, -jnp.inf, r)
        m2 = jnp.max(r2, axis=1, keepdims=True)
        i2 = jnp.min(jnp.where((r2 == m2) & (lane != i1), lane, S - 1),
                     axis=1, keepdims=True)
        lane16 = lax.broadcasted_iota(I32, (16, S), 1)
        row16 = lax.broadcasted_iota(I32, (16, S), 0)
        sel = ((row16 == 0) & (lane16 == i1)) | ((row16 == 1) & (lane16 == i2))
        onehot = jnp.where(sel, 1.0, 0.0).astype(BF)
        xsel = _dot(onehot, x_s[...], NN).astype(BF)
        return gate, i1, i2, m1, m2, xsel

    def branch_b_ffn(m1, m2, xsel):
        g = _dot(xsel, wg_s[...], NN)
        u = _dot(xsel, wu_s[...], NN)
        hid = (g * _sigmoid(g) * u).astype(BF)
        y = _dot(hid, wd_s[...], NT)
        y1 = y[0:1, :] * _sigmoid(m1)
        y2 = y[1:2, :] * _sigmoid(m2)
        pad = jnp.zeros((TQ, 512 - M), F32)

        def as_col(v):
            vb = jnp.concatenate([jnp.broadcast_to(v, (TQ, M)), pad], axis=1)
            return vb.T[:M, :]
        return as_col(y1), as_col(y2)

    def head(h, first, last):
        slot = (h // 2) % 2
        oslot = h % 2
        if isinstance(h, int):
            shift = jnp.uint32(16 * (1 - h % 2))
        else:
            shift = (16 * (1 - h % 2)).astype(U32)

        def unpack(w):
            hi = (w << shift) & jnp.uint32(0xFFFF0000)
            return pltpu.bitcast(hi, F32).astype(BF)

        w = {}
        if not first:
            w["kv"] = jnp.concatenate(
                [unpack(wk32[slot]), unpack(wv32[slot])], axis=1)
            w["q"] = unpack(wq32[slot])
        sv, pv, bb = {}, {}, {}
        for kind, i in _task_order():
            if kind == "P":
                rows = slice(PB * i, PB * (i + 1))
                if first:
                    cp_ckv(i).wait()
                if first and i == 0:
                    cp_wk(0, 0).wait()
                    wk = unpack(wk32[0])
                    k_s[rows, :] = _dot(ckv_s[rows, :], wk, NN).astype(BF)
                    cp_wv(0, 0).wait()
                    wv = unpack(wv32[0])
                    v_s[rows, :] = _dot(ckv_s[rows, :], wv, NN).astype(BF)
                    w["kv"] = jnp.concatenate([wk, wv], axis=1)
                else:
                    kv = _dot(ckv_s[rows, :], w["kv"], NN)
                    k_s[rows, :] = kv[:, :D].astype(BF)
                    v_s[rows, :] = kv[:, D:].astype(BF)
                if first:
                    cp_xt(i).wait()
                    x_s[rows, :] = xT_s[:, rows].T
                    if i == 0:
                        cp_wq(0, 0).wait()
                        w["q"] = unpack(wq32[0])
                q_s[rows, :] = (_dot(x_s[rows, :], w["q"], NN) * QSCALE).astype(BF)
                if last and i == 0:
                    bb["route"] = branch_b_route()
                if last and i == 1:
                    gate, i1, i2, m1, m2, xsel = bb["route"]
                    bb["y"] = branch_b_ffn(m1, m2, xsel)
            elif kind == "QK":
                n = TQ * (i + 1)
                s = _dot(q_s[TQ * i:TQ * (i + 1), :], k_s[0:n, :], NT)
                sd = jnp.where(tri, s[:, n - TQ:], NEG)
                s = sd if i == 0 else jnp.concatenate([s[:, :n - TQ], sd], axis=1)
                sv[i] = (s, jnp.max(s, axis=1, keepdims=True))
            elif kind == "SM":
                s, m = sv.pop(i)
                p = jnp.exp2(s - m)
                l = jnp.sum(p, axis=1, keepdims=True)
                pv[i] = (p.astype(BF), _recip(l))
            elif kind == "PV":
                n = TQ * (i + 1)
                p, rl = pv.pop(i)
                o = _dot(p, v_s[0:n, :], NN)
                ctx_s[TQ * i:TQ * (i + 1), :] = (o * rl).astype(BF)
            elif kind == "O":
                cols = slice(OB * i, OB * (i + 1))
                if first and i == 0:
                    cp_wo(0, 0).wait()
                a = _dot(wo_s[oslot], ctx_s[cols, :], NT)
                if first:
                    acc[:, cols] = a
                elif not last:
                    acc[:, cols] += a
                else:
                    a = a + acc[:, cols]
                    gate, i1, i2 = bb["route"][:3]
                    y1, y2 = bb["y"]
                    for t in range(OB // TQ):
                        c0 = OB * i + TQ * t
                        lane = lax.broadcasted_iota(I32, (1, TQ), 1) + c0
                        upd = jnp.where(lane == i1, y1,
                                        jnp.where(lane == i2, y2, 0.0))
                        b = xT_s[:, c0:c0 + TQ].astype(F32) + upd
                        g = gate[:, c0:c0 + TQ]
                        out_s[:, c0:c0 + TQ] = (
                            g * a[:, TQ * t:TQ * (t + 1)] + (1.0 - g) * b
                        ).astype(BF)
                    cp_out(i).start()

    cp_wk(0, 0).start()
    cp_ckv(0).start()
    cp_wv(0, 0).start()
    cp_xt(0).start()
    cp_wq(0, 0).start()
    for i in range(1, NPB):
        cp_ckv(i).start()
        cp_xt(i).start()
        if i == 1:
            cp_wo(0, 0).start()
    cp_wo(1, 1).start()
    cp_wk(1, 1).start()
    cp_wv(1, 1).start()
    cp_wq(1, 1).start()
    for c in misc:
        c.start()
    head(0, True, False)

    def mid(h, carry):
        oslot = h % 2
        cp_wo(h, oslot).wait()
        cp_wo(h + 1, 1 - oslot).start()

        @pl.when(oslot == 0)
        def _():
            p = h // 2
            slot = p % 2
            cp_wk(p, slot).wait()
            cp_wv(p, slot).wait()
            cp_wq(p, slot).wait()

            @pl.when(p + 1 < H // 2)
            def _():
                cp_wk(p + 1, 1 - slot).start()
                cp_wv(p + 1, 1 - slot).start()
                cp_wq(p + 1, 1 - slot).start()

        head(h, False, False)
        return carry

    lax.fori_loop(1, H - 1, mid, 0)

    cp_wo(H - 1, (H - 1) % 2).wait()
    for c in misc:
        c.wait()
    head(H - 1, False, True)
    for i in range(NOB):
        cp_out(i).wait()


@jax.jit
def pallas_gated_mix__compressed_kv_cla__moe_arch_mod__prompt_kernel(
    A_x: jax.Array,
    A_c_kv: jax.Array,
    A_w_q: jax.Array,
    A_w_uk: jax.Array,
    A_w_uv: jax.Array,
    A_w_o: jax.Array,
    B_x: jax.Array,
    B_w_r: jax.Array,
    B_w_gate: jax.Array,
    B_w_up: jax.Array,
    B_w_down: jax.Array,
    gate_w: jax.Array,
):
    del B_x
    xT = A_x.reshape(S, M).T
    ckv = A_c_kv.reshape(S, C)
    woT = jnp.transpose(A_w_o, (0, 2, 1))
    wdT = B_w_down.T

    V = pltpu.VMEM
    scratch = [
        V((M, S), BF),
        V((S, M), BF),
        V((S, C), BF),
        V((2, M, D), U32),
        V((2, C, D), U32),
        V((2, C, D), U32),
        V((2, M, D), BF),
        V((S, D), BF),
        V((S, D), BF),
        V((S, D), BF),
        V((S, D), BF),
        V((M, S), F32),
        V((M,), BF),
        V((M,), BF),
        V((M, F), BF),
        V((M, F), BF),
        V((M, F), BF),
        V((M, S), BF),
        pltpu.SemaphoreType.DMA((NSEM,)),
    ]
    outT = pl.pallas_call(
        _kernel,
        in_specs=[pl.BlockSpec(memory_space=pl.ANY)] * 11,
        out_specs=pl.BlockSpec(memory_space=pl.ANY),
        out_shape=jax.ShapeDtypeStruct((M, S), BF),
        scratch_shapes=scratch,
        compiler_params=pltpu.CompilerParams(
            vmem_limit_bytes=100 * 1024 * 1024),
    )(xT, ckv, A_w_q, A_w_uk, A_w_uv, woT, B_w_r, B_w_gate, B_w_up, wdT, gate_w)
    return outT.T.reshape(1, S, M)
```

```python
import math

import jax
import jax.numpy as jnp
from jax import lax
import jax.experimental.pallas as pl
import jax.experimental.pallas.tpu as pltpu

S, M, C, H, D, F = 2048, 448, 1024, 16, 256, 1792
TQ = 128
NQ = S // TQ
PB = 512
NPB = S // PB
NF = F // TQ

BF, F32, U32, I32 = jnp.bfloat16, jnp.float32, jnp.uint32, jnp.int32
NN = (((1,), (0,)), ((), ()))
NT = (((1,), (1,)), ((), ()))
LOG2E = math.log2(math.e)
QSCALE = (D ** -0.5) * LOG2E
NEG = -1e9 * LOG2E
HI16 = 0xFFFF0000

(S_WK, S_WV, S_WQ, S_WO0, S_WO1, S_WR, S_GW, S_WG, S_WU, S_WD, S_BAR,
 S_BULK) = range(12)
S_CKV = 12
S_XT = S_CKV + NPB
S_OUT = S_XT + NPB
NSEM = S_OUT + NPB


def _dot(a, b, dn):
    return lax.dot_general(a, b, dn, preferred_element_type=F32)


def _recip(l):
    r = pl.reciprocal(l, approx=True)
    return r * (2.0 - l * r)


def _sigmoid(z):
    return 1.0 / (1.0 + jnp.exp(-z))


def _rows(ref, r0, r1):
    return pltpu.bitcast(ref[r0 // 2:r1 // 2, :], BF)


def _cols(ref, c0, c1):
    return pltpu.bitcast(ref[:, c0:c1], BF)


def _put_rows(ref, r0, r1, v):
    ref[r0 // 2:r1 // 2, :] = pltpu.bitcast(v, U32)


def _steady_order(j0):
    t = []
    for j in range(j0, NQ + 2):
        if 1 <= j <= NQ:
            t.append(("PV", j - 1))
        if j + 1 < NQ:
            if (j + 1) % 4 == 0:
                t += [("KV", (j + 1) // 4), ("Q", (j + 1) // 4)]
            t.append(("QK", j + 1))
        if j >= 2 and (j - 1) % 4 == 0:
            t.append(("O", (j - 2) // 4))
    return t


def _dedup(t):
    out, seen = [], set()
    for e in t:
        if e not in seen:
            seen.add(e)
            out.append(e)
    return out


def _mid_order():
    t = [("Q", 0), ("KV", 0), ("QK", 0), ("QK", 1), ("QK", 2), ("QK", 3),
         ("KV", 1), ("PV", 0), ("PV", 1), ("PV", 2), ("Q", 1)]
    return _dedup(t + _steady_order(3))


def _first_order():
    t = [("W", 0), ("K", 0), ("W", 1), ("V", 0), ("W", 2), ("KV", 1),
         ("W", 3), ("T", 0), ("T", 1), ("G4", 0), ("G4", 1), ("Q", 0),
         ("QK", 0), ("QK", 1), ("QK", 2), ("QK", 3), ("Q", 1),
         ("PV", 0), ("PV", 1), ("PV", 2)]
    out = []
    g = 8
    for e in _dedup(t + _steady_order(3)):
        if e == ("KV", 2):
            out += [("W", 4), ("T", 2), ("T", 3)]
        out.append(e)
        if ("W", 4) in out and g < NQ and e[0] in ("KV", "Q", "QK"):
            out.append(("G", g))
            g += 1
    return out


def _second_order():
    out = [("TOPK", 0)]
    small = []
    for c in range(NF + 1):
        if c < NF:
            small += [("FG", c), ("FU", c)]
        if c >= 1:
            small.append(("FD", c - 1))
    started = False
    for e in _mid_order():
        if e == ("O", NPB - 1):
            out += small + [("UPD", 0)]
            small = []
        out.append(e)
        started = started or e == ("KV", 0)
        if started and e[0] in ("KV", "Q", "QK", "O", "PV"):
            n = 2 if e[0] == "KV" else 1
            out += small[:n]
            small = small[n:]
    return out


def _last_order():
    out = []
    for e in _mid_order():
        out.append(e)
        if e == ("O", NPB - 2):
            out.append(("BAR", 0))
    return out


def _kernel(xT_hbm, ckv_hbm, wq_hbm, wk_hbm, wv_hbm, wo_hbm, wr_hbm, wg_hbm,
            wu_hbm, wd_hbm, gw_hbm, out_hbm,
            xT_s, x_s, ckv_s, wq32, wk32, wv32, wo_s, q_s, k_s, v_s, ctx_s, acc,
            r_s, g_s, wr_s, gw_s, bar_s, wg_s, wu_s, wd_s, out_s, sem):
    (xT_u, ckv_u, wq_u, wk_u, wv_u, wo_u, wg_u, wu_u, wd_u) = (
        r.bitcast(U32) for r in (xT_hbm, ckv_hbm, wq_hbm, wk_hbm, wv_hbm,
                                 wo_hbm, wg_hbm, wu_hbm, wd_hbm))

    def cp(src, dst, s):
        return pltpu.make_async_copy(src, dst, sem.at[s])

    def cp_pair(w_u, w_s, p, s):
        return cp(w_u.at[:, p, :], w_s.at[p], s)

    def cp_ckv(i):
        r = pl.ds(PB // 2 * i, PB // 2)
        return cp(ckv_u.at[r, :], ckv_s.at[r, :], S_CKV + i)

    def cp_xt(i):
        r = pl.ds(PB * i, PB)
        return cp(xT_u.at[:, r], xT_s.at[:, r], S_XT + i)

    def cp_out(i):
        r = pl.ds(PB * i, PB)
        return cp(out_s.at[:, r], out_hbm.at[:, r], S_OUT + i)

    c_wk, c_wv, c_wq = (cp_pair(wk_u, wk32, 0, S_WK), cp_pair(wv_u, wv32, 0, S_WV),
                        cp_pair(wq_u, wq32, 0, S_WQ))
    c_wo0, c_wo1 = cp(wo_u.at[0], wo_s.at[0], S_WO0), cp(wo_u.at[1], wo_s.at[1], S_WO1)
    c_wr, c_gw = cp(wr_hbm, wr_s, S_WR), cp(gw_hbm, gw_s, S_GW)
    c_ffn = [cp(wg_u, wg_s, S_WG), cp(wu_u, wu_s, S_WU), cp(wd_u, wd_s, S_WD)]
    c_bar = cp(gw_hbm, bar_s, S_BAR)
    rest = pl.ds(2, H - 2)
    bulk = [cp(wo_u.at[rest], wo_s.at[rest], S_BULK)]
    for p in range(1, H // 2):
        bulk += [cp_pair(wk_u, wk32, p, S_BULK), cp_pair(wv_u, wv32, p, S_BULK),
                 cp_pair(wq_u, wq32, p, S_BULK)]
    first_waits = [
        [c_wk, cp_ckv(0)], [c_wv], [cp_ckv(1)],
        [cp_xt(0), c_wq, cp_xt(1), c_wr, c_gw, c_wo0],
        [cp_ckv(2), cp_xt(2), cp_ckv(3), cp_xt(3)],
    ]

    row = lax.broadcasted_iota(I32, (TQ, TQ), 0)
    col = lax.broadcasted_iota(I32, (TQ, TQ), 1)
    tri = col <= row
    r16 = lax.broadcasted_iota(I32, (16, M), 0)

    def head(h, order, first=False, last=False):
        pair = h // 2
        if isinstance(h, int):
            shift = jnp.uint32(16 * (1 - h % 2))
        else:
            shift = (16 * (1 - h % 2)).astype(U32)

        cache = {}

        def weight(name, ref):
            if name not in cache:
                hi = (ref[pair] << shift) & jnp.uint32(HI16)
                cache[name] = pltpu.bitcast(hi, F32).astype(BF)
            return cache[name]

        def route(c0, c1):
            if "rg" not in cache:
                wr = wr_s[...].astype(F32).reshape(1, M)
                gw = gw_s[...].astype(F32).reshape(1, M)
                cache["rg"] = jnp.where(
                    r16 == 0, wr, jnp.where(r16 == 1, gw, 0.0)).astype(BF)
            rg = _dot(cache["rg"], _cols(xT_s, c0, c1), NN)
            r_s[:, c0:c1] = rg[0:1, :].astype(BF).astype(F32)
            g_s[:, c0:c1] = _sigmoid(rg[1:2, :])

        sv, rinv, b = {}, {}, {}
        for kind, i in order:
            r0, r1 = PB * i, PB * (i + 1)
            t0, t1 = TQ * i, TQ * (i + 1)
            if kind == "W":
                for c in first_waits[i]:
                    c.wait()
                if i == len(first_waits) - 1:
                    for c in bulk:
                        c.start()
            elif kind == "BAR":
                c_bar.wait()
            elif kind == "T":
                _put_rows(x_s, r0, r1, _cols(xT_s, r0, r1).T)
            elif kind == "G4":
                route(r0, r1)
            elif kind == "G":
                route(t0, t1)
            elif kind == "K":
                k = _dot(_rows(ckv_s, r0, r1), weight("k", wk32), NN)
                _put_rows(k_s, r0, r1, k.astype(BF))
            elif kind == "V":
                v = _dot(_rows(ckv_s, r0, r1), weight("v", wv32), NN)
                _put_rows(v_s, r0, r1, v.astype(BF))
            elif kind == "KV":
                wkv = jnp.concatenate([weight("k", wk32), weight("v", wv32)], axis=1)
                kv = _dot(_rows(ckv_s, r0, r1), wkv, NN)
                _put_rows(k_s, r0, r1, kv[:, :D].astype(BF))
                _put_rows(v_s, r0, r1, kv[:, D:].astype(BF))
            elif kind == "Q":
                q = _dot(_rows(x_s, r0, r1), weight("q", wq32), NN) * QSCALE
                _put_rows(q_s, r0, r1, q.astype(BF))
            elif kind == "QK":
                s = _dot(_rows(q_s, t0, t1), _rows(k_s, 0, t1), NT)
                sd = jnp.where(tri, s[:, t0:], NEG)
                s = sd if i == 0 else jnp.concatenate([s[:, :t0], sd], axis=1)
                sv[i] = (s, jnp.max(s, axis=1, keepdims=True))
            elif kind == "PV":
                s, m = sv.pop(i)
                p = jnp.exp2(s - m).astype(BF)
                _put_rows(ctx_s, t0, t1, _dot(p, _rows(v_s, 0, t1), NN).astype(BF))
                pf = p.astype(F32)
                la = pf[:, 0:TQ]
                for t in range(1, i + 1):
                    la = la + pf[:, TQ * t:TQ * (t + 1)]
                hi = la.astype(BF)
                lo = (la - hi.astype(F32)).astype(BF)
                l = _dot(jnp.ones((16, 2 * TQ), BF),
                         jnp.concatenate([hi, lo], axis=1), NT)[0:1, :]
                rinv[i] = _recip(l)
            elif kind == "O":
                a = _dot(pltpu.bitcast(wo_s[h], BF), _rows(ctx_s, r0, r1), NT)
                g = g_s[:, r0:r1]
                a = a * (g * jnp.concatenate(
                    [rinv.pop(t) for t in range(4 * i, 4 * i + 4)], axis=1))
                if first:
                    acc[:, r0:r1] = a + (1.0 - g) * _cols(xT_s, r0, r1).astype(F32)
                elif not last:
                    acc[:, r0:r1] += a
                else:
                    out_s[:, r0:r1] = (acc[:, r0:r1] + a).astype(BF)
                    cp_out(i).start()
            elif kind == "TOPK":
                r = r_s[...]
                lane = lax.broadcasted_iota(I32, (1, S), 1)
                m1 = jnp.max(r, axis=1, keepdims=True)
                i1 = jnp.min(jnp.where(r == m1, lane, S - 1))
                r2 = jnp.where(lane == i1, -jnp.inf, r)
                m2 = jnp.max(r2, axis=1, keepdims=True)
                i2 = jnp.min(jnp.where((r2 == m2) & (lane != i1), lane, S - 1))

                def token(idx):
                    w = x_s[pl.ds(idx // 2, 1), :]
                    sh = (16 * (1 - idx % 2)).astype(U32)
                    return pltpu.bitcast((w << sh) & jnp.uint32(HI16), F32)
                b["x"] = jnp.where(r16 == 0, token(i1),
                                   jnp.where(r16 == 1, token(i2), 0.0)).astype(BF)
                b["sel"] = ((i1, m1), (i2, m2))
            elif kind == "FG":
                b["g", i] = _dot(b["x"], _cols(wg_s, t0, t1), NN)
            elif kind == "FU":
                b["u", i] = _dot(b["x"], _cols(wu_s, t0, t1), NN)
            elif kind == "FD":
                g, u = b.pop(("g", i)), b.pop(("u", i))
                hid = (g * _sigmoid(g) * u).astype(BF)
                y = _dot(hid, _cols(wd_s, t0, t1), NT)
                b["y"] = y if i == 0 else b["y"] + y
            elif kind == "UPD":
                pad = jnp.zeros((TQ, 512 - M), F32)
                lane = lax.broadcasted_iota(I32, (1, TQ), 1)
                for t, (idx, score) in enumerate(b["sel"]):
                    yb = jnp.broadcast_to(b["y"][t:t + 1, :] * _sigmoid(score), (TQ, M))
                    ycol = jnp.concatenate([yb, pad], axis=1).T[:M, :]
                    blk = pl.ds(pl.multiple_of(idx // TQ * TQ, TQ), TQ)
                    old = acc[:, blk]
                    acc[:, blk] = jnp.where(lane == idx % TQ,
                                            old + (1.0 - g_s[:, blk]) * ycol, old)

    for grp in first_waits:
        for c in grp:
            c.start()
    for c in [c_wo1] + c_ffn + [c_bar]:
        c.start()
    head(0, _first_order(), first=True)

    for c in [c_wo1] + c_ffn:
        c.wait()
    head(1, _second_order())

    for c in bulk:
        c.wait()

    def mid(h, carry):
        head(h, _mid_order())
        return carry

    lax.fori_loop(2, H - 1, mid, 0)

    head(H - 1, _last_order(), last=True)
    for i in range(NPB):
        cp_out(i).wait()


@jax.jit
def pallas_gated_mix__compressed_kv_cla__moe_arch_mod__prompt_kernel(
    A_x: jax.Array,
    A_c_kv: jax.Array,
    A_w_q: jax.Array,
    A_w_uk: jax.Array,
    A_w_uv: jax.Array,
    A_w_o: jax.Array,
    B_x: jax.Array,
    B_w_r: jax.Array,
    B_w_gate: jax.Array,
    B_w_up: jax.Array,
    B_w_down: jax.Array,
    gate_w: jax.Array,
):
    del B_x
    xT = A_x.reshape(S, M).T
    ckv = A_c_kv.reshape(S, C)
    woT = jnp.transpose(A_w_o, (0, 2, 1))
    wdT = B_w_down.T

    V = pltpu.VMEM
    scratch = [
        V((M // 2, S), U32),
        V((S // 2, M), U32),
        V((S // 2, C), U32),
        V((H // 2, M, D), U32),
        V((H // 2, C, D), U32),
        V((H // 2, C, D), U32),
        V((H, M // 2, D), U32),
        V((S // 2, D), U32),
        V((S // 2, D), U32),
        V((S // 2, D), U32),
        V((S // 2, D), U32),
        V((M, S), F32),
        V((1, S), F32),
        V((1, S), F32),
        V((M,), BF),
        V((M,), BF),
        V((M,), BF),
        V((M // 2, F), U32),
        V((M // 2, F), U32),
        V((M // 2, F), U32),
        V((M, S), BF),
        pltpu.SemaphoreType.DMA((NSEM,)),
    ]
    outT = pl.pallas_call(
        _kernel,
        in_specs=[pl.BlockSpec(memory_space=pl.ANY)] * 11,
        out_specs=pl.BlockSpec(memory_space=pl.ANY),
        out_shape=jax.ShapeDtypeStruct((M, S), BF),
        scratch_shapes=scratch,
        compiler_params=pltpu.CompilerParams(
            vmem_limit_bytes=100 * 1024 * 1024),
    )(xT, ckv, A_w_q, A_w_uk, A_w_uv, woT, B_w_r, B_w_gate, B_w_up, wdT, gate_w)
    return outT.T.reshape(1, S, M)
```

```python
import math

import jax
import jax.numpy as jnp
from jax import lax
import jax.experimental.pallas as pl
import jax.experimental.pallas.tpu as pltpu

S, M, C, H, D, F = 2048, 448, 1024, 16, 256, 1792
TQ = 128
NQ = S // TQ
PB = 512
NPB = S // PB
NF = F // TQ

BF, F32, U32, I32 = jnp.bfloat16, jnp.float32, jnp.uint32, jnp.int32
NN = (((1,), (0,)), ((), ()))
NT = (((1,), (1,)), ((), ()))
LOG2E = math.log2(math.e)
QSCALE = (D ** -0.5) * LOG2E
NEG = -1e9 * LOG2E
HI16 = 0xFFFF0000

S_WK, S_WV, S_HEAD0, S_HEAD1, S_BULK, S_OUT, S_CKV = range(7)
NSEM = S_CKV + NPB


def _dot(a, b, dn):
    return lax.dot_general(a, b, dn, preferred_element_type=F32)


def _recip(l):
    r = pl.reciprocal(l, approx=True)
    return r * (2.0 - l * r)


def _sigmoid(z):
    return 1.0 / (1.0 + jnp.exp(-z))


def _rows(ref, r0, r1):
    return pltpu.bitcast(ref[r0 // 2:r1 // 2, :], BF)


def _cols(ref, c0, c1):
    return pltpu.bitcast(ref[:, c0:c1], BF)


def _put_rows(ref, r0, r1, v):
    ref[r0 // 2:r1 // 2, :] = pltpu.bitcast(v, U32)


def _steady_order(j0):
    t = []
    for j in range(j0, NQ + 2):
        if 1 <= j <= NQ:
            t.append(("PV", j - 1))
        if j + 1 < NQ:
            if (j + 1) % 4 == 0:
                t += [("KV", (j + 1) // 4), ("Q", (j + 1) // 4)]
            t.append(("QK", j + 1))
        if j >= 2 and (j - 1) % 4 == 0:
            t.append(("O", (j - 2) // 4))
    return t


def _dedup(t):
    out, seen = [], set()
    for e in t:
        if e not in seen:
            seen.add(e)
            out.append(e)
    return out


def _mid_order():
    t = [("Q", 0), ("KV", 0), ("QK", 0), ("QK", 1), ("QK", 2), ("QK", 3),
         ("KV", 1), ("PV", 0), ("PV", 1), ("PV", 2), ("Q", 1)]
    return _dedup(t + _steady_order(3))


def _first_order():
    t = [("T", 0), ("T", 1), ("T", 2), ("T", 3), ("G4", 0), ("G4", 1), ("Q", 0),
         ("QK", 0), ("QK", 1), ("QK", 2), ("QK", 3), ("Q", 1),
         ("PV", 0), ("PV", 1), ("PV", 2)]
    out = []
    g = 8
    for e in _dedup(t + _steady_order(3)):
        if e[0] == "KV":
            continue
        out.append(e)
        if ("Q", 1) in out and g < NQ and e[0] in ("Q", "QK"):
            out.append(("G", g))
            g += 1
        if e == ("O", 1):
            out.append(("TOPK", 0))
    return out


def _loop_order():
    out = []
    for e in _mid_order():
        if e == ("O", NPB - 1):
            out.append(("UPD", 0))
        out.append(e)
        if e == ("KV", 0):
            out.append(("FG", 0))
        if e == ("KV", 1):
            out.append(("FU", 0))
        if e == ("KV", 2):
            out.append(("FD", 0))
    return out


def _kernel(xT_hbm, ckv_hbm, wq_hbm, wk_hbm, wv_hbm, wo_hbm, wr_hbm, wg_hbm,
            wu_hbm, wd_hbm, gw_hbm, out_hbm,
            xT_s, x_s, ckv_s, wq32, wkv32, wo_s, q_s, kv_s, ctx_s, acc,
            r_s, g_s, wr_s, gw_s, wg_s, wu_s, wd_s, xsel_s, sig_s, idx_s,
            out_s, sem):
    wk32, wv32 = wkv32.at[0], wkv32.at[1]
    k_s, v_s = kv_s.at[0], kv_s.at[1]
    (xT_u, ckv_u, wq_u, wk_u, wv_u, wo_u, wg_u, wu_u, wd_u) = (
        r.bitcast(U32) for r in (xT_hbm, ckv_hbm, wq_hbm, wk_hbm, wv_hbm,
                                 wo_hbm, wg_hbm, wu_hbm, wd_hbm))

    def cp(src, dst, s):
        return pltpu.make_async_copy(src, dst, sem.at[s])

    def cp_pair(w_u, w_s, p, s):
        return cp(w_u.at[:, p, :], w_s.at[p], s)

    def cp_ckv(i):
        r = pl.ds(pl.multiple_of(PB // 2 * i, PB // 2), PB // 2)
        return cp(ckv_u.at[r, :], ckv_s.at[r, :], S_CKV + i)

    def cp_out(i):
        r = pl.ds(PB * i, PB)
        return cp(out_s.at[:, r], out_hbm.at[:, r], S_OUT)

    c_wk, c_wv = cp_pair(wk_u, wk32, 0, S_WK), cp_pair(wv_u, wv32, 0, S_WV)
    head0 = [cp(xT_u, xT_s, S_HEAD0), cp_pair(wq_u, wq32, 0, S_HEAD0),
             cp(wr_hbm, wr_s, S_HEAD0), cp(gw_hbm, gw_s, S_HEAD0),
             cp(wo_u.at[0], wo_s.at[0], S_HEAD0)]
    head1 = [cp(wo_u.at[1], wo_s.at[1], S_HEAD1), cp(wg_u, wg_s, S_HEAD1),
             cp(wu_u, wu_s, S_HEAD1), cp(wd_u, wd_s, S_HEAD1)]
    rest = pl.ds(2, H - 2)
    bulk = [cp(wo_u.at[rest], wo_s.at[rest], S_BULK)]
    for p in range(1, H // 2):
        bulk += [cp_pair(wk_u, wk32, p, S_BULK), cp_pair(wv_u, wv32, p, S_BULK),
                 cp_pair(wq_u, wq32, p, S_BULK)]

    row = lax.broadcasted_iota(I32, (TQ, TQ), 0)
    col = lax.broadcasted_iota(I32, (TQ, TQ), 1)
    tri = col <= row
    r16 = lax.broadcasted_iota(I32, (16, M), 0)

    def head(h, order, first=False):
        pair = h // 2
        if isinstance(h, int):
            shift = jnp.uint32(16 * (1 - h % 2))
        else:
            shift = (16 * (1 - h % 2)).astype(U32)

        cache = {}

        def weight(name, ref):
            if name not in cache:
                hi = (ref[pair] << shift) & jnp.uint32(HI16)
                cache[name] = pltpu.bitcast(hi, F32).astype(BF)
            return cache[name]

        def route(c0, c1):
            if "rg" not in cache:
                wr = wr_s[...].astype(F32).reshape(1, M)
                gw = gw_s[...].astype(F32).reshape(1, M)
                cache["rg"] = jnp.where(
                    r16 == 0, wr, jnp.where(r16 == 1, gw, 0.0)).astype(BF)
            rg = _dot(cache["rg"], _cols(xT_s, c0, c1), NN)
            r_s[:, c0:c1] = rg[0:1, :].astype(BF).astype(F32)
            g_s[:, c0:c1] = _sigmoid(rg[1:2, :])

        sv, rinv, b = {}, {}, {}
        for kind, i in order:
            r0, r1 = PB * i, PB * (i + 1)
            t0, t1 = TQ * i, TQ * (i + 1)
            if kind == "T":
                _put_rows(x_s, r0, r1, _cols(xT_s, r0, r1).T)
            elif kind == "G4":
                route(r0, r1)
            elif kind == "G":
                route(t0, t1)
            elif kind == "KV":
                wkv = jnp.concatenate([weight("k", wk32), weight("v", wv32)], axis=1)
                kv = _dot(_rows(ckv_s, r0, r1), wkv, NN)
                _put_rows(k_s, r0, r1, kv[:, :D].astype(BF))
                _put_rows(v_s, r0, r1, kv[:, D:].astype(BF))
            elif kind == "Q":
                q = _dot(_rows(x_s, r0, r1), weight("q", wq32), NN) * QSCALE
                _put_rows(q_s, r0, r1, q.astype(BF))
            elif kind == "QK":
                s = _dot(_rows(q_s, t0, t1), _rows(k_s, 0, t1), NT)
                sd = jnp.where(tri, s[:, t0:], NEG)
                s = sd if i == 0 else jnp.concatenate([s[:, :t0], sd], axis=1)
                sv[i] = (s, jnp.max(s, axis=1, keepdims=True))
            elif kind == "PV":
                s, m = sv.pop(i)
                p = jnp.exp2(s - m).astype(BF)
                _put_rows(ctx_s, t0, t1, _dot(p, _rows(v_s, 0, t1), NN).astype(BF))
                pf = p.astype(F32)
                la = pf[:, 0:TQ]
                for t in range(1, i + 1):
                    la = la + pf[:, TQ * t:TQ * (t + 1)]
                hi = la.astype(BF)
                lo = (la - hi.astype(F32)).astype(BF)
                l = _dot(jnp.ones((16, 2 * TQ), BF),
                         jnp.concatenate([hi, lo], axis=1), NT)[0:1, :]
                rinv[i] = _recip(l)
            elif kind == "O":
                a = _dot(pltpu.bitcast(wo_s[h], BF), _rows(ctx_s, r0, r1), NT)
                g = g_s[:, r0:r1]
                a = a * (g * jnp.concatenate(
                    [rinv.pop(t) for t in range(4 * i, 4 * i + 4)], axis=1))
                if first:
                    acc[:, r0:r1] = a + (1.0 - g) * _cols(xT_s, r0, r1).astype(F32)
                else:
                    a = acc[:, r0:r1] + a
                    acc[:, r0:r1] = a
                    out_s[:, r0:r1] = a.astype(BF)

                    @pl.when(h == H - 1)
                    def _():
                        cp_out(i).start()
            elif kind == "TOPK":
                r = r_s[...]
                lane = lax.broadcasted_iota(I32, (1, S), 1)
                m1 = jnp.max(r, axis=1, keepdims=True)
                i1 = jnp.min(jnp.where(r == m1, lane, S - 1))
                r2 = jnp.where(lane == i1, -jnp.inf, r)
                m2 = jnp.max(r2, axis=1, keepdims=True)
                i2 = jnp.min(jnp.where((r2 == m2) & (lane != i1), lane, S - 1))

                def token(idx):
                    w = x_s[pl.ds(idx // 2, 1), :]
                    sh = (16 * (1 - idx % 2)).astype(U32)
                    return pltpu.bitcast((w << sh) & jnp.uint32(HI16), F32)
                xsel = jnp.where(r16 == 0, token(i1),
                                 jnp.where(r16 == 1, token(i2), 0.0))
                xsel_s[...] = pltpu.bitcast(xsel.astype(BF), U32)
                r8 = lax.broadcasted_iota(I32, (8, TQ), 0)
                sig_s[...] = jnp.where(r8 == 0, _sigmoid(m1), _sigmoid(m2))
                idx_s[0] = i1
                idx_s[1] = i2
            elif kind in ("FG", "FU"):
                chunk = jnp.minimum(h - 1, NF - 1)
                b["c"] = pl.ds(pl.multiple_of(chunk * TQ, TQ), TQ)
                w_s = wg_s if kind == "FG" else wu_s
                b[kind] = _dot(pltpu.bitcast(xsel_s[...], BF),
                               pltpu.bitcast(w_s[:, b["c"]], BF), NN)
            elif kind == "FD":
                g, u = b["FG"], b["FU"]
                hid = (g * _sigmoid(g) * u).astype(BF)
                b["y"] = _dot(hid, pltpu.bitcast(wd_s[:, b["c"]], BF), NT)
            elif kind == "UPD":
                pad = jnp.zeros((TQ, 512 - M), F32)
                lane = lax.broadcasted_iota(I32, (1, TQ), 1)
                for t in range(2):
                    idx = idx_s[t]
                    yb = jnp.broadcast_to(
                        b["y"][t:t + 1, :] * sig_s[t:t + 1, 0:1], (TQ, M))
                    ycol = jnp.concatenate([yb, pad], axis=1).T[:M, :]
                    blk = pl.ds(pl.multiple_of(idx // TQ * TQ, TQ), TQ)
                    hit = lane == jnp.where(h <= NF, idx % TQ, -1)
                    old = acc[:, blk]
                    acc[:, blk] = jnp.where(
                        hit, old + (1.0 - g_s[:, blk]) * ycol, old)

    for c in [c_wk, cp_ckv(0), c_wv] + [cp_ckv(i) for i in range(1, NPB)]:
        c.start()
    for c in head0 + head1 + bulk:
        c.start()

    def proj0(t, carry):
        which, blk = t % 2, t // 2

        @pl.when(t == 0)
        def _():
            c_wk.wait()

        @pl.when(t == 1)
        def _():
            c_wv.wait()

        @pl.when(which == 0)
        def _():
            cp_ckv(blk).wait()

        r = pl.ds(pl.multiple_of(blk * (PB // 2), PB // 2), PB // 2)
        w = pltpu.bitcast(wkv32[which, 0] << 16, F32).astype(BF)
        y = _dot(pltpu.bitcast(ckv_s[r, :], BF), w, NN)
        kv_s[which, r, :] = pltpu.bitcast(y.astype(BF), U32)
        return carry

    lax.fori_loop(0, 2 * NPB, proj0, 0)
    for c in head0:
        c.wait()
    head(0, _first_order(), first=True)
    for c in head1:
        c.wait()

    def step(h, carry):
        @pl.when(h == 2)
        def _():
            for c in bulk:
                c.wait()

        head(h, _loop_order())
        return carry

    lax.fori_loop(1, H, step, 0)
    for i in range(NPB):
        cp_out(i).wait()


@jax.jit
def pallas_gated_mix__compressed_kv_cla__moe_arch_mod__prompt_kernel(
    A_x: jax.Array,
    A_c_kv: jax.Array,
    A_w_q: jax.Array,
    A_w_uk: jax.Array,
    A_w_uv: jax.Array,
    A_w_o: jax.Array,
    B_x: jax.Array,
    B_w_r: jax.Array,
    B_w_gate: jax.Array,
    B_w_up: jax.Array,
    B_w_down: jax.Array,
    gate_w: jax.Array,
):
    del B_x
    xT = A_x.reshape(S, M).T
    ckv = A_c_kv.reshape(S, C)
    woT = jnp.transpose(A_w_o, (0, 2, 1))
    wdT = B_w_down.T

    V = pltpu.VMEM
    scratch = [
        V((M // 2, S), U32),
        V((S // 2, M), U32),
        V((S // 2, C), U32),
        V((H // 2, M, D), U32),
        V((2, H // 2, C, D), U32),
        V((H, M // 2, D), U32),
        V((S // 2, D), U32),
        V((2, S // 2, D), U32),
        V((S // 2, D), U32),
        V((M, S), F32),
        V((1, S), F32),
        V((1, S), F32),
        V((M,), BF),
        V((M,), BF),
        V((M // 2, F), U32),
        V((M // 2, F), U32),
        V((M // 2, F), U32),
        V((8, M), U32),
        V((8, TQ), F32),
        pltpu.SMEM((2,), I32),
        V((M, S), BF),
        pltpu.SemaphoreType.DMA((NSEM,)),
    ]
    outT = pl.pallas_call(
        _kernel,
        in_specs=[pl.BlockSpec(memory_space=pl.ANY)] * 11,
        out_specs=pl.BlockSpec(memory_space=pl.ANY),
        out_shape=jax.ShapeDtypeStruct((M, S), BF),
        scratch_shapes=scratch,
        compiler_params=pltpu.CompilerParams(
            vmem_limit_bytes=100 * 1024 * 1024),
    )(xT, ckv, A_w_q, A_w_uk, A_w_uv, woT, B_w_r, B_w_gate, B_w_up, wdT, gate_w)
    return outT.T.reshape(1, S, M)
```

```python
import math
import re
_CFG = {'fpos': 'FV:KV0'}


def E(k, d=''):
    return _CFG.get(k, d)
def _parse(txt):
    return [(re.match(r'[A-Z]+4?(?=\d)', t).group() if t.startswith('G4') else re.match(r'[A-Z]+', t).group(), int(re.search(r'(\d+)$', t[2:] if t.startswith('G4') else t).group())) for t in txt.split(',')]

import jax
import jax.numpy as jnp
from jax import lax
import jax.experimental.pallas as pl
import jax.experimental.pallas.tpu as pltpu

S, M, C, H, D, F = 2048, 448, 1024, 16, 256, 1792
TQ = 128
NQ = S // TQ
PB = 512
NPB = S // PB
NF = F // TQ

BF, F32, U32, I32 = jnp.bfloat16, jnp.float32, jnp.uint32, jnp.int32
NN = (((1,), (0,)), ((), ()))
NT = (((1,), (1,)), ((), ()))
LOG2E = math.log2(math.e)
QSCALE = (D ** -0.5) * LOG2E
NEG = -1e9 * LOG2E
HI16 = 0xFFFF0000

S_WK, S_WV, S_HEAD0, S_HEAD1, S_BULK, S_OUT, S_CKV = range(7)
NSEM = S_CKV + NPB


HYB = int(E('hyb', 14))
VF = E('ffn', 'vpu') == 'vpu'


def _dot(a, b, dn):
    return lax.dot_general(a, b, dn, preferred_element_type=F32)


def _recip(l):
    r = pl.reciprocal(l, approx=True)
    return r * (2.0 - l * r)


def _sigmoid(z):
    return 1.0 / (1.0 + jnp.exp(-z))


def _rows(ref, r0, r1):
    return pltpu.bitcast(ref[r0 // 2:r1 // 2, :], BF)


def _cols(ref, c0, c1):
    return pltpu.bitcast(ref[:, c0:c1], BF)


def _put_rows(ref, r0, r1, v):
    ref[r0 // 2:r1 // 2, :] = pltpu.bitcast(v, U32)


def _steady_order(j0):
    t = []
    for j in range(j0, NQ + 2):
        if 1 <= j <= NQ:
            t.append(("PV", j - 1))
        if j + 1 < NQ:
            if (j + 1) % 4 == 0:
                t += [("KV", (j + 1) // 4), ("Q", (j + 1) // 4)]
            t.append(("QK", j + 1))
        if j >= 2 and (j - 1) % 4 == 0:
            t.append(("O", (j - 2) // 4))
    return t


def _dedup(t):
    out, seen = [], set()
    for e in t:
        if e not in seen:
            seen.add(e)
            out.append(e)
    return out


def _mid_order():
    t = [("Q", 0), ("KV", 0), ("QK", 0), ("QK", 1), ("QK", 2), ("QK", 3),
         ("KV", 1), ("PV", 0), ("PV", 1), ("PV", 2), ("Q", 1)]
    return _dedup(t + _steady_order(3))


def _first_order():
    if E('first'):
        return _parse(E('first'))
    t = [("T", 0), ("T", 1), ("T", 2), ("T", 3), ("G4", 0), ("G4", 1), ("Q", 0),
         ("QK", 0), ("QK", 1), ("QK", 2), ("QK", 3), ("Q", 1),
         ("PV", 0), ("PV", 1), ("PV", 2)]
    out = []
    g = 8
    for e in _dedup(t + _steady_order(3)):
        if e[0] == "KV":
            continue
        out.append(e)
        if ("Q", 1) in out and g < NQ and e[0] in ("Q", "QK"):
            out.append(("G", g))
            g += 1
        if e == ("O", 1):
            out.append(("TOPK", 0))
    return out


def _loop_order():
    if E('loop'):
        return _parse(E('loop'))
    pos = dict(kv.split(':') for kv in E('fpos', 'FV:KV1' if VF else 'FG:KV1;FU:KV2;FD:KV3;UPD:QK15').split(';'))
    base = _mid_order()
    if E('head'):
        hd = _parse(E('head')); base = _dedup(hd + base)
    if E('tail'):
        tl = _parse(E('tail')); base = [e for e in base if e not in tl] + tl
    out = []
    for e in base:
        out.append(e)
        for k in ('FG', 'FU', 'FD', 'UPD', 'FV'):
            if pos.get(k) == '%s%d' % e:
                out.append((k, 0))
    return out
    out = []
    for e in _mid_order():
        if e == ("O", NPB - 1):
            out.append(("UPD", 0))
        out.append(e)
        if e == ("KV", 0):
            out.append(("FG", 0))
        if e == ("KV", 1):
            out.append(("FU", 0))
        if e == ("KV", 2):
            out.append(("FD", 0))
    return out


def _kernel(xT_hbm, ckv_hbm, wq_hbm, wk_hbm, wv_hbm, wo_hbm, wr_hbm, wg_hbm,
            wu_hbm, wd_hbm, gw_hbm, out_hbm,
            xT_s, x_s, ckv_s, wq32, wkv32, wo_s, q_s, kv_s, ctx_s, acc,
            r_s, g_s, wr_s, gw_s, wg_s, wu_s, wd_s, xsel_s, sig_s, idx_s, xcol_s, ypart_s,
            out_s, sem):
    wk32, wv32 = wkv32.at[0], wkv32.at[1]
    k_s, v_s = kv_s.at[0], kv_s.at[1]
    (xT_u, ckv_u, wq_u, wk_u, wv_u, wo_u, wg_u, wu_u, wd_u) = (
        r.bitcast(U32) for r in (xT_hbm, ckv_hbm, wq_hbm, wk_hbm, wv_hbm,
                                 wo_hbm, wg_hbm, wu_hbm, wd_hbm))

    def cp(src, dst, s):
        return pltpu.make_async_copy(src, dst, sem.at[s])

    def cp_pair(w_u, w_s, p, s):
        return cp(w_u.at[:, p, :], w_s.at[p], s)

    def cp_ckv(i):
        r = pl.ds(pl.multiple_of(PB // 2 * i, PB // 2), PB // 2)
        return cp(ckv_u.at[r, :], ckv_s.at[r, :], S_CKV + i)

    def cp_out(i):
        r = pl.ds(PB * i, PB)
        return cp(out_s.at[:, r], out_hbm.at[:, r], S_OUT)

    c_wk, c_wv = cp_pair(wk_u, wk32, 0, S_WK), cp_pair(wv_u, wv32, 0, S_WV)
    head0 = [cp(xT_u, xT_s, S_HEAD0), cp_pair(wq_u, wq32, 0, S_HEAD0),
             cp(wr_hbm, wr_s, S_HEAD0), cp(gw_hbm, gw_s, S_HEAD0),
             cp(wo_u.at[0], wo_s.at[0], S_HEAD0)]
    head1 = [cp(wo_u.at[1], wo_s.at[1], S_HEAD1), cp(wg_u, wg_s, S_HEAD1),
             cp(wu_u, wu_s, S_HEAD1), cp(wd_u, wd_s, S_HEAD1)]
    rest = pl.ds(2, H - 2)
    bulk = [cp(wo_u.at[rest], wo_s.at[rest], S_BULK)]
    for p in range(1, H // 2):
        bulk += [cp_pair(wk_u, wk32, p, S_BULK), cp_pair(wv_u, wv32, p, S_BULK),
                 cp_pair(wq_u, wq32, p, S_BULK)]

    row = lax.broadcasted_iota(I32, (TQ, TQ), 0)
    col = lax.broadcasted_iota(I32, (TQ, TQ), 1)
    tri = col <= row
    r16 = lax.broadcasted_iota(I32, (16, M), 0)

    def head(h, order, first=False):
        pair = h // 2
        if isinstance(h, int):
            shift = jnp.uint32(16 * (1 - h % 2))
        else:
            shift = (16 * (1 - h % 2)).astype(U32)

        cache = {}

        def weight(name, ref):
            if name not in cache:
                hi = (ref[pair] << shift) & jnp.uint32(HI16)
                cache[name] = pltpu.bitcast(hi, F32).astype(BF)
            return cache[name]

        def route(c0, c1):
            if "rg" not in cache:
                wr = wr_s[...].astype(F32).reshape(1, M)
                gw = gw_s[...].astype(F32).reshape(1, M)
                cache["rg"] = jnp.where(
                    r16 == 0, wr, jnp.where(r16 == 1, gw, 0.0)).astype(BF)
            rg = _dot(cache["rg"], _cols(xT_s, c0, c1), NN)
            r_s[:, c0:c1] = rg[0:1, :].astype(BF).astype(F32)
            g_s[:, c0:c1] = _sigmoid(rg[1:2, :])

        sv, rinv, b = {}, {}, {}
        for kind, i in order:
            r0, r1 = PB * i, PB * (i + 1)
            t0, t1 = TQ * i, TQ * (i + 1)
            if kind == "T":
                _put_rows(x_s, r0, r1, _cols(xT_s, r0, r1).T)
            elif kind == "G4":
                route(r0, r1)
            elif kind == "G":
                route(t0, t1)
            elif kind == "KV":
                wkv = jnp.concatenate([weight("k", wk32), weight("v", wv32)], axis=1)
                kv = _dot(_rows(ckv_s, r0, r1), wkv, NN)
                _put_rows(k_s, r0, r1, kv[:, :D].astype(BF))
                _put_rows(v_s, r0, r1, kv[:, D:].astype(BF))
            elif kind == "Q":
                q = _dot(_rows(x_s, r0, r1), weight("q", wq32), NN) * QSCALE
                _put_rows(q_s, r0, r1, q.astype(BF))
            elif kind == "QK":
                s = _dot(_rows(q_s, t0, t1), _rows(k_s, 0, t1), NT)
                sd = jnp.where(tri, s[:, t0:], NEG)
                s = sd if i == 0 else jnp.concatenate([s[:, :t0], sd], axis=1)
                sv[i] = (s, jnp.max(s, axis=1, keepdims=True))
            elif kind == "PV":
                s, m = sv.pop(i)
                p = jnp.exp2(s - m).astype(BF)
                o = _dot(p, _rows(v_s, 0, t1), NN)
                pf = p.astype(F32)
                if i < HYB:
                    o = o * _recip(jnp.sum(pf, axis=1, keepdims=True))
                    rinv[i] = None
                _put_rows(ctx_s, t0, t1, o.astype(BF))
                if i >= HYB:
                    la = pf[:, 0:TQ]
                    for t in range(1, i + 1):
                        la = la + pf[:, TQ * t:TQ * (t + 1)]
                    hi = la.astype(BF)
                    lo = (la - hi.astype(F32)).astype(BF)
                    l = _dot(jnp.ones((16, 2 * TQ), BF),
                             jnp.concatenate([hi, lo], axis=1), NT)[0:1, :]
                    rinv[i] = _recip(l)
            elif kind == "O":
                a = _dot(pltpu.bitcast(wo_s[h], BF), _rows(ctx_s, r0, r1), NT)
                g = g_s[:, r0:r1]
                f = []
                for t in range(4):
                    gt, rt = g[:, TQ * t:TQ * (t + 1)], rinv.pop(4 * i + t)
                    f.append(gt if rt is None else gt * rt)
                a = a * jnp.concatenate(f, axis=1)
                if first:
                    acc[:, r0:r1] = a + (1.0 - g) * _cols(xT_s, r0, r1).astype(F32)
                else:
                    a = acc[:, r0:r1] + a
                    acc[:, r0:r1] = a
                    out_s[:, r0:r1] = a.astype(BF)

                    @pl.when(h == H - 1)
                    def _():
                        cp_out(i).start()
            elif kind == "TOPK":
                r = r_s[...]
                lane = lax.broadcasted_iota(I32, (1, S), 1)
                m1 = jnp.max(r, axis=1, keepdims=True)
                i1 = jnp.min(jnp.where(r == m1, lane, S - 1))
                r2 = jnp.where(lane == i1, -jnp.inf, r)
                m2 = jnp.max(r2, axis=1, keepdims=True)
                i2 = jnp.min(jnp.where((r2 == m2) & (lane != i1), lane, S - 1))

                def token(idx):
                    w = x_s[pl.ds(idx // 2, 1), :]
                    sh = (16 * (1 - idx % 2)).astype(U32)
                    return pltpu.bitcast((w << sh) & jnp.uint32(HI16), F32)
                xsel = jnp.where(r16 == 0, token(i1),
                                 jnp.where(r16 == 1, token(i2), 0.0))
                xsel_s[...] = pltpu.bitcast(xsel.astype(BF), U32)
                r8 = lax.broadcasted_iota(I32, (8, TQ), 0)
                sig_s[...] = jnp.where(r8 == 0, _sigmoid(m1), _sigmoid(m2))
                idx_s[0] = i1
                idx_s[1] = i2
                if VF:
                    lane = lax.broadcasted_iota(I32, (1, TQ), 1)
                    for t, idx in enumerate((i1, i2)):
                        blk = pl.ds(pl.multiple_of(idx // TQ * TQ, TQ), TQ)
                        xb = pltpu.bitcast(xT_s[:, blk], BF).astype(F32)
                        xc = jnp.sum(jnp.where(lane == idx % TQ, xb, 0.0),
                                     axis=1, keepdims=True)
                        xcol_s[t] = jnp.broadcast_to(xc, (M, TQ))
                    ypart_s[...] = jnp.zeros_like(ypart_s)
            elif kind == "FV":
                chunk = jnp.minimum(h - 1, NF - 1)
                c = pl.ds(pl.multiple_of(chunk * TQ, TQ), TQ)
                wg, wu, wd = (pltpu.bitcast(w[:, c], BF).astype(F32)
                              for w in (wg_s, wu_s, wd_s))
                for t in range(2):
                    xc = xcol_s[t]
                    g = jnp.sum(xc * wg, axis=0, keepdims=True)
                    u = jnp.sum(xc * wu, axis=0, keepdims=True)
                    ypart_s[t] += wd * (g * _sigmoid(g) * u)
            elif kind in ("FG", "FU"):
                chunk = jnp.minimum(h - 1, NF - 1)
                b["c"] = pl.ds(pl.multiple_of(chunk * TQ, TQ), TQ)
                w_s = wg_s if kind == "FG" else wu_s
                b[kind] = _dot(pltpu.bitcast(xsel_s[...], BF),
                               pltpu.bitcast(w_s[:, b["c"]], BF), NN)
            elif kind == "FD":
                g, u = b["FG"], b["FU"]
                hid = (g * _sigmoid(g) * u).astype(BF)
                b["y"] = _dot(hid, pltpu.bitcast(wd_s[:, b["c"]], BF), NT)
            elif kind == "UPD":
                pad = jnp.zeros((TQ, 512 - M), F32)
                lane = lax.broadcasted_iota(I32, (1, TQ), 1)
                for t in range(2):
                    idx = idx_s[t]
                    yb = jnp.broadcast_to(
                        b["y"][t:t + 1, :] * sig_s[t:t + 1, 0:1], (TQ, M))
                    ycol = jnp.concatenate([yb, pad], axis=1).T[:M, :]
                    blk = pl.ds(pl.multiple_of(idx // TQ * TQ, TQ), TQ)
                    hit = lane == jnp.where(h <= NF, idx % TQ, -1)
                    old = acc[:, blk]
                    acc[:, blk] = jnp.where(
                        hit, old + (1.0 - g_s[:, blk]) * ycol, old)

    for c in [c_wk, cp_ckv(0), c_wv] + [cp_ckv(i) for i in range(1, NPB)]:
        c.start()
    for c in head0 + head1 + bulk:
        c.start()

    def proj0(t, carry):
        which, blk = t % 2, t // 2

        @pl.when(t == 0)
        def _():
            c_wk.wait()

        @pl.when(t == 1)
        def _():
            c_wv.wait()

        @pl.when(which == 0)
        def _():
            cp_ckv(blk).wait()

        r = pl.ds(pl.multiple_of(blk * (PB // 2), PB // 2), PB // 2)
        w = pltpu.bitcast(wkv32[which, 0] << 16, F32).astype(BF)
        y = _dot(pltpu.bitcast(ckv_s[r, :], BF), w, NN)
        kv_s[which, r, :] = pltpu.bitcast(y.astype(BF), U32)
        return carry

    lax.fori_loop(0, 2 * NPB, proj0, 0)
    for c in head0:
        c.wait()
    head(0, _first_order(), first=True)
    for c in head1:
        c.wait()

    def step(h, carry):
        @pl.when(h == 2)
        def _():
            for c in bulk:
                c.wait()

        if VF:
            @pl.when(h == H - 1)
            def _():
                lane = lax.broadcasted_iota(I32, (1, TQ), 1)
                for t in range(2):
                    idx = idx_s[t]
                    y = jnp.sum(ypart_s[t], axis=1, keepdims=True) * sig_s[t:t + 1, :]
                    blk = pl.ds(pl.multiple_of(idx // TQ * TQ, TQ), TQ)
                    old = acc[:, blk]
                    acc[:, blk] = jnp.where(
                        lane == idx % TQ, old + (1.0 - g_s[:, blk]) * y, old)

        head(h, _loop_order())
        return carry

    lax.fori_loop(1, H, step, 0)
    for i in range(NPB):
        cp_out(i).wait()


@jax.jit
def pallas_gated_mix__compressed_kv_cla__moe_arch_mod__prompt_kernel(
    A_x: jax.Array,
    A_c_kv: jax.Array,
    A_w_q: jax.Array,
    A_w_uk: jax.Array,
    A_w_uv: jax.Array,
    A_w_o: jax.Array,
    B_x: jax.Array,
    B_w_r: jax.Array,
    B_w_gate: jax.Array,
    B_w_up: jax.Array,
    B_w_down: jax.Array,
    gate_w: jax.Array,
):
    del B_x
    xT = A_x.reshape(S, M).T
    ckv = A_c_kv.reshape(S, C)
    woT = jnp.transpose(A_w_o, (0, 2, 1))
    wdT = B_w_down.T

    V = pltpu.VMEM
    scratch = [
        V((M // 2, S), U32),
        V((S // 2, M), U32),
        V((S // 2, C), U32),
        V((H // 2, M, D), U32),
        V((2, H // 2, C, D), U32),
        V((H, M // 2, D), U32),
        V((S // 2, D), U32),
        V((2, S // 2, D), U32),
        V((S // 2, D), U32),
        V((M, S), F32),
        V((1, S), F32),
        V((1, S), F32),
        V((M,), BF),
        V((M,), BF),
        V((M // 2, F), U32),
        V((M // 2, F), U32),
        V((M // 2, F), U32),
        V((8, M), U32),
        V((8, TQ), F32),
        pltpu.SMEM((2,), I32),
        V((2, M, TQ), F32),
        V((2, M, TQ), F32),
        V((M, S), BF),
        pltpu.SemaphoreType.DMA((NSEM,)),
    ]
    outT = pl.pallas_call(
        _kernel,
        in_specs=[pl.BlockSpec(memory_space=pl.ANY)] * 11,
        out_specs=pl.BlockSpec(memory_space=pl.ANY),
        out_shape=jax.ShapeDtypeStruct((M, S), BF),
        scratch_shapes=scratch,
        compiler_params=pltpu.CompilerParams(
            vmem_limit_bytes=100 * 1024 * 1024),
    )(xT, ckv, A_w_q, A_w_uk, A_w_uv, woT, B_w_r, B_w_gate, B_w_up, wdT, gate_w)
    return outT.T.reshape(1, S, M)
```

```python
import math
import re
_CFG = {}


def E(k, d=''):
    return _CFG.get(k, d)
def _parse(txt):
    return [(re.match(r'[A-Z]+4?(?=\d)', t).group() if t.startswith('G4') else re.match(r'[A-Z]+', t).group(), int(re.search(r'(\d+)$', t[2:] if t.startswith('G4') else t).group())) for t in txt.split(',')]

import jax
import jax.numpy as jnp
from jax import lax
import jax.experimental.pallas as pl
import jax.experimental.pallas.tpu as pltpu

S, M, C, H, D, F = 2048, 448, 1024, 16, 256, 1792
TQ = 128
NQ = S // TQ
PB = 512
NPB = S // PB
NF = F // TQ

BF, F32, U32, I32 = jnp.bfloat16, jnp.float32, jnp.uint32, jnp.int32
NN = (((1,), (0,)), ((), ()))
NT = (((1,), (1,)), ((), ()))
LOG2E = math.log2(math.e)
QSCALE = (D ** -0.5) * LOG2E
NEG = -1e9 * LOG2E
HI16 = 0xFFFF0000

S_WK, S_WV, S_HEAD0, S_HEAD1, S_BULK, S_OUT, S_CKV = range(7)
NSEM = S_CKV + NPB


HYB = int(E('hyb', 14))
VF = E('ffn', 'vpu') == 'vpu'
ST = int(E('st', 1))
HB, HC = PB // 2, C // 2


def _dot(a, b, dn):
    return lax.dot_general(a, b, dn, preferred_element_type=F32)


def _recip(l):
    r = pl.reciprocal(l, approx=True)
    return r * (2.0 - l * r)


def _sigmoid(z):
    return 1.0 / (1.0 + jnp.exp(-z))


def _rows(ref, r0, r1):
    return pltpu.bitcast(ref[r0 // 2:r1 // 2, :], BF)


def _cols(ref, c0, c1):
    return pltpu.bitcast(ref[:, c0:c1], BF)


def _put_rows(ref, r0, r1, v):
    ref[r0 // 2:r1 // 2, :] = pltpu.bitcast(v, U32)


def _lhs_sums(a11, a12, a21, a22):
    return a11 + a22, a21 + a22, a11 + a12, a21 - a11, a12 - a22


def _rhs_terms(f, k, n):
    b11, b12, b21, b22 = f[:k, :n], f[:k, n:], f[k:, :n], f[k:, n:]
    return [t.astype(BF) for t in (b11 + b22, b11, b12 - b22, b21 - b11, b22,
                                   b11 + b12, b21 + b22)]


def _strassen(sums, a11, a22, rhs):
    lhs = [sums[0], sums[1], a11, a22, sums[2], sums[3], sums[4]]
    m = {n: _dot(lhs[n], rhs[n], NN) for n in (3, 1, 0, 4, 6, 2, 5)}
    top = jnp.concatenate([m[0] + m[3] - m[4] + m[6], m[2] + m[4]], axis=1)
    bot = jnp.concatenate([m[1] + m[3], m[0] - m[1] + m[2] + m[5]], axis=1)
    return top, bot


def _steady_order(j0):
    t = []
    for j in range(j0, NQ + 2):
        if 1 <= j <= NQ:
            t.append(("PV", j - 1))
        if j + 1 < NQ:
            if (j + 1) % 4 == 0:
                t += [("KV", (j + 1) // 4), ("Q", (j + 1) // 4)]
            t.append(("QK", j + 1))
        if j >= 2 and (j - 1) % 4 == 0:
            t.append(("O", (j - 2) // 4))
    return t


def _dedup(t):
    out, seen = [], set()
    for e in t:
        if e not in seen:
            seen.add(e)
            out.append(e)
    return out


def _mid_order():
    t = [("Q", 0), ("KV", 0), ("QK", 0), ("QK", 1), ("QK", 2), ("QK", 3),
         ("KV", 1), ("PV", 0), ("PV", 1), ("PV", 2), ("Q", 1)]
    return _dedup(t + _steady_order(3))


def _first_order():
    if E('first'):
        return _parse(E('first'))
    t = [("T", 0), ("T", 1), ("T", 2), ("T", 3), ("G4", 0), ("G4", 1), ("Q", 0),
         ("QK", 0), ("QK", 1), ("QK", 2), ("QK", 3), ("Q", 1),
         ("PV", 0), ("PV", 1), ("PV", 2)]
    out = []
    g = 8
    for e in _dedup(t + _steady_order(3)):
        if e[0] == "KV":
            continue
        out.append(e)
        if ("Q", 1) in out and g < NQ and e[0] in ("Q", "QK"):
            out.append(("G", g))
            g += 1
        if e == ("O", 1):
            out.append(("TOPK", 0))
        if ST and E('asum', '') == 'first' and e[0] == E('ask', 'QK') and int(E('as0', 4)) <= e[1] < int(E('as0', 4)) + 8:
            out.append(("AS", e[1] - int(E('as0', 4))))
    return out


def _loop_order():
    if E('loop'):
        return _parse(E('loop'))
    pos = dict(kv.split(':') for kv in E('fpos', 'FV:KV0' if VF else 'FG:KV1;FU:KV2;FD:KV3;UPD:QK15').split(';'))
    base = _mid_order()
    if E('head'):
        hd = _parse(E('head')); base = _dedup(hd + base)
    if E('tail'):
        tl = _parse(E('tail')); base = [e for e in base if e not in tl] + tl
    out = []
    for e in base:
        out.append(e)
        for k in ('FG', 'FU', 'FD', 'UPD', 'FV'):
            if pos.get(k) == '%s%d' % e:
                out.append((k, 0))
    return out
    out = []
    for e in _mid_order():
        if e == ("O", NPB - 1):
            out.append(("UPD", 0))
        out.append(e)
        if e == ("KV", 0):
            out.append(("FG", 0))
        if e == ("KV", 1):
            out.append(("FU", 0))
        if e == ("KV", 2):
            out.append(("FD", 0))
    return out


def _kernel(xT_hbm, ckv_hbm, wq_hbm, wk_hbm, wv_hbm, wo_hbm, wr_hbm, wg_hbm,
            wu_hbm, wd_hbm, gw_hbm, out_hbm,
            xT_s, x_s, ckv_s, wq32, wkv32, wo_s, q_s, kv_s, ctx_s, acc,
            r_s, g_s, wr_s, gw_s, wg_s, wu_s, wd_s, xsel_s, sig_s, idx_s, xcol_s, ypart_s, asum_s,
            out_s, sem):
    wk32, wv32 = wkv32.at[0], wkv32.at[1]
    k_s, v_s = kv_s.at[0], kv_s.at[1]
    (xT_u, ckv_u, wq_u, wk_u, wv_u, wo_u, wg_u, wu_u, wd_u) = (
        r.bitcast(U32) for r in (xT_hbm, ckv_hbm, wq_hbm, wk_hbm, wv_hbm,
                                 wo_hbm, wg_hbm, wu_hbm, wd_hbm))

    def cp(src, dst, s):
        return pltpu.make_async_copy(src, dst, sem.at[s])

    def cp_pair(w_u, w_s, p, s):
        return cp(w_u.at[:, p, :], w_s.at[p], s)

    def cp_ckv(i):
        r = pl.ds(pl.multiple_of(PB // 2 * i, PB // 2), PB // 2)
        return cp(ckv_u.at[r, :], ckv_s.at[r, :], S_CKV + i)

    def cp_out(i):
        r = pl.ds(PB * i, PB)
        return cp(out_s.at[:, r], out_hbm.at[:, r], S_OUT)

    c_wk, c_wv = cp_pair(wk_u, wk32, 0, S_WK), cp_pair(wv_u, wv32, 0, S_WV)
    head0 = [cp(xT_u, xT_s, S_HEAD0), cp_pair(wq_u, wq32, 0, S_HEAD0),
             cp(wr_hbm, wr_s, S_HEAD0), cp(gw_hbm, gw_s, S_HEAD0),
             cp(wo_u.at[0], wo_s.at[0], S_HEAD0)]
    head1 = [cp(wo_u.at[1], wo_s.at[1], S_HEAD1), cp(wg_u, wg_s, S_HEAD1),
             cp(wu_u, wu_s, S_HEAD1), cp(wd_u, wd_s, S_HEAD1)]
    rest = pl.ds(2, H - 2)
    bulk = [cp(wo_u.at[rest], wo_s.at[rest], S_BULK)]
    for p in range(1, H // 2):
        bulk += [cp_pair(wk_u, wk32, p, S_BULK), cp_pair(wv_u, wv32, p, S_BULK),
                 cp_pair(wq_u, wq32, p, S_BULK)]

    row = lax.broadcasted_iota(I32, (TQ, TQ), 0)
    col = lax.broadcasted_iota(I32, (TQ, TQ), 1)
    tri = col <= row
    r16 = lax.broadcasted_iota(I32, (16, M), 0)

    def head(h, order, first=False):
        pair = h // 2
        if isinstance(h, int):
            shift = jnp.uint32(16 * (1 - h % 2))
        else:
            shift = (16 * (1 - h % 2)).astype(U32)

        cache = {}

        def weight(name, ref):
            if name not in cache:
                hi = (ref[pair] << shift) & jnp.uint32(HI16)
                cache[name] = pltpu.bitcast(hi, F32).astype(BF)
            return cache[name]

        def route(c0, c1):
            if "rg" not in cache:
                wr = wr_s[...].astype(F32).reshape(1, M)
                gw = gw_s[...].astype(F32).reshape(1, M)
                cache["rg"] = jnp.where(
                    r16 == 0, wr, jnp.where(r16 == 1, gw, 0.0)).astype(BF)
            rg = _dot(cache["rg"], _cols(xT_s, c0, c1), NN)
            r_s[:, c0:c1] = rg[0:1, :].astype(BF).astype(F32)
            g_s[:, c0:c1] = _sigmoid(rg[1:2, :])

        sv, rinv, b = {}, {}, {}
        for kind, i in order:
            r0, r1 = PB * i, PB * (i + 1)
            t0, t1 = TQ * i, TQ * (i + 1)
            if kind == "T":
                _put_rows(x_s, r0, r1, _cols(xT_s, r0, r1).T)
            elif kind == "AS":
                blk, part = i // 2, i % 2
                n0 = HB // 2
                top0 = PB * blk + n0 * part
                at = _rows(ckv_s, top0, top0 + n0).astype(F32)
                ab = _rows(ckv_s, top0 + HB, top0 + HB + n0).astype(F32)
                a11, a12, a21, a22 = at[:, :HC], at[:, HC:], ab[:, :HC], ab[:, HC:]
                d0 = (HB * blk + n0 * part) // 2
                for n, v in enumerate((a11 + a22, a21 + a22, a11 + a12,
                                       a21 - a11, a12 - a22)):
                    asum_s[n, d0:d0 + n0 // 2, :] = pltpu.bitcast(v.astype(BF), U32)
            elif kind == "G4":
                route(r0, r1)
            elif kind == "G":
                route(t0, t1)
            elif kind == "KV" and ST:
                w0, w1 = HB * i // 2, HB * (i + 1) // 2
                a = [pltpu.bitcast(asum_s[n, w0:w1, :], BF) for n in range(5)]
                a11 = pltpu.bitcast(ckv_s[r0 // 2:(r0 + HB) // 2, :HC], BF)
                a22 = pltpu.bitcast(ckv_s[(r0 + HB) // 2:r1 // 2, HC:], BF)
                for name, ref, dst in (("k", wk32, k_s), ("v", wv32, v_s)):
                    if name not in cache:
                        cache[name] = _rhs_terms(pltpu.bitcast(
                            (ref[pair] << shift) & jnp.uint32(HI16), F32), HC, TQ)
                    top, bot = _strassen(a, a11, a22, cache[name])
                    _put_rows(dst, r0, r0 + HB, top.astype(BF))
                    _put_rows(dst, r0 + HB, r1, bot.astype(BF))
            elif kind == "KV":
                wkv = jnp.concatenate([weight("k", wk32), weight("v", wv32)], axis=1)
                kv = _dot(_rows(ckv_s, r0, r1), wkv, NN)
                _put_rows(k_s, r0, r1, kv[:, :D].astype(BF))
                _put_rows(v_s, r0, r1, kv[:, D:].astype(BF))
            elif kind == "Q":
                q = _dot(_rows(x_s, r0, r1), weight("q", wq32), NN) * QSCALE
                _put_rows(q_s, r0, r1, q.astype(BF))
            elif kind == "QK":
                s = _dot(_rows(q_s, t0, t1), _rows(k_s, 0, t1), NT)
                sd = jnp.where(tri, s[:, t0:], NEG)
                s = sd if i == 0 else jnp.concatenate([s[:, :t0], sd], axis=1)
                sv[i] = (s, jnp.max(s, axis=1, keepdims=True))
            elif kind == "PV":
                s, m = sv.pop(i)
                p = jnp.exp2(s - m).astype(BF)
                o = _dot(p, _rows(v_s, 0, t1), NN)
                pf = p.astype(F32)
                if i < HYB:
                    o = o * _recip(jnp.sum(pf, axis=1, keepdims=True))
                    rinv[i] = None
                _put_rows(ctx_s, t0, t1, o.astype(BF))
                if i >= HYB:
                    la = pf[:, 0:TQ]
                    for t in range(1, i + 1):
                        la = la + pf[:, TQ * t:TQ * (t + 1)]
                    hi = la.astype(BF)
                    lo = (la - hi.astype(F32)).astype(BF)
                    l = _dot(jnp.ones((16, 2 * TQ), BF),
                             jnp.concatenate([hi, lo], axis=1), NT)[0:1, :]
                    rinv[i] = _recip(l)
            elif kind == "O":
                a = _dot(pltpu.bitcast(wo_s[h], BF), _rows(ctx_s, r0, r1), NT)
                g = g_s[:, r0:r1]
                f = []
                for t in range(4):
                    gt, rt = g[:, TQ * t:TQ * (t + 1)], rinv.pop(4 * i + t)
                    f.append(gt if rt is None else gt * rt)
                a = a * jnp.concatenate(f, axis=1)
                if first:
                    acc[:, r0:r1] = a + (1.0 - g) * _cols(xT_s, r0, r1).astype(F32)
                else:
                    a = acc[:, r0:r1] + a
                    acc[:, r0:r1] = a
                    out_s[:, r0:r1] = a.astype(BF)

                    @pl.when(h == H - 1)
                    def _():
                        cp_out(i).start()
            elif kind == "TOPK":
                r = r_s[...]
                lane = lax.broadcasted_iota(I32, (1, S), 1)
                m1 = jnp.max(r, axis=1, keepdims=True)
                i1 = jnp.min(jnp.where(r == m1, lane, S - 1))
                r2 = jnp.where(lane == i1, -jnp.inf, r)
                m2 = jnp.max(r2, axis=1, keepdims=True)
                i2 = jnp.min(jnp.where((r2 == m2) & (lane != i1), lane, S - 1))

                def token(idx):
                    w = x_s[pl.ds(idx // 2, 1), :]
                    sh = (16 * (1 - idx % 2)).astype(U32)
                    return pltpu.bitcast((w << sh) & jnp.uint32(HI16), F32)
                xsel = jnp.where(r16 == 0, token(i1),
                                 jnp.where(r16 == 1, token(i2), 0.0))
                xsel_s[...] = pltpu.bitcast(xsel.astype(BF), U32)
                r8 = lax.broadcasted_iota(I32, (8, TQ), 0)
                sig_s[...] = jnp.where(r8 == 0, _sigmoid(m1), _sigmoid(m2))
                idx_s[0] = i1
                idx_s[1] = i2
                if VF:
                    lane = lax.broadcasted_iota(I32, (1, TQ), 1)
                    for t, idx in enumerate((i1, i2)):
                        blk = pl.ds(pl.multiple_of(idx // TQ * TQ, TQ), TQ)
                        xb = pltpu.bitcast(xT_s[:, blk], BF).astype(F32)
                        xc = jnp.sum(jnp.where(lane == idx % TQ, xb, 0.0),
                                     axis=1, keepdims=True)
                        xcol_s[t] = jnp.broadcast_to(xc, (M, TQ))
                    ypart_s[...] = jnp.zeros_like(ypart_s)
            elif kind == "FV":
                chunk = jnp.minimum(h - 1, NF - 1)
                c = pl.ds(pl.multiple_of(chunk * TQ, TQ), TQ)
                wg, wu, wd = (pltpu.bitcast(w[:, c], BF).astype(F32)
                              for w in (wg_s, wu_s, wd_s))
                for t in range(2):
                    xc = xcol_s[t]
                    g = jnp.sum(xc * wg, axis=0, keepdims=True)
                    u = jnp.sum(xc * wu, axis=0, keepdims=True)
                    ypart_s[t] += wd * (g * _sigmoid(g) * u)
            elif kind in ("FG", "FU"):
                chunk = jnp.minimum(h - 1, NF - 1)
                b["c"] = pl.ds(pl.multiple_of(chunk * TQ, TQ), TQ)
                w_s = wg_s if kind == "FG" else wu_s
                b[kind] = _dot(pltpu.bitcast(xsel_s[...], BF),
                               pltpu.bitcast(w_s[:, b["c"]], BF), NN)
            elif kind == "FD":
                g, u = b["FG"], b["FU"]
                hid = (g * _sigmoid(g) * u).astype(BF)
                b["y"] = _dot(hid, pltpu.bitcast(wd_s[:, b["c"]], BF), NT)
            elif kind == "UPD":
                pad = jnp.zeros((TQ, 512 - M), F32)
                lane = lax.broadcasted_iota(I32, (1, TQ), 1)
                for t in range(2):
                    idx = idx_s[t]
                    yb = jnp.broadcast_to(
                        b["y"][t:t + 1, :] * sig_s[t:t + 1, 0:1], (TQ, M))
                    ycol = jnp.concatenate([yb, pad], axis=1).T[:M, :]
                    blk = pl.ds(pl.multiple_of(idx // TQ * TQ, TQ), TQ)
                    hit = lane == jnp.where(h <= NF, idx % TQ, -1)
                    old = acc[:, blk]
                    acc[:, blk] = jnp.where(
                        hit, old + (1.0 - g_s[:, blk]) * ycol, old)

    for c in [cp_ckv(0), c_wk, c_wv] + [cp_ckv(i) for i in range(1, NPB)]:
        c.start()
    for c in head0 + head1 + bulk:
        c.start()

    def proj0(t, carry):
        which, blk = t % 2, t // 2
        base = pl.multiple_of(blk * (PB // 2), PB // 2)
        half = pl.multiple_of(blk * (HB // 2), HB // 2)

        @pl.when(which == 0)
        def _():
            cp_ckv(blk).wait()
            for j in range(0, HB // 2, 8):
                at = pltpu.bitcast(ckv_s[pl.ds(base + j, 8), :], BF).astype(F32)
                ab = pltpu.bitcast(
                    ckv_s[pl.ds(base + HB // 2 + j, 8), :], BF).astype(F32)
                for n, v in enumerate(_lhs_sums(at[:, :HC], at[:, HC:],
                                                ab[:, :HC], ab[:, HC:])):
                    asum_s[n, pl.ds(half + j, 8), :] = pltpu.bitcast(v.astype(BF), U32)

        @pl.when(t == 0)
        def _():
            c_wk.wait()

        @pl.when(t == 1)
        def _():
            c_wv.wait()

        top, bot = pl.ds(base, HB // 2), pl.ds(base + HB // 2, HB // 2)
        a = [pltpu.bitcast(asum_s[n, pl.ds(half, HB // 2), :], BF) for n in range(5)]
        a11 = pltpu.bitcast(ckv_s[top, :HC], BF)
        a22 = pltpu.bitcast(ckv_s[bot, HC:], BF)
        rhs = _rhs_terms(pltpu.bitcast(wkv32[which, 0] << 16, F32), HC, TQ)
        ct, cb = _strassen(a, a11, a22, rhs)
        kv_s[which, top, :] = pltpu.bitcast(ct.astype(BF), U32)
        kv_s[which, bot, :] = pltpu.bitcast(cb.astype(BF), U32)
        return carry

    lax.fori_loop(0, 2 * NPB, proj0, 0)
    for c in head0:
        c.wait()
    head(0, _first_order(), first=True)
    for c in head1:
        c.wait()

    def step(h, carry):
        @pl.when(h == 2)
        def _():
            for c in bulk:
                c.wait()

        if VF:
            @pl.when(h == H - 1)
            def _():
                lane = lax.broadcasted_iota(I32, (1, TQ), 1)
                for t in range(2):
                    idx = idx_s[t]
                    y = jnp.sum(ypart_s[t], axis=1, keepdims=True) * sig_s[t:t + 1, :]
                    blk = pl.ds(pl.multiple_of(idx // TQ * TQ, TQ), TQ)
                    old = acc[:, blk]
                    acc[:, blk] = jnp.where(
                        lane == idx % TQ, old + (1.0 - g_s[:, blk]) * y, old)

        head(h, _loop_order())
        return carry

    lax.fori_loop(1, H, step, 0)
    for i in range(NPB):
        cp_out(i).wait()


@jax.jit
def pallas_gated_mix__compressed_kv_cla__moe_arch_mod__prompt_kernel(
    A_x: jax.Array,
    A_c_kv: jax.Array,
    A_w_q: jax.Array,
    A_w_uk: jax.Array,
    A_w_uv: jax.Array,
    A_w_o: jax.Array,
    B_x: jax.Array,
    B_w_r: jax.Array,
    B_w_gate: jax.Array,
    B_w_up: jax.Array,
    B_w_down: jax.Array,
    gate_w: jax.Array,
):
    del B_x
    xT = A_x.reshape(S, M).T
    ckv = A_c_kv.reshape(S, C)
    woT = jnp.transpose(A_w_o, (0, 2, 1))
    wdT = B_w_down.T

    V = pltpu.VMEM
    scratch = [
        V((M // 2, S), U32),
        V((S // 2, M), U32),
        V((S // 2, C), U32),
        V((H // 2, M, D), U32),
        V((2, H // 2, C, D), U32),
        V((H, M // 2, D), U32),
        V((S // 2, D), U32),
        V((2, S // 2, D), U32),
        V((S // 2, D), U32),
        V((M, S), F32),
        V((1, S), F32),
        V((1, S), F32),
        V((M,), BF),
        V((M,), BF),
        V((M // 2, F), U32),
        V((M // 2, F), U32),
        V((M // 2, F), U32),
        V((8, M), U32),
        V((8, TQ), F32),
        pltpu.SMEM((2,), I32),
        V((2, M, TQ), F32),
        V((2, M, TQ), F32),
        V((5, S // 4, C // 2), U32),
        V((M, S), BF),
        pltpu.SemaphoreType.DMA((NSEM,)),
    ]
    outT = pl.pallas_call(
        _kernel,
        in_specs=[pl.BlockSpec(memory_space=pl.ANY)] * 11,
        out_specs=pl.BlockSpec(memory_space=pl.ANY),
        out_shape=jax.ShapeDtypeStruct((M, S), BF),
        scratch_shapes=scratch,
        compiler_params=pltpu.CompilerParams(
            vmem_limit_bytes=100 * 1024 * 1024),
    )(xT, ckv, A_w_q, A_w_uk, A_w_uv, woT, B_w_r, B_w_gate, B_w_up, wdT, gate_w)
    return outT.T.reshape(1, S, M)
```

```python
import math
import re
_CFG = {'loop': 'Q0,K0,V0,FV0,SA0,SB0,SD1,K1,SS1,V1.4,V1.1,V1,PB0,PA0,Q1,SD2,SS2,PA1,PB1,SS3,SD3,PD2,K2,V2.1,V2.4,PS2,O0,V2,Q2.3,Q2,SS4.1,SS4,PD3,PS3,SD4,SS5,K3,SD5,PS4,PD4,V3.4,Q3.5,O1,Q3,V3,SS6,PS5.5,SD6,PS5,PA6,PD5,SS7,SD7,PB6,PS7.2,PS7.4,O2,PS7,PD7,O3', 'oP': '2316450', 'oO': '1603425', 'oV': '4153620', 'oK': '1403625', 'oS': '0134625', 'qkc': '1', 'oQ': '3604125', 'hyb': '14'}


def E(k, d=''):
    return _CFG.get(k, d)

import jax
import jax.numpy as jnp
from jax import lax
import jax.experimental.pallas as pl
import jax.experimental.pallas.tpu as pltpu

S, M, C, H, D, F = 2048, 448, 1024, 16, 256, 1792
TQ = 128
NQ = S // TQ
PR = 2 * TQ
NP = S // PR
PB = 512
NPB = S // PB
NF = F // TQ
HB, HC, HM = PB // 2, C // 2, M // 2
MP = 512

BF, F32, U32, I32 = jnp.bfloat16, jnp.float32, jnp.uint32, jnp.int32
NN = (((1,), (0,)), ((), ()))
NT = (((1,), (1,)), ((), ()))
LOG2E = math.log2(math.e)
QSCALE = (D ** -0.5) * LOG2E
NEG = -1e9 * LOG2E
HI16 = 0xFFFF0000

S_WK, S_WV, S_HEAD0, S_HEAD1, S_BULK, S_OUT, S_CKV = range(7)
NSEM = S_CKV + NPB

HYB = int(E('hyb', 14))
STQ = int(E('stq', 1))
QK0 = int(E('qk0', 99))
PV0 = int(E('pv0', 1))
STO = int(E('sto', 0))
LSRC = int(E('lsrc', 2))
QKC = int(E('qkc', 1))
OC = int(E('oc', 1))
ORD = {k: [int(c) for c in E('o' + k, d)] for k, d in
       (('K', '3104625'), ('V', '3104625'), ('Q', '3104625'), ('S', '3104625'),
        ('P', '2304156'), ('O', '0346125'))}
ONLY = E('only')


def _parse(txt):
    out = []
    for t in txt.split(','):
        m = re.match(r'([A-Z]+)(\d+)(?:\.(\d))?$', t)
        out.append((m.group(1), int(m.group(2)), int(m.group(3) or 0)))
    return out


def _dot(a, b, dn):
    return lax.dot_general(a, b, dn, preferred_element_type=F32)


def _cat(xs, axis):
    return xs[0] if len(xs) == 1 else jnp.concatenate(xs, axis=axis)


def _recip(l):
    r = pl.reciprocal(l, approx=True)
    return r * (2.0 - l * r)


def _sigmoid(z):
    return 1.0 / (1.0 + jnp.exp(-z))


def _bf(w):
    return pltpu.bitcast(w, BF)


def _u32(v):
    return pltpu.bitcast(v.astype(BF), U32)


def _rows(ref, r0, r1):
    return _bf(ref[r0 // 2:r1 // 2, :])


def _put_rows(ref, r0, r1, v):
    ref[r0 // 2:r1 // 2, :] = _u32(v)


def _lhs_terms(a11, a12, a21, a22):
    return [a11 + a22, a21 + a22, a11, a22, a11 + a12, a21 - a11, a12 - a22]


def _rhs_terms(b11, b12, b21, b22):
    return [b11 + b22, b11, b12 - b22, b21 - b11, b22, b11 + b12, b21 + b22]


def _quads(f):
    k, n = f.shape[0] // 2, f.shape[1] // 2
    return f[:k, :n], f[:k, n:], f[k:, :n], f[k:, n:]


def _combine(m):
    return (m[0] + m[3] - m[4] + m[6], m[2] + m[4],
            m[1] + m[3], m[0] - m[1] + m[2] + m[5])


SUMS = (0, 1, 4, 5, 6)


def _att(i, st):
    qk = [("SS", i, 0), ("SD", i, 0)] if st and i >= max(QK0, 1) else [("SA", i, 0), ("SB", i, 0)]
    pv = [("PS", i, 0), ("PD", i, 0)] if st and i >= max(PV0, 1) else [("PA", i, 0), ("PB", i, 0)]
    return qk, pv


def _order(st, proj):
    q = lambda b: [("Q", b, 0)]
    kv = lambda b: [("K", b, 0), ("V", b, 0)] if proj else []
    t = q(0) + kv(0) + _att(0, st)[0] + _att(1, st)[0] + kv(1) + _att(0, st)[1] + q(1)
    for i in range(1, NP + 1):
        if i + 1 < NP:
            if i % 2 == 1 and i > 1:
                t += kv((i + 1) // 2) + q((i + 1) // 2)
            t += _att(i + 1, st)[0]
        if i < NP:
            t += _att(i, st)[1]
        if i % 2 == 0:
            t.append(("O", i // 2 - 1, 0))
    return t


def _first_order():
    if E('first'):
        return _parse(E('first'))
    out = [("T", b, 0) for b in range(NPB)] + [("GB", 0, 0), ("GB", 1, 0)]
    g = 8
    for e in _order(False, False):
        out.append(e)
        if ("Q", 1, 0) in out and g < NQ and e[0] in ("Q", "SA", "SB"):
            out.append(("G", g, 0))
            g += 1
        if e == ("O", 1, 0):
            out.append(("TOPK", 0, 0))
    if STQ:
        out += [("XS", b, 0) for b in range(NPB)]
    return out


def _loop_order():
    if E('loop'):
        return _parse(E('loop'))
    out = []
    for e in _order(True, True):
        out.append(e)
        if e == ("V", 0, 0):
            out.append(("FV", 0, 0))
    return out


def _kernel(xT_hbm, ckv_hbm, wq_hbm, wk_hbm, wv_hbm, wo_hbm, wr_hbm, wg_hbm,
            wu_hbm, wd_hbm, gw_hbm, out_hbm,
            xT_s, x_s, ckv_s, wq32, wkv32, wo_s, q_s, kv_s, ctx_s, acc,
            r_s, g_s, wr_s, gw_s, wg_s, wu_s, wd_s, sig_s, idx_s, xcol_s, ypart_s,
            asum_s, xsum_s, qt_s, kt_s, vt_s, ct_s, out_s, sem):
    wk32, wv32 = wkv32.at[0], wkv32.at[1]
    k_s, v_s = kv_s.at[0], kv_s.at[1]
    (xT_u, ckv_u, wq_u, wk_u, wv_u, wo_u, wg_u, wu_u, wd_u) = (
        r.bitcast(U32) for r in (xT_hbm, ckv_hbm, wq_hbm, wk_hbm, wv_hbm,
                                 wo_hbm, wg_hbm, wu_hbm, wd_hbm))

    def cp(src, dst, s):
        return pltpu.make_async_copy(src, dst, sem.at[s])

    def cp_pair(w_u, w_s, p, s):
        return cp(w_u.at[:, p, :], w_s.at[p], s)

    def cp_ckv(i):
        r = pl.ds(pl.multiple_of(PB // 2 * i, PB // 2), PB // 2)
        return cp(ckv_u.at[r, :], ckv_s.at[r, :], S_CKV + i)

    def cp_out(i):
        r = pl.ds(PB * i, PB)
        return cp(out_s.at[:, r], out_hbm.at[:, r], S_OUT)

    c_wk, c_wv = cp_pair(wk_u, wk32, 0, S_WK), cp_pair(wv_u, wv32, 0, S_WV)
    head0 = [cp(xT_u, xT_s, S_HEAD0), cp_pair(wq_u, wq32, 0, S_HEAD0),
             cp(wr_hbm, wr_s, S_HEAD0), cp(gw_hbm, gw_s, S_HEAD0),
             cp(wo_u.at[0], wo_s.at[0], S_HEAD0)]
    head1 = [cp(wo_u.at[1], wo_s.at[1], S_HEAD1), cp(wg_u, wg_s, S_HEAD1),
             cp(wu_u, wu_s, S_HEAD1), cp(wd_u, wd_s, S_HEAD1)]
    rest = pl.ds(2, H - 2)
    bulk = [cp(wo_u.at[rest], wo_s.at[rest], S_BULK)]
    for p in range(1, H // 2):
        bulk += [cp_pair(wk_u, wk32, p, S_BULK), cp_pair(wv_u, wv32, p, S_BULK),
                 cp_pair(wq_u, wq32, p, S_BULK)]

    row = lax.broadcasted_iota(I32, (TQ, TQ), 0)
    col = lax.broadcasted_iota(I32, (TQ, TQ), 1)
    tri = col <= row

    def term(ref, n, j0, j1):
        return _bf(ref[n, TQ // 2 * j0:TQ // 2 * j1, :])

    def put_terms(ref, j, terms):
        for n, t in enumerate(terms):
            ref[n, TQ // 2 * j:TQ // 2 * (j + 1), :] = _u32(t)

    def head(h, order, first=False):
        pair = h // 2
        if isinstance(h, int):
            shift = jnp.uint32(16 * (1 - h % 2))
        else:
            shift = (16 * (1 - h % 2)).astype(U32)
        kinds = {(k, i) for k, i, _ in order}
        cache, prog = {}, {}

        def weight32(ref):
            return pltpu.bitcast((ref[pair] << shift) & jnp.uint32(HI16), F32)

        def wterms(name):
            if name not in cache:
                if name == "O":
                    f = _bf(wo_s[h]).astype(F32)
                    cache[name] = [t.astype(BF) for t in _lhs_terms(*_quads(f))]
                else:
                    f = weight32({"K": wk32, "V": wv32, "Q": wq32}[name])
                    if name == "Q":
                        f = jnp.concatenate([f, jnp.zeros((MP - M, D), F32)], axis=0)
                    cache[name] = [t.astype(BF) for t in _rhs_terms(*_quads(f))]
            return cache[name]

        def run(key, cnt, product):
            m = prog.setdefault(key, {})
            todo = [n for n in ORD[key[0]] if n not in m]
            for n in (todo[:cnt] if cnt else todo):
                m[n] = product(n)
            return len(m) == 7

        def route(c0, c1):
            if "rg" not in cache:
                r16 = lax.broadcasted_iota(I32, (16, M), 0)
                wr = wr_s[...].astype(F32).reshape(1, M)
                gw = gw_s[...].astype(F32).reshape(1, M)
                cache["rg"] = jnp.where(
                    r16 == 0, wr, jnp.where(r16 == 1, gw, 0.0)).astype(BF)
            rg = _dot(cache["rg"], _bf(xT_s[:, c0:c1]), NN)
            r_s[:, c0:c1] = rg[0:1, :].astype(BF).astype(F32)
            g_s[:, c0:c1] = _sigmoid(rg[1:2, :])

        st, pp, ov, rinv = {}, {}, {}, {}

        def set_scores(q, s0, s):
            for t in range(s.shape[1] // TQ):
                blk = s[:, TQ * t:TQ * (t + 1)]
                st.setdefault(q, {})[s0 + t] = jnp.where(tri, blk, NEG) if s0 + t == q else blk

        def probs(q, perm):
            if q not in pp:
                tiles = st.pop(q)
                s = _cat([tiles[t] for t in perm], 1)
                p = jnp.exp2(s - jnp.max(s, axis=1, keepdims=True))
                pp[q] = (p, p.astype(BF))
            return pp[q]

        def finish(q, o, src):
            if q < HYB:
                rinv[q] = None
                return o * _recip(jnp.sum(src, axis=1, keepdims=True))
            la = src[:, 0:TQ]
            for t in range(1, src.shape[1] // TQ):
                la = la + src[:, TQ * t:TQ * (t + 1)]
            hi = la.astype(BF)
            lo = (la - hi.astype(F32)).astype(BF)
            l = _dot(jnp.ones((16, 2 * TQ), BF),
                     jnp.concatenate([hi, lo], axis=1), NT)[0:1, :]
            rinv[q] = _recip(l)
            return o

        def store_ctx(q, o):
            i = q // 2
            if STO and not first and 2 * i + 1 < HYB:
                ov[q] = o
                if 2 * i in ov and 2 * i + 1 in ov:
                    oa, ob = ov.pop(2 * i), ov.pop(2 * i + 1)
                    put_terms(ct_s, i, _rhs_terms(oa[:, :TQ], ob[:, :TQ],
                                                  oa[:, TQ:], ob[:, TQ:]))
            else:
                _put_rows(ctx_s, TQ * q, TQ * (q + 1), o)

        def pv_done(i):
            if ("PS", i) in prog.get("done", ()) and ("PD", i) in prog.get("done", ()):
                c11, c12, c21, c22 = _combine(prog.pop(("P", i)))
                da, db = prog.pop(("PDv", i))
                lt = prog.pop(("L", i))
                w = TQ * i
                for q, o, ln in ((2 * i, jnp.concatenate([c11, c12], axis=1) + da, 4),
                                 (2 * i + 1, jnp.concatenate([c21, c22], axis=1) + db, 1)):
                    pf, pb = pp.pop(q)
                    if LSRC == 2:
                        src = jnp.concatenate([lt[ln], pb[:, 2 * w:]], axis=1).astype(F32)
                    elif LSRC == 1:
                        src = pb.astype(F32)
                    else:
                        src = pf
                    store_ctx(q, finish(q, o, src))

        for kind, i, cnt in order:
            r0, r1 = PB * i, PB * (i + 1)
            n0 = PR * i
            qa, qb = 2 * i, 2 * i + 1
            eo = [2 * j for j in range(i)] + [2 * j + 1 for j in range(i)]
            if kind == "T":
                _put_rows(x_s, r0, r1, _bf(xT_s[:, r0:r1]).T)
            elif kind == "XS":
                for j in range(0, HB, 16):
                    z = jnp.zeros((16, MP - M), F32)
                    at = jnp.concatenate([_rows(x_s, r0 + j, r0 + j + 16).astype(F32), z], axis=1)
                    ab = jnp.concatenate([_rows(x_s, r0 + HB + j, r0 + HB + j + 16).astype(F32), z], axis=1)
                    tt = _lhs_terms(at[:, :PR], at[:, PR:], ab[:, :PR], ab[:, PR:])
                    for n in range(7):
                        if n != 2:
                            xsum_s[n, (HB * i + j) // 2:(HB * i + j) // 2 + 8, :] = _u32(tt[n])
            elif kind == "GB":
                route(r0, r1)
            elif kind == "G":
                route(TQ * i, TQ * (i + 1))
            elif kind in ("K", "V", "Q"):
                w0, w1 = HB * i // 2, HB * (i + 1) // 2
                if kind == "Q" and (first or not STQ):
                    if "q" not in cache:
                        cache["q"] = weight32(wq32).astype(BF)
                    res = _quads(_dot(_rows(x_s, r0, r1), cache["q"], NN))
                else:
                    def lhs(n):
                        if kind == "Q":
                            if n == 2:
                                return _bf(x_s[r0 // 2:(r0 + HB) // 2, :PR])
                            return _bf(xsum_s[n, w0:w1, :])
                        if n == 2:
                            return _bf(ckv_s[r0 // 2:(r0 + HB) // 2, :HC])
                        if n == 3:
                            return _bf(ckv_s[(r0 + HB) // 2:r1 // 2, HC:])
                        return _bf(asum_s[SUMS.index(n), w0:w1, :])
                    if not run((kind, i), cnt, lambda n: _dot(lhs(n), wterms(kind)[n], NN)):
                        continue
                    res = _combine(prog.pop((kind, i)))
                if kind == "Q":
                    res = [c * QSCALE for c in res]
                dst = {"K": k_s, "V": v_s, "Q": q_s}[kind]
                for j, (c0, c1) in ((2 * i, res[:2]), (2 * i + 1, res[2:])):
                    _put_rows(dst, PR * j, PR * (j + 1), jnp.concatenate([c0, c1], axis=1))
                    if kind == "V" and any(("PS", u) in kinds for u in range(j + 1, NP)):
                        put_terms(vt_s, j, _rhs_terms(c0[:TQ], c1[:TQ], c0[TQ:], c1[TQ:]))
                    if kind == "K" and any(("SS", u) in kinds for u in range(j + 1, NP)):
                        put_terms(kt_s, j, _rhs_terms(c0[:TQ], c0[TQ:], c1[:TQ], c1[TQ:]))
                    if kind == "Q" and ("SS", j) in kinds:
                        put_terms(qt_s, j, _lhs_terms(c0[:TQ], c1[:TQ], c0[TQ:], c1[TQ:]))
            elif kind in ("SA", "SB"):
                q = qa if kind == "SA" else qb
                set_scores(q, 0, _dot(_rows(q_s, TQ * q, TQ * (q + 1)),
                                      _rows(k_s, 0, TQ * (q + 1)), NT))
            elif kind == "SD":
                for q in (qa, qb):
                    set_scores(q, qa, _dot(_rows(q_s, TQ * q, TQ * (q + 1)),
                                           _rows(k_s, n0, TQ * (q + 1)), NT))
            elif kind == "SS":
                qts = [term(qt_s, n, i, i + 1) for n in range(7)]
                done = prog.setdefault(("SSj", i), [0])
                j_end = min(i, done[0] + cnt) if cnt else i
                for j0 in range(done[0], j_end, QKC):
                    j1 = min(j_end, j0 + QKC)
                    cs = _combine({n: _dot(qts[n], term(kt_s, n, j0, j1), NT)
                                   for n in ORD["S"]})
                    for j in range(j0, j1):
                        sl = slice(TQ * (j - j0), TQ * (j - j0 + 1))
                        st.setdefault(qa, {})[2 * j] = cs[0][:, sl]
                        st[qa][2 * j + 1] = cs[1][:, sl]
                        st.setdefault(qb, {})[2 * j] = cs[2][:, sl]
                        st[qb][2 * j + 1] = cs[3][:, sl]
                done[0] = j_end
            elif kind in ("PA", "PB"):
                q = qa if kind == "PA" else qb
                pf, pb = probs(q, range(q + 1))
                pp.pop(q)
                o = _dot(pb, _rows(v_s, 0, TQ * (q + 1)), NN)
                store_ctx(q, finish(q, o, pb.astype(F32) if LSRC else pf))
            elif kind in ("PS", "PD"):
                w = TQ * i
                (paf, pab), (pbf, pbb) = probs(qa, eo + [qa]), probs(qb, eo + [qa, qb])
                if kind == "PD":
                    prog["PDv", i] = (_dot(pab[:, 2 * w:], _rows(v_s, n0, n0 + TQ), NN),
                                      _dot(pbb[:, 2 * w:], _rows(v_s, n0, n0 + PR), NN))
                else:
                    if ("L", i) not in prog:
                        lt = [t.astype(BF) for t in _lhs_terms(
                            paf[:, :w], paf[:, w:2 * w], pbf[:, :w], pbf[:, w:2 * w])]
                        lt[2], lt[3] = pab[:, :w], pbb[:, w:2 * w]
                        prog["L", i] = lt
                    if not run(("P", i), cnt, lambda n: _dot(
                            prog["L", i][n], term(vt_s, n, 0, i), NN)):
                        continue
                prog.setdefault("done", set()).add((kind, i))
                pv_done(i)
            elif kind == "O":
                j0, j1 = 2 * i, 2 * i + 2
                js = min(j1, HYB // 2) if STO and not first else j0
                cols = []
                for j in range(j0, js, OC):
                    je = min(js, j + OC)
                    c11, c12, c21, c22 = _combine(
                        {n: _dot(wterms("O")[n], term(ct_s, n, j, je), NT) for n in ORD["O"]})
                    ca = jnp.concatenate([c11, c21], axis=0)
                    cb = jnp.concatenate([c12, c22], axis=0)
                    for t in range(je - j):
                        cols += [ca[:, TQ * t:TQ * (t + 1)], cb[:, TQ * t:TQ * (t + 1)]]
                if j1 > js:
                    cols.append(_dot(_bf(wo_s[h]), _rows(ctx_s, PR * js, PR * j1), NT))
                g = g_s[:, r0:r1]
                f = []
                for t in range(4):
                    gt, rt = g[:, TQ * t:TQ * (t + 1)], rinv.pop(4 * i + t)
                    f.append(gt if rt is None else gt * rt)
                a = _cat(cols, 1) * jnp.concatenate(f, axis=1)
                if first:
                    acc[:, r0:r1] = a + (1.0 - g) * _bf(xT_s[:, r0:r1]).astype(F32)
                else:
                    a = acc[:, r0:r1] + a
                    acc[:, r0:r1] = a
                    out_s[:, r0:r1] = a.astype(BF)

                    @pl.when(h == H - 1)
                    def _():
                        cp_out(i).start()
            elif kind == "TOPK":
                r = r_s[...]
                lane = lax.broadcasted_iota(I32, (1, S), 1)
                m1 = jnp.max(r, axis=1, keepdims=True)
                i1 = jnp.min(jnp.where(r == m1, lane, S - 1))
                r2 = jnp.where(lane == i1, -jnp.inf, r)
                m2 = jnp.max(r2, axis=1, keepdims=True)
                i2 = jnp.min(jnp.where((r2 == m2) & (lane != i1), lane, S - 1))
                r8 = lax.broadcasted_iota(I32, (8, TQ), 0)
                sig_s[...] = jnp.where(r8 == 0, _sigmoid(m1), _sigmoid(m2))
                lane = lax.broadcasted_iota(I32, (1, TQ), 1)
                for t, idx in enumerate((i1, i2)):
                    idx_s[t] = idx
                    blk = pl.ds(pl.multiple_of(idx // TQ * TQ, TQ), TQ)
                    xb = _bf(xT_s[:, blk]).astype(F32)
                    xc = jnp.sum(jnp.where(lane == idx % TQ, xb, 0.0),
                                 axis=1, keepdims=True)
                    xcol_s[t] = jnp.broadcast_to(xc, (M, TQ))
                ypart_s[...] = jnp.zeros_like(ypart_s)
            elif kind == "FV":
                chunk = jnp.minimum(h - 1, NF - 1)
                c = pl.ds(pl.multiple_of(chunk * TQ, TQ), TQ)
                wg, wu, wd = (_bf(w[:, c]).astype(F32) for w in (wg_s, wu_s, wd_s))
                for t in range(2):
                    xc = xcol_s[t]
                    g = jnp.sum(xc * wg, axis=0, keepdims=True)
                    u = jnp.sum(xc * wu, axis=0, keepdims=True)
                    ypart_s[t] += wd * (g * _sigmoid(g) * u)
            else:
                raise ValueError(kind)
        assert not st and not pp and not rinv and not ov, (st.keys(), pp.keys(), rinv.keys())

    for c in [cp_ckv(0), c_wk, c_wv] + [cp_ckv(i) for i in range(1, NPB)]:
        c.start()
    for c in head0 + head1 + bulk:
        c.start()

    def proj0(t, carry):
        which, blk = t % 2, t // 2
        base = pl.multiple_of(blk * (PB // 2), PB // 2)
        half = pl.multiple_of(blk * (HB // 2), HB // 2)

        @pl.when(which == 0)
        def _():
            cp_ckv(blk).wait()
            for j in range(0, HB // 2, 8):
                at = _bf(ckv_s[pl.ds(base + j, 8), :]).astype(F32)
                ab = _bf(ckv_s[pl.ds(base + HB // 2 + j, 8), :]).astype(F32)
                tt = _lhs_terms(at[:, :HC], at[:, HC:], ab[:, :HC], ab[:, HC:])
                for k, n in enumerate(SUMS):
                    asum_s[k, pl.ds(half + j, 8), :] = _u32(tt[n])

        @pl.when(t == 0)
        def _():
            c_wk.wait()

        @pl.when(t == 1)
        def _():
            c_wv.wait()

        top, bot = pl.ds(base, HB // 2), pl.ds(base + HB // 2, HB // 2)
        lhs = {n: _bf(asum_s[k, pl.ds(half, HB // 2), :]) for k, n in enumerate(SUMS)}
        lhs[2], lhs[3] = _bf(ckv_s[top, :HC]), _bf(ckv_s[bot, HC:])
        f = pltpu.bitcast(wkv32[which, 0] << 16, F32)
        rhs = [t_.astype(BF) for t_ in _rhs_terms(*_quads(f))]
        c11, c12, c21, c22 = _combine({n: _dot(lhs[n], rhs[n], NN) for n in ORD["K"]})
        kv_s[which, top, :] = _u32(jnp.concatenate([c11, c12], axis=1))
        kv_s[which, bot, :] = _u32(jnp.concatenate([c21, c22], axis=1))
        return carry

    lax.fori_loop(0, 2 * NPB, proj0, 0)
    for c in head0:
        c.wait()
    if ONLY != 'loop':
        head(0, _first_order(), first=True)
    for c in head1:
        c.wait()

    def step(h, carry):
        @pl.when(h == 2)
        def _():
            for c in bulk:
                c.wait()

        @pl.when(h == H - 1)
        def _():
            lane = lax.broadcasted_iota(I32, (1, TQ), 1)
            for t in range(2):
                idx = idx_s[t]
                y = jnp.sum(ypart_s[t], axis=1, keepdims=True) * sig_s[t:t + 1, :]
                blk = pl.ds(pl.multiple_of(idx // TQ * TQ, TQ), TQ)
                old = acc[:, blk]
                acc[:, blk] = jnp.where(
                    lane == idx % TQ, old + (1.0 - g_s[:, blk]) * y, old)

        head(h, _loop_order())
        return carry

    if ONLY != 'first':
        lax.fori_loop(1, H, step, 0)
        for i in range(NPB):
            cp_out(i).wait()
    else:
        for c in bulk:
            c.wait()


@jax.jit
def pallas_gated_mix__compressed_kv_cla__moe_arch_mod__prompt_kernel(
    A_x: jax.Array,
    A_c_kv: jax.Array,
    A_w_q: jax.Array,
    A_w_uk: jax.Array,
    A_w_uv: jax.Array,
    A_w_o: jax.Array,
    B_x: jax.Array,
    B_w_r: jax.Array,
    B_w_gate: jax.Array,
    B_w_up: jax.Array,
    B_w_down: jax.Array,
    gate_w: jax.Array,
):
    del B_x
    xT = A_x.reshape(S, M).T
    ckv = A_c_kv.reshape(S, C)
    woT = jnp.transpose(A_w_o, (0, 2, 1))
    wdT = B_w_down.T

    V = pltpu.VMEM
    scratch = [
        V((M // 2, S), U32),
        V((S // 2, M), U32),
        V((S // 2, C), U32),
        V((H // 2, M, D), U32),
        V((2, H // 2, C, D), U32),
        V((H, M // 2, D), U32),
        V((S // 2, D), U32),
        V((2, S // 2, D), U32),
        V((S // 2, D), U32),
        V((M, S), F32),
        V((1, S), F32),
        V((1, S), F32),
        V((M,), BF),
        V((M,), BF),
        V((M // 2, F), U32),
        V((M // 2, F), U32),
        V((M // 2, F), U32),
        V((8, TQ), F32),
        pltpu.SMEM((2,), I32),
        V((2, M, TQ), F32),
        V((2, M, TQ), F32),
        V((5, S // 4, HC), U32),
        V((7, S // 4, PR), U32),
        V((7, S // 4, TQ), U32),
        V((7, S // 4, TQ), U32),
        V((7, S // 4, TQ), U32),
        V((7, S // 4, TQ), U32),
        V((M, S), BF),
        pltpu.SemaphoreType.DMA((NSEM,)),
    ]
    outT = pl.pallas_call(
        _kernel,
        in_specs=[pl.BlockSpec(memory_space=pl.ANY)] * 11,
        out_specs=pl.BlockSpec(memory_space=pl.ANY),
        out_shape=jax.ShapeDtypeStruct((M, S), BF),
        scratch_shapes=scratch,
        compiler_params=pltpu.CompilerParams(
            vmem_limit_bytes=100 * 1024 * 1024),
    )(xT, ckv, A_w_q, A_w_uk, A_w_uv, woT, B_w_r, B_w_gate, B_w_up, wdT, gate_w)
    return outT.T.reshape(1, S, M)
```

```python
import math
import re
_CFG = {'loop': 'Q0,K0,V0,FV0,SB0,SD1,SA0,K1,Q1.1,SS1,V1.4,V1,PA0,PB0,Q1,SD2,SS2.1,SS2,PA1,PB1,K2.4,PD2,SD3,SS3,K2.2,K2,V2.4,PS2,O0,V2.1,V2,Q2.3,Q2,SS4.1,SS4,SS5.1,SS5,PD3,PS3,SD4,SD5,K3.1,K3.5,K3,PS4,V3.1,PD4,Q3,V3,SS6.4,PS5.5,PS5.1,SS6,O1,PS5,PD5,SD6,SS7,PS6,PD6,SD7,O2,PS7.4,PS7.2,PD7,PS7,O3', 'oP': '2014653', 'oO': '1642350', 'oV': '4156023', 'oK': '1043625', 'oS': '0136425', 'qkc': '1', 'oQ': '2634501', 'hyb': '14', 'pform': '1', 'raw': '1', 'lsrc': '2', 'pl': '0', 'fhyb': '14', 'first': 'T0,T2,T3,T1,GB0,GB1,Q0,SA0,SB0,SA1,PB0,SB1,G8,Q1,PA0,SA2,PB1,G9,SB2,G10,PA1,SA3,G11,SB3,G12,PA2,O0,Q2,PB2,G13,SA4,G14,SB4,G15,PA3,PB3,SA5,SB5,PB4,O1,TOPK0,Q3,SA6,SB6,PA4,PA5,PB5,SA7,SB7,PA6,PB6,PA7,O2,PB7,XS0,XS1,XS2,XS3,O3', 'flsrc': '1'}


def E(k, d=''):
    return _CFG.get(k, d)

import jax
import jax.numpy as jnp
from jax import lax
import jax.experimental.pallas as pl
import jax.experimental.pallas.tpu as pltpu

S, M, C, H, D, F = 2048, 448, 1024, 16, 256, 1792
TQ = 128
NQ = S // TQ
PR = 2 * TQ
NP = S // PR
PB = 512
NPB = S // PB
NF = F // TQ
HB, HC, HM = PB // 2, C // 2, M // 2
MP = 512

BF, F32, U32, I32 = jnp.bfloat16, jnp.float32, jnp.uint32, jnp.int32
NN = (((1,), (0,)), ((), ()))
NT = (((1,), (1,)), ((), ()))
LOG2E = math.log2(math.e)
QSCALE = (D ** -0.5) * LOG2E
NEG = -1e9 * LOG2E
HI16 = 0xFFFF0000

S_WK, S_WV, S_HEAD0, S_HEAD1, S_BULK, S_OUT, S_CKV = range(7)
NSEM = S_CKV + NPB

HYB_ = int(E('hyb', 14))
STQ = int(E('stq', 1))
QK0 = int(E('qk0', 99))
PV0 = int(E('pv0', 1))
STO = int(E('sto', 0))
LSRC_ = int(E('lsrc', 2))
QKC = int(E('qkc', 1))
OC = int(E('oc', 1))
ORD = {k: [int(c) for c in E('o' + k, d)] for k, d in
       (('K', '3104625'), ('V', '3104625'), ('Q', '3104625'), ('S', '3104625'),
        ('P', '2304156'), ('O', '0346125'))}
ONLY = E('only')
RAW = int(E('raw', 1))
PFORM = int(E('pform', 0))
PL = int(E('pl', 1))


def _parse(txt):
    out = []
    for t in txt.split(','):
        m = re.match(r'([A-Z]+)(\d+)(?:\.(\d))?$', t)
        out.append((m.group(1), int(m.group(2)), int(m.group(3) or 0)))
    return out


def _dot(a, b, dn):
    return lax.dot_general(a, b, dn, preferred_element_type=F32)


def _cat(xs, axis):
    return xs[0] if len(xs) == 1 else jnp.concatenate(xs, axis=axis)


def _recip(l):
    r = pl.reciprocal(l, approx=True)
    return r * (2.0 - l * r)


def _sigmoid(z):
    return 1.0 / (1.0 + jnp.exp(-z))


def _bf(w):
    return pltpu.bitcast(w, BF)


def _u32(v):
    return pltpu.bitcast(v.astype(BF), U32)


def _rows(ref, r0, r1):
    return _bf(ref[r0 // 2:r1 // 2, :])


def _put_rows(ref, r0, r1, v):
    ref[r0 // 2:r1 // 2, :] = _u32(v)


def _lhs_terms(a11, a12, a21, a22):
    return [a11 + a22, a21 + a22, a11, a22, a11 + a12, a21 - a11, a12 - a22]


def _rhs_terms(b11, b12, b21, b22):
    return [b11 + b22, b11, b12 - b22, b21 - b11, b22, b11 + b12, b21 + b22]


def _quads(f):
    k, n = f.shape[0] // 2, f.shape[1] // 2
    return f[:k, :n], f[:k, n:], f[k:, :n], f[k:, n:]


def _combine(m):
    return (m[0] + m[3] - m[4] + m[6], m[2] + m[4],
            m[1] + m[3], m[0] - m[1] + m[2] + m[5])


SUMS = (0, 1, 4, 5, 6)


def _att(i, st):
    qk = [("SS", i, 0), ("SD", i, 0)] if st and i >= max(QK0, 1) else [("SA", i, 0), ("SB", i, 0)]
    pv = [("PS", i, 0), ("PD", i, 0)] if st and i >= max(PV0, 1) else [("PA", i, 0), ("PB", i, 0)]
    return qk, pv


def _order(st, proj):
    q = lambda b: [("Q", b, 0)]
    kv = lambda b: [("K", b, 0), ("V", b, 0)] if proj else []
    t = q(0) + kv(0) + _att(0, st)[0] + _att(1, st)[0] + kv(1) + _att(0, st)[1] + q(1)
    for i in range(1, NP + 1):
        if i + 1 < NP:
            if i % 2 == 1 and i > 1:
                t += kv((i + 1) // 2) + q((i + 1) // 2)
            t += _att(i + 1, st)[0]
        if i < NP:
            t += _att(i, st)[1]
        if i % 2 == 0:
            t.append(("O", i // 2 - 1, 0))
    return t


def _first_order():
    if E('first'):
        return _parse(E('first'))
    out = [("T", b, 0) for b in range(NPB)] + [("GB", 0, 0), ("GB", 1, 0)]
    g = 8
    for e in _order(False, False):
        out.append(e)
        if ("Q", 1, 0) in out and g < NQ and e[0] in ("Q", "SA", "SB"):
            out.append(("G", g, 0))
            g += 1
        if e == ("O", 1, 0):
            out.append(("TOPK", 0, 0))
    if STQ and E('xp', '0') == '0':
        out += [("XS", b, 0) for b in range(NPB)]
    elif STQ:
        k, res = 0, []
        for e in out:
            res.append(e)
            if e[0] in ("SA", "SB") and e[1] >= int(E('xp0', 0)) and k < 16:
                res.append(("XP", k, 0))
                k += 1
        out = res + [("XP", j, 0) for j in range(k, 16)]
    return out


def _loop_order():
    if E('loop'):
        return _parse(E('loop'))
    out = []
    for e in _order(True, True):
        out.append(e)
        if e == ("V", 0, 0):
            out.append(("FV", 0, 0))
    return out


def _kernel(xT_hbm, ckv_hbm, wq_hbm, wk_hbm, wv_hbm, wo_hbm, wr_hbm, wg_hbm,
            wu_hbm, wd_hbm, gw_hbm, out_hbm,
            xT_s, x_s, ckv_s, wq32, wkv32, wo_s, q_s, kv_s, ctx_s, acc,
            r_s, g_s, wr_s, gw_s, wg_s, wu_s, wd_s, sig_s, idx_s, xcol_s, ypart_s,
            asum_s, xsum_s, qt_s, kt_s, vt_s, ct_s, out_s, sem):
    wk32, wv32 = wkv32.at[0], wkv32.at[1]
    k_s, v_s = kv_s.at[0], kv_s.at[1]
    (xT_u, ckv_u, wq_u, wk_u, wv_u, wo_u, wg_u, wu_u, wd_u) = (
        r.bitcast(U32) for r in (xT_hbm, ckv_hbm, wq_hbm, wk_hbm, wv_hbm,
                                 wo_hbm, wg_hbm, wu_hbm, wd_hbm))

    def cp(src, dst, s):
        return pltpu.make_async_copy(src, dst, sem.at[s])

    def cp_pair(w_u, w_s, p, s):
        return cp(w_u.at[:, p, :], w_s.at[p], s)

    def cp_ckv(i):
        r = pl.ds(pl.multiple_of(PB // 2 * i, PB // 2), PB // 2)
        return cp(ckv_u.at[r, :], ckv_s.at[r, :], S_CKV + i)

    def cp_out(c0, c1):
        r = pl.ds(c0, c1 - c0)
        return cp(out_s.at[:, r], out_hbm.at[:, r], S_OUT)

    def out_blocks(i):
        r0, r1 = PB * i, PB * (i + 1)
        return [(r0, r1)] if i < NPB - 1 else [(r0, r0 + PR), (r0 + PR, r1)]

    c_wk, c_wv = cp_pair(wk_u, wk32, 0, S_WK), cp_pair(wv_u, wv32, 0, S_WV)
    head0 = [cp(xT_u, xT_s, S_HEAD0), cp_pair(wq_u, wq32, 0, S_HEAD0),
             cp(wr_hbm, wr_s, S_HEAD0), cp(gw_hbm, gw_s, S_HEAD0),
             cp(wo_u.at[0], wo_s.at[0], S_HEAD0)]
    head1 = [cp(wo_u.at[1], wo_s.at[1], S_HEAD1), cp(wg_u, wg_s, S_HEAD1),
             cp(wu_u, wu_s, S_HEAD1), cp(wd_u, wd_s, S_HEAD1)]
    rest = pl.ds(2, H - 2)
    bulk = [cp(wo_u.at[rest], wo_s.at[rest], S_BULK)]
    for p in range(1, H // 2):
        bulk += [cp_pair(wk_u, wk32, p, S_BULK), cp_pair(wv_u, wv32, p, S_BULK),
                 cp_pair(wq_u, wq32, p, S_BULK)]

    row = lax.broadcasted_iota(I32, (TQ, TQ), 0)
    col = lax.broadcasted_iota(I32, (TQ, TQ), 1)
    tri = col <= row

    W = TQ // 2

    def term(ref, n, j0, j1):
        raw = RAW and {id(qt_s): (q_s, 2, 3), id(kt_s): (k_s, 1, 4),
                       id(vt_s): (v_s, 1, 4)}.get(id(ref))
        if raw and n in raw[1:]:
            odd = int(n == raw[2])
            return _bf(_cat([raw[0][W * (2 * j + odd):W * (2 * j + odd + 1),
                                    TQ * odd:TQ * (odd + 1)]
                             for j in range(j0, j1)], 0))
        return _bf(ref[n, W * j0:W * j1, :])

    def put_terms(ref, j, terms):
        skip = () if not RAW or ref is ct_s else (2, 3) if ref is qt_s else (1, 4)
        for n, t in enumerate(terms):
            if n not in skip:
                ref[n, W * j:W * (j + 1), :] = _u32(t)

    def head(h, order, first=False):
        if isinstance(h, int):
            pair, shift = h // 2, jnp.uint32(16 * (1 - h % 2))
        else:
            pair = lax.shift_right_logical(h, 1)
            shift = (16 - 16 * (h & 1)).astype(U32)
        kinds = {(k, i) for k, i, _ in order}
        HYB = int(E('fhyb', 14)) if first else HYB_
        LSRC = int(E('flsrc', 2)) if first else LSRC_
        cache, prog = {}, {}

        def weight32(ref):
            return pltpu.bitcast((ref[pair] << shift) & jnp.uint32(HI16), F32)

        def wterms(name):
            if name not in cache:
                if name == "O":
                    f = _bf(wo_s[h]).astype(F32)
                    cache[name] = [t.astype(BF) for t in _lhs_terms(*_quads(f))]
                else:
                    f = weight32({"K": wk32, "V": wv32, "Q": wq32}[name])
                    if name == "Q":
                        f = jnp.concatenate([f, jnp.zeros((MP - M, D), F32)], axis=0)
                    cache[name] = [t.astype(BF) for t in _rhs_terms(*_quads(f))]
            return cache[name]

        def run(key, cnt, product):
            m = prog.setdefault(key, {})
            todo = [n for n in ORD[key[0]] if n not in m]
            for n in (todo[:cnt] if cnt else todo):
                m[n] = product(n)
            return len(m) == 7

        def route(c0, c1):
            if "rg" not in cache:
                r16 = lax.broadcasted_iota(I32, (16, M), 0)
                wr = wr_s[...].astype(F32).reshape(1, M)
                gw = gw_s[...].astype(F32).reshape(1, M)
                cache["rg"] = jnp.where(
                    r16 == 0, wr, jnp.where(r16 == 1, gw, 0.0)).astype(BF)
            rg = _dot(cache["rg"], _bf(xT_s[:, c0:c1]), NN)
            r_s[:, c0:c1] = rg[0:1, :].astype(BF).astype(F32)
            g_s[:, c0:c1] = _sigmoid(rg[1:2, :])

        st, pp, ov, rinv = {}, {}, {}, {}
        last = {}

        def anchor():
            u = pltpu.bitcast(last["v"][0:8, 0:TQ], I32)[0, 0]
            return lax.shift_right_logical(lax.shift_right_logical(u, 31), 1)

        def set_scores(q, s0, s):
            last["v"] = s
            for t in range(s.shape[1] // TQ):
                blk = s[:, TQ * t:TQ * (t + 1)]
                st.setdefault(q, {})[s0 + t] = jnp.where(tri, blk, NEG) if s0 + t == q else blk

        def probs(q, perm):
            if q not in pp:
                tiles = st.pop(q)
                s = _cat([tiles[t] for t in perm], 1)
                p = jnp.exp2(s - jnp.max(s, axis=1, keepdims=True))
                pp[q] = (p, p.astype(BF))
            return pp[q]

        def finish(q, o, src):
            if q < HYB:
                rinv[q] = None
                return o * _recip(jnp.sum(src, axis=1, keepdims=True))
            la = src[:, 0:TQ]
            for t in range(1, src.shape[1] // TQ):
                la = la + src[:, TQ * t:TQ * (t + 1)]
            hi = la.astype(BF)
            lo = (la - hi.astype(F32)).astype(BF)
            l = _dot(jnp.ones((16, 2 * TQ), BF),
                     jnp.concatenate([hi, lo], axis=1), NT)[0:1, :]
            rinv[q] = _recip(l)
            return o

        def store_ctx(q, o):
            last["v"] = o
            i = q // 2
            if STO and not first and 2 * i + 1 < HYB:
                ov[q] = o
                if 2 * i in ov and 2 * i + 1 in ov:
                    oa, ob = ov.pop(2 * i), ov.pop(2 * i + 1)
                    put_terms(ct_s, i, _rhs_terms(oa[:, :TQ], ob[:, :TQ],
                                                  oa[:, TQ:], ob[:, TQ:]))
            else:
                _put_rows(ctx_s, TQ * q, TQ * (q + 1), o)

        def pv_done(i):
            if ("PS", i) in prog.get("done", ()) and ("PD", i) in prog.get("done", ()):
                c11, c12, c21, c22 = _combine(prog.pop(("P", i)))
                da, db = prog.pop(("PDv", i))
                lt = prog.pop(("L", i))
                w = TQ * i
                lf, dg = prog.pop(("Lf", i)), prog.pop(("D", i))
                for q, o, ln in ((2 * i, jnp.concatenate([c11, c12], axis=1) + da, 4),
                                 (2 * i + 1, jnp.concatenate([c21, c22], axis=1) + db, 1)):
                    pf, pb = pp.pop(q)
                    if LSRC == 3:
                        src = jnp.concatenate([lf[ln], pf[:, 2 * w:]], axis=1)
                    elif LSRC == 2:
                        src = jnp.concatenate([lt[ln], dg[q % 2]], axis=1).astype(F32)
                    elif LSRC == 1:
                        src = pb.astype(F32)
                    else:
                        src = pf
                    store_ctx(q, finish(q, o, src))

        for kind, i, cnt in order:
            r0, r1 = PB * i, PB * (i + 1)
            n0 = PR * i
            qa, qb = 2 * i, 2 * i + 1
            eo = [2 * j for j in range(i)] + [2 * j + 1 for j in range(i)]
            if kind == "T":
                _put_rows(x_s, r0, r1, _bf(xT_s[:, r0:r1]).T)
            elif kind == "XS":
                for j in range(0, HB, 16):
                    z = jnp.zeros((16, MP - M), F32)
                    at = jnp.concatenate([_rows(x_s, r0 + j, r0 + j + 16).astype(F32), z], axis=1)
                    ab = jnp.concatenate([_rows(x_s, r0 + HB + j, r0 + HB + j + 16).astype(F32), z], axis=1)
                    tt = _lhs_terms(at[:, :PR], at[:, PR:], ab[:, :PR], ab[:, PR:])
                    for n in range(7):
                        if n != 2:
                            xsum_s[n, (HB * i + j) // 2:(HB * i + j) // 2 + 8, :] = _u32(tt[n])
            elif kind == "XP":
                blk, part = i // 4, i % 4
                z0 = anchor() * 8
                for j in range(64 * part, 64 * part + 64, 16):
                    z = jnp.zeros((16, MP - M), F32)
                    ld = lambda r: jnp.concatenate([_bf(x_s[pl.ds(pl.multiple_of(
                        jnp.minimum(r // 2 + z0, S // 2 - 8), 8), 8), :]).astype(F32), z], axis=1)
                    at, ab = ld(PB * blk + j), ld(PB * blk + HB + j)
                    tt = _lhs_terms(at[:, :PR], at[:, PR:], ab[:, :PR], ab[:, PR:])
                    d0 = (HB * blk + j) // 2
                    for n in range(7):
                        if n != 2:
                            xsum_s[n, d0:d0 + 8, :] = _u32(tt[n])
            elif kind == "GB":
                route(r0, r1)
            elif kind == "G":
                route(TQ * i, TQ * (i + 1))
            elif kind in ("K", "V", "Q"):
                w0, w1 = HB * i // 2, HB * (i + 1) // 2
                if kind == "Q" and (first or not STQ):
                    if "q" not in cache:
                        cache["q"] = weight32(wq32).astype(BF)
                    res = _quads(_dot(_rows(x_s, r0, r1), cache["q"], NN))
                else:
                    def lhs(n):
                        if kind == "Q":
                            if n == 2:
                                return _bf(x_s[r0 // 2:(r0 + HB) // 2, :PR])
                            return _bf(xsum_s[n, w0:w1, :])
                        if n == 2:
                            return _bf(ckv_s[r0 // 2:(r0 + HB) // 2, :HC])
                        if n == 3:
                            return _bf(ckv_s[(r0 + HB) // 2:r1 // 2, HC:])
                        return _bf(asum_s[SUMS.index(n), w0:w1, :])
                    if not run((kind, i), cnt, lambda n: _dot(lhs(n), wterms(kind)[n], NN)):
                        continue
                    res = _combine(prog.pop((kind, i)))
                if kind == "Q":
                    res = [c * QSCALE for c in res]
                dst = {"K": k_s, "V": v_s, "Q": q_s}[kind]
                for j, (c0, c1) in ((2 * i, res[:2]), (2 * i + 1, res[2:])):
                    _put_rows(dst, PR * j, PR * (j + 1), jnp.concatenate([c0, c1], axis=1))
                    if kind == "V" and any(("PS", u) in kinds for u in range(j + 1, NP)):
                        put_terms(vt_s, j, _rhs_terms(c0[:TQ], c1[:TQ], c0[TQ:], c1[TQ:]))
                    if kind == "K" and any(("SS", u) in kinds for u in range(j + 1, NP)):
                        put_terms(kt_s, j, _rhs_terms(c0[:TQ], c0[TQ:], c1[:TQ], c1[TQ:]))
                    if kind == "Q" and ("SS", j) in kinds:
                        put_terms(qt_s, j, _lhs_terms(c0[:TQ], c1[:TQ], c0[TQ:], c1[TQ:]))
            elif kind in ("SA", "SB"):
                q = qa if kind == "SA" else qb
                set_scores(q, 0, _dot(_rows(q_s, TQ * q, TQ * (q + 1)),
                                      _rows(k_s, 0, TQ * (q + 1)), NT))
            elif kind == "SD":
                for q in (qa, qb):
                    set_scores(q, qa, _dot(_rows(q_s, TQ * q, TQ * (q + 1)),
                                           _rows(k_s, n0, TQ * (q + 1)), NT))
            elif kind == "SS":
                qts = [term(qt_s, n, i, i + 1) for n in range(7)]
                done = prog.setdefault(("SSj", i), [0])
                j_end = min(i, done[0] + cnt) if cnt else i
                for j0 in range(done[0], j_end, QKC):
                    j1 = min(j_end, j0 + QKC)
                    cs = _combine({n: _dot(qts[n], term(kt_s, n, j0, j1), NT)
                                   for n in ORD["S"]})
                    for j in range(j0, j1):
                        sl = slice(TQ * (j - j0), TQ * (j - j0 + 1))
                        st.setdefault(qa, {})[2 * j] = cs[0][:, sl]
                        st[qa][2 * j + 1] = cs[1][:, sl]
                        st.setdefault(qb, {})[2 * j] = cs[2][:, sl]
                        st[qb][2 * j + 1] = cs[3][:, sl]
                done[0] = j_end
            elif kind in ("PA", "PB"):
                q = qa if kind == "PA" else qb
                pf, pb = probs(q, range(q + 1))
                pp.pop(q)
                o = _dot(pb, _rows(v_s, 0, TQ * (q + 1)), NN)
                store_ctx(q, finish(q, o, pb.astype(F32) if LSRC in (1, 2) or (LSRC == 3 and PL) else pf))
            elif kind in ("PS", "PD"):
                w = TQ * i
                (paf, pab), (pbf, pbb) = probs(qa, eo + [qa]), probs(qb, eo + [qa, qb])
                if ("D", i) not in prog:
                    prog["D", i] = ((paf[:, 2 * w:].astype(BF), pbf[:, 2 * w:].astype(BF))
                                    if PFORM else (pab[:, 2 * w:], pbb[:, 2 * w:]))
                if kind == "PD":
                    prog["PDv", i] = (_dot(prog["D", i][0], _rows(v_s, n0, n0 + TQ), NN),
                                      _dot(prog["D", i][1], _rows(v_s, n0, n0 + PR), NN))
                else:
                    if ("L", i) not in prog:
                        lf = _lhs_terms(paf[:, :w], paf[:, w:2 * w],
                                        pbf[:, :w], pbf[:, w:2 * w])
                        lt = [t.astype(BF) for t in lf]
                        if not PFORM:
                            lt[2], lt[3] = pab[:, :w], pbb[:, w:2 * w]
                        prog["L", i], prog["Lf", i] = lt, lf
                    if not run(("P", i), cnt, lambda n: _dot(
                            prog["L", i][n], term(vt_s, n, 0, i), NN)):
                        continue
                prog.setdefault("done", set()).add((kind, i))
                pv_done(i)
            elif kind == "O":
                j0, j1 = 2 * i, 2 * i + 2
                js = min(j1, HYB // 2) if STO and not first else j0
                cols = []
                for j in range(j0, js, OC):
                    je = min(js, j + OC)
                    c11, c12, c21, c22 = _combine(
                        {n: _dot(wterms("O")[n], term(ct_s, n, j, je), NT) for n in ORD["O"]})
                    ca = jnp.concatenate([c11, c21], axis=0)
                    cb = jnp.concatenate([c12, c22], axis=0)
                    for t in range(je - j):
                        cols += [ca[:, TQ * t:TQ * (t + 1)], cb[:, TQ * t:TQ * (t + 1)]]
                if j1 > js:
                    cols.append(_dot(_bf(wo_s[h]), _rows(ctx_s, PR * js, PR * j1), NT))
                g = g_s[:, r0:r1]
                f = []
                for t in range(4):
                    gt, rt = g[:, TQ * t:TQ * (t + 1)], rinv.pop(4 * i + t)
                    f.append(gt if rt is None else gt * rt)
                a = _cat(cols, 1) * jnp.concatenate(f, axis=1)
                if first:
                    acc[:, r0:r1] = a + (1.0 - g) * _bf(xT_s[:, r0:r1]).astype(F32)
                else:
                    a = acc[:, r0:r1] + a
                    acc[:, r0:r1] = a
                    for c0, c1 in out_blocks(i):
                        out_s[:, c0:c1] = a[:, c0 - r0:c1 - r0].astype(BF)

                        @pl.when(h == H - 1)
                        def _():
                            cp_out(c0, c1).start()
            elif kind == "TOPK":
                r = r_s[...]
                lane = lax.broadcasted_iota(I32, (1, S), 1)
                m1 = jnp.max(r, axis=1, keepdims=True)
                i1 = jnp.min(jnp.where(r == m1, lane, S - 1))
                r2 = jnp.where(lane == i1, -jnp.inf, r)
                m2 = jnp.max(r2, axis=1, keepdims=True)
                i2 = jnp.min(jnp.where((r2 == m2) & (lane != i1), lane, S - 1))
                r8 = lax.broadcasted_iota(I32, (8, TQ), 0)
                sig_s[...] = jnp.where(r8 == 0, _sigmoid(m1), _sigmoid(m2))
                lane = lax.broadcasted_iota(I32, (1, TQ), 1)
                for t, idx in enumerate((i1, i2)):
                    idx_s[t] = idx
                    blk = pl.ds(pl.multiple_of(idx // TQ * TQ, TQ), TQ)
                    xb = _bf(xT_s[:, blk]).astype(F32)
                    xc = jnp.sum(jnp.where(lane == idx % TQ, xb, 0.0),
                                 axis=1, keepdims=True)
                    xcol_s[t] = jnp.broadcast_to(xc, (M, TQ))
                ypart_s[...] = jnp.zeros_like(ypart_s)
            elif kind == "FV":
                chunk = jnp.minimum(h - 1, NF - 1)
                c = pl.ds(pl.multiple_of(chunk * TQ, TQ), TQ)
                wg, wu, wd = (_bf(w[:, c]).astype(F32) for w in (wg_s, wu_s, wd_s))
                for t in range(2):
                    xc = xcol_s[t]
                    g = jnp.sum(xc * wg, axis=0, keepdims=True)
                    u = jnp.sum(xc * wu, axis=0, keepdims=True)
                    ypart_s[t] += wd * (g * _sigmoid(g) * u)
            else:
                raise ValueError(kind)
        assert not st and not pp and not rinv and not ov, (st.keys(), pp.keys(), rinv.keys())

    for c in [cp_ckv(0), c_wk, c_wv] + [cp_ckv(i) for i in range(1, NPB)]:
        c.start()
    for c in head0 + head1 + bulk:
        c.start()

    def proj0(t, carry):
        which, blk = t % 2, t // 2
        base = pl.multiple_of(blk * (PB // 2), PB // 2)
        half = pl.multiple_of(blk * (HB // 2), HB // 2)

        @pl.when(which == 0)
        def _():
            cp_ckv(blk).wait()
            for j in range(0, HB // 2, 8):
                at = _bf(ckv_s[pl.ds(base + j, 8), :]).astype(F32)
                ab = _bf(ckv_s[pl.ds(base + HB // 2 + j, 8), :]).astype(F32)
                tt = _lhs_terms(at[:, :HC], at[:, HC:], ab[:, :HC], ab[:, HC:])
                for k, n in enumerate(SUMS):
                    asum_s[k, pl.ds(half + j, 8), :] = _u32(tt[n])

        @pl.when(t == 0)
        def _():
            c_wk.wait()

        @pl.when(t == 1)
        def _():
            c_wv.wait()

        top, bot = pl.ds(base, HB // 2), pl.ds(base + HB // 2, HB // 2)
        lhs = {n: _bf(asum_s[k, pl.ds(half, HB // 2), :]) for k, n in enumerate(SUMS)}
        lhs[2], lhs[3] = _bf(ckv_s[top, :HC]), _bf(ckv_s[bot, HC:])
        f = pltpu.bitcast(wkv32[which, 0] << 16, F32)
        rhs = [t_.astype(BF) for t_ in _rhs_terms(*_quads(f))]
        c11, c12, c21, c22 = _combine({n: _dot(lhs[n], rhs[n], NN) for n in ORD["K"]})
        kv_s[which, top, :] = _u32(jnp.concatenate([c11, c12], axis=1))
        kv_s[which, bot, :] = _u32(jnp.concatenate([c21, c22], axis=1))
        return carry

    lax.fori_loop(0, 2 * NPB, proj0, 0)
    for c in head0:
        c.wait()
    if ONLY != 'loop':
        head(0, _first_order(), first=True)
    for c in head1:
        c.wait()

    def step(h, carry):
        @pl.when(h == 2)
        def _():
            for c in bulk:
                c.wait()

        @pl.when(h == H - 1)
        def _():
            lane = lax.broadcasted_iota(I32, (1, TQ), 1)
            for t in range(2):
                idx = idx_s[t]
                y = jnp.sum(ypart_s[t], axis=1, keepdims=True) * sig_s[t:t + 1, :]
                blk = pl.ds(pl.multiple_of(idx // TQ * TQ, TQ), TQ)
                old = acc[:, blk]
                acc[:, blk] = jnp.where(
                    lane == idx % TQ, old + (1.0 - g_s[:, blk]) * y, old)

        head(h, _loop_order())
        return carry

    if ONLY != 'first':
        lax.fori_loop(1, H, step, 0)
        for i in range(NPB):
            for c0, c1 in out_blocks(i):
                cp_out(c0, c1).wait()
    else:
        for c in bulk:
            c.wait()
        k = idx_s[0] & 7
        r = pl.ds(pl.multiple_of((idx_s[1] & 63) * 8, 8), 8)
        out_s[0:16, 0:PR] = _bf(xsum_s[jnp.minimum(k, 6), r, :]) + xcol_s[0, 0:16, 0:1].astype(BF) + \
            acc[pl.ds(pl.multiple_of(k * 16, 16), 16), 0:PR].astype(BF) + ypart_s[1, 0:16, 0:1].astype(BF)
        cp_out(0, PB).start()
        cp_out(0, PB).wait()


@jax.jit
def pallas_gated_mix__compressed_kv_cla__moe_arch_mod__prompt_kernel(
    A_x: jax.Array,
    A_c_kv: jax.Array,
    A_w_q: jax.Array,
    A_w_uk: jax.Array,
    A_w_uv: jax.Array,
    A_w_o: jax.Array,
    B_x: jax.Array,
    B_w_r: jax.Array,
    B_w_gate: jax.Array,
    B_w_up: jax.Array,
    B_w_down: jax.Array,
    gate_w: jax.Array,
):
    del B_x
    xT = A_x.reshape(S, M).T
    ckv = A_c_kv.reshape(S, C)
    woT = jnp.transpose(A_w_o, (0, 2, 1))
    wdT = B_w_down.T

    V = pltpu.VMEM
    scratch = [
        V((M // 2, S), U32),
        V((S // 2, M), U32),
        V((S // 2, C), U32),
        V((H // 2, M, D), U32),
        V((2, H // 2, C, D), U32),
        V((H, M // 2, D), U32),
        V((S // 2, D), U32),
        V((2, S // 2, D), U32),
        V((S // 2, D), U32),
        V((M, S), F32),
        V((1, S), F32),
        V((1, S), F32),
        V((M,), BF),
        V((M,), BF),
        V((M // 2, F), U32),
        V((M // 2, F), U32),
        V((M // 2, F), U32),
        V((8, TQ), F32),
        pltpu.SMEM((2,), I32),
        V((2, M, TQ), F32),
        V((2, M, TQ), F32),
        V((5, S // 4, HC), U32),
        V((7, S // 4, PR), U32),
        V((7, S // 4, TQ), U32),
        V((7, S // 4, TQ), U32),
        V((7, S // 4, TQ), U32),
        V((7, S // 4, TQ), U32),
        V((M, S), BF),
        pltpu.SemaphoreType.DMA((NSEM,)),
    ]
    outT = pl.pallas_call(
        _kernel,
        in_specs=[pl.BlockSpec(memory_space=pl.ANY)] * 11,
        out_specs=pl.BlockSpec(memory_space=pl.ANY),
        out_shape=jax.ShapeDtypeStruct((M, S), BF),
        scratch_shapes=scratch,
        compiler_params=pltpu.CompilerParams(
            vmem_limit_bytes=100 * 1024 * 1024),
    )(xT, ckv, A_w_q, A_w_uk, A_w_uv, woT, B_w_r, B_w_gate, B_w_up, wdT, gate_w)
    return outT.T.reshape(1, S, M)
```

```python
import math
import re
_CFG = {'loop': 'K0.4,K0.2,Q0,K0,V0,SD1,SB0,SS1,SA0,K1,V1.4,FV0,V1,PA0,Q1,SD2,SS2,PA1,PB1,K2.2,PB0,SD3,PD2,K2.2,V2.1,K2,SS3,V2.4,PS2,V2,Q2.3,O0,Q2,SS4.1,SS4,SS5.1,SS5.1,K3.1,SS5,SD4,PS3,SD5,K3.5,K3,PD3,PS4,PD4,Q3,SS6.4,PS5.5,V3,PS5.1,SS6,O1,PD5,SD6,SS7,PS6,PS5,PD6,SD7,O2,PS7.4,PS7.2,PD7,PS7,O3', 'oP': '2014653', 'oO': '0341625', 'oV': '4150623', 'oK': '1403625', 'oS': '0136425', 'qkc': '1', 'oQ': '2546301', 'hyb': '14', 'pform': '1', 'raw': '1', 'lsrc': '2', 'pl': '1', 'sto': '2', 'oc': '2', 'fhyb': '14', 'first': 'T0,T2,T3,T1,GB0,GB1,Q0,SA0,SB0,SA1,PB0,SB1,G8,Q1,PA0,SA2,PB1,G9,SB2,G10,PA1,SA3,G11,SB3,G12,PA2,O0,Q2,PB2,G13,SA4,G14,SB4,G15,PA3,PB3,SA5,SB5,PB4,O1,TOPK0,Q3,SA6,SB6,PA4,PA5,PB5,SA7,SB7,PA6,PB6,PA7,O2,PB7,XS0,XS1,XS2,XS3,O3', 'flsrc': '1'}


def E(k, d=''):
    return _CFG.get(k, d)

import jax
import jax.numpy as jnp
from jax import lax
import jax.experimental.pallas as pl
import jax.experimental.pallas.tpu as pltpu

S, M, C, H, D, F = 2048, 448, 1024, 16, 256, 1792
TQ = 128
NQ = S // TQ
PR = 2 * TQ
NP = S // PR
PB = 512
NPB = S // PB
NF = F // TQ
HB, HC, HM = PB // 2, C // 2, M // 2
MP = 512

BF, F32, U32, I32 = jnp.bfloat16, jnp.float32, jnp.uint32, jnp.int32
NN = (((1,), (0,)), ((), ()))
NT = (((1,), (1,)), ((), ()))
LOG2E = math.log2(math.e)
QSCALE = (D ** -0.5) * LOG2E
NEG = -1e9 * LOG2E
HI16 = 0xFFFF0000

S_WK, S_WV, S_HEAD0, S_HEAD1, S_BULK, S_OUT, S_CKV = range(7)
NSEM = S_CKV + NPB

HYB_ = int(E('hyb', 14))
STQ = int(E('stq', 1))
QK0 = int(E('qk0', 99))
PV0 = int(E('pv0', 1))
STO = int(E('sto', 0))
LSRC_ = int(E('lsrc', 2))
QKC = int(E('qkc', 1))
OC = int(E('oc', 1))
ORD = {k: [int(c) for c in E('o' + k, d)] for k, d in
       (('K', '3104625'), ('V', '3104625'), ('Q', '3104625'), ('S', '3104625'),
        ('P', '2304156'), ('O', '0346125'))}
ONLY = E('only')
RAW = int(E('raw', 1))
PFORM = int(E('pform', 0))
PL = int(E('pl', 1))
TVAL = int(E('tval', 0))


def _parse(txt):
    out = []
    for t in txt.split(','):
        m = re.match(r'([A-Z]+)(\d+)(?:\.(\d))?$', t)
        out.append((m.group(1), int(m.group(2)), int(m.group(3) or 0)))
    return out


def _dot(a, b, dn):
    return lax.dot_general(a, b, dn, preferred_element_type=F32)


def _cat(xs, axis):
    return xs[0] if len(xs) == 1 else jnp.concatenate(xs, axis=axis)


def _recip(l):
    r = pl.reciprocal(l, approx=True)
    return r * (2.0 - l * r)


def _sigmoid(z):
    return 1.0 / (1.0 + jnp.exp(-z))


def _bf(w):
    return pltpu.bitcast(w, BF)


def _u32(v):
    return pltpu.bitcast(v.astype(BF), U32)


def _rows(ref, r0, r1):
    return _bf(ref[r0 // 2:r1 // 2, :])


def _put_rows(ref, r0, r1, v):
    ref[r0 // 2:r1 // 2, :] = _u32(v)


def _lhs_terms(a11, a12, a21, a22):
    return [a11 + a22, a21 + a22, a11, a22, a11 + a12, a21 - a11, a12 - a22]


def _rhs_terms(b11, b12, b21, b22):
    return [b11 + b22, b11, b12 - b22, b21 - b11, b22, b11 + b12, b21 + b22]


def _quads(f):
    k, n = f.shape[0] // 2, f.shape[1] // 2
    return f[:k, :n], f[:k, n:], f[k:, :n], f[k:, n:]


def _combine(m):
    return (m[0] + m[3] - m[4] + m[6], m[2] + m[4],
            m[1] + m[3], m[0] - m[1] + m[2] + m[5])


SUMS = (0, 1, 4, 5, 6)


def _att(i, st):
    qk = [("SS", i, 0), ("SD", i, 0)] if st and i >= max(QK0, 1) else [("SA", i, 0), ("SB", i, 0)]
    pv = [("PS", i, 0), ("PD", i, 0)] if st and i >= max(PV0, 1) else [("PA", i, 0), ("PB", i, 0)]
    return qk, pv


def _order(st, proj):
    q = lambda b: [("Q", b, 0)]
    kv = lambda b: [("K", b, 0), ("V", b, 0)] if proj else []
    t = q(0) + kv(0) + _att(0, st)[0] + _att(1, st)[0] + kv(1) + _att(0, st)[1] + q(1)
    for i in range(1, NP + 1):
        if i + 1 < NP:
            if i % 2 == 1 and i > 1:
                t += kv((i + 1) // 2) + q((i + 1) // 2)
            t += _att(i + 1, st)[0]
        if i < NP:
            t += _att(i, st)[1]
        if i % 2 == 0:
            t.append(("O", i // 2 - 1, 0))
    return t


def _first_order():
    if E('first'):
        return _parse(E('first'))
    out = [("T", b, 0) for b in range(NPB)] + [("GB", 0, 0), ("GB", 1, 0)]
    g = 8
    for e in _order(False, False):
        out.append(e)
        if ("Q", 1, 0) in out and g < NQ and e[0] in ("Q", "SA", "SB"):
            out.append(("G", g, 0))
            g += 1
        if e == ("O", 1, 0):
            out.append(("TOPK", 0, 0))
    if STQ and E('xp', '0') == '0':
        out += [("XS", b, 0) for b in range(NPB)]
    elif STQ:
        k, res = 0, []
        for e in out:
            res.append(e)
            if e[0] in ("SA", "SB") and e[1] >= int(E('xp0', 0)) and k < 16:
                res.append(("XP", k, 0))
                k += 1
        out = res + [("XP", j, 0) for j in range(k, 16)]
    return out


def _loop_order():
    if E('loop'):
        return _parse(E('loop'))
    out = []
    for e in _order(True, True):
        out.append(e)
        if e == ("V", 0, 0):
            out.append(("FV", 0, 0))
    return out


def _kernel(xT_hbm, ckv_hbm, wq_hbm, wk_hbm, wv_hbm, wo_hbm, wr_hbm, wg_hbm,
            wu_hbm, wd_hbm, gw_hbm, out_hbm,
            xT_s, x_s, ckv_s, wq32, wkv32, wo_s, q_s, kv_s, ctx_s, acc,
            r_s, g_s, wr_s, gw_s, wg_s, wu_s, wd_s, sig_s, idx_s, xcol_s, ypart_s,
            asum_s, xsum_s, qt_s, kt_s, vt_s, ct_s, out_s, sem):
    wk32, wv32 = wkv32.at[0], wkv32.at[1]
    k_s, v_s = kv_s.at[0], kv_s.at[1]
    (xT_u, ckv_u, wq_u, wk_u, wv_u, wo_u, wg_u, wu_u, wd_u) = (
        r.bitcast(U32) for r in (xT_hbm, ckv_hbm, wq_hbm, wk_hbm, wv_hbm,
                                 wo_hbm, wg_hbm, wu_hbm, wd_hbm))

    def cp(src, dst, s):
        return pltpu.make_async_copy(src, dst, sem.at[s])

    def cp_pair(w_u, w_s, p, s):
        return cp(w_u.at[:, p, :], w_s.at[p], s)

    def cp_ckv(i):
        r = pl.ds(pl.multiple_of(PB // 2 * i, PB // 2), PB // 2)
        return cp(ckv_u.at[r, :], ckv_s.at[r, :], S_CKV + i)

    def cp_out(c0, c1):
        r = pl.ds(c0, c1 - c0)
        return cp(out_s.at[:, r], out_hbm.at[:, r], S_OUT)

    def out_blocks(i):
        r0, r1 = PB * i, PB * (i + 1)
        return [(r0, r1)] if i < NPB - 1 else [(r0, r0 + PR), (r0 + PR, r1)]

    c_wk, c_wv = cp_pair(wk_u, wk32, 0, S_WK), cp_pair(wv_u, wv32, 0, S_WV)
    head0 = [cp(xT_u, xT_s, S_HEAD0), cp_pair(wq_u, wq32, 0, S_HEAD0),
             cp(wr_hbm, wr_s, S_HEAD0), cp(gw_hbm, gw_s, S_HEAD0),
             cp(wo_u.at[0], wo_s.at[0], S_HEAD0)]
    head1 = [cp(wo_u.at[1], wo_s.at[1], S_HEAD1), cp(wg_u, wg_s, S_HEAD1),
             cp(wu_u, wu_s, S_HEAD1), cp(wd_u, wd_s, S_HEAD1)]
    rest = pl.ds(2, H - 2)
    bulk = [cp(wo_u.at[rest], wo_s.at[rest], S_BULK)]
    for p in range(1, H // 2):
        bulk += [cp_pair(wk_u, wk32, p, S_BULK), cp_pair(wv_u, wv32, p, S_BULK),
                 cp_pair(wq_u, wq32, p, S_BULK)]

    row = lax.broadcasted_iota(I32, (TQ, TQ), 0)
    col = lax.broadcasted_iota(I32, (TQ, TQ), 1)
    tri = col <= row

    W = TQ // 2

    def term(ref, n, j0, j1):
        raw = RAW and {id(qt_s): (q_s, 2, 3), id(kt_s): (k_s, 1, 4),
                       id(vt_s): (v_s, 1, 4)}.get(id(ref))
        if raw and n in raw[1:]:
            odd = int(n == raw[2])
            return _bf(_cat([raw[0][W * (2 * j + odd):W * (2 * j + odd + 1),
                                    TQ * odd:TQ * (odd + 1)]
                             for j in range(j0, j1)], 0))
        if (id(ref), n, j0) in held:
            return _cat([held[id(ref), n, j] for j in range(j0, j1)], 0)
        return _bf(ref[n, W * j0:W * j1, :])

    held = {}

    def put_terms(ref, j, terms):
        skip = () if not RAW or ref is ct_s else (2, 3) if ref is qt_s else (1, 4)
        bit = {id(ct_s): 1, id(kt_s): 2, id(qt_s): 4, id(vt_s): 8}[id(ref)]
        for n, t in enumerate(terms):
            if n in skip:
                continue
            if TVAL & bit:
                held[id(ref), n, j] = t.astype(BF)
            else:
                ref[n, W * j:W * (j + 1), :] = _u32(t)

    def head(h, order, first=False):
        if isinstance(h, int):
            pair, shift = h // 2, jnp.uint32(16 * (1 - h % 2))
        else:
            pair = lax.shift_right_logical(h, 1)
            shift = (16 - 16 * (h & 1)).astype(U32)
        kinds = {(k, i) for k, i, _ in order}
        HYB = int(E('fhyb', 14)) if first else HYB_
        LSRC = int(E('flsrc', 2)) if first else LSRC_
        cache, prog = {}, {}

        def weight32(ref):
            return pltpu.bitcast((ref[pair] << shift) & jnp.uint32(HI16), F32)

        def wterms(name):
            if name not in cache:
                if name == "O":
                    f = _bf(wo_s[h]).astype(F32)
                    cache[name] = [t.astype(BF) for t in _lhs_terms(*_quads(f))]
                else:
                    f = weight32({"K": wk32, "V": wv32, "Q": wq32}[name])
                    if name == "Q":
                        f = jnp.concatenate([f, jnp.zeros((MP - M, D), F32)], axis=0)
                    cache[name] = [t.astype(BF) for t in _rhs_terms(*_quads(f))]
            return cache[name]

        def run(key, cnt, product):
            m = prog.setdefault(key, {})
            todo = [n for n in ORD[key[0]] if n not in m]
            for n in (todo[:cnt] if cnt else todo):
                m[n] = product(n)
            return len(m) == 7

        def route(c0, c1):
            if "rg" not in cache:
                r16 = lax.broadcasted_iota(I32, (16, M), 0)
                wr = wr_s[...].astype(F32).reshape(1, M)
                gw = gw_s[...].astype(F32).reshape(1, M)
                cache["rg"] = jnp.where(
                    r16 == 0, wr, jnp.where(r16 == 1, gw, 0.0)).astype(BF)
            rg = _dot(cache["rg"], _bf(xT_s[:, c0:c1]), NN)
            r_s[:, c0:c1] = rg[0:1, :].astype(BF).astype(F32)
            g_s[:, c0:c1] = _sigmoid(rg[1:2, :])

        st, pp, ov, rinv = {}, {}, {}, {}
        last = {}

        def anchor():
            u = pltpu.bitcast(last["v"][0:8, 0:TQ], I32)[0, 0]
            return lax.shift_right_logical(lax.shift_right_logical(u, 31), 1)

        def set_scores(q, s0, s):
            last["v"] = s
            for t in range(s.shape[1] // TQ):
                blk = s[:, TQ * t:TQ * (t + 1)]
                st.setdefault(q, {})[s0 + t] = jnp.where(tri, blk, NEG) if s0 + t == q else blk

        def probs(q, perm):
            if q not in pp:
                tiles = st.pop(q)
                s = _cat([tiles[t] for t in perm], 1)
                p = jnp.exp2(s - jnp.max(s, axis=1, keepdims=True))
                pp[q] = (p, p.astype(BF))
            return pp[q]

        def finish(q, o, src):
            if q < HYB:
                rinv[q] = None
                return o * _recip(jnp.sum(src, axis=1, keepdims=True))
            la = src[:, 0:TQ]
            for t in range(1, src.shape[1] // TQ):
                la = la + src[:, TQ * t:TQ * (t + 1)]
            hi = la.astype(BF)
            lo = (la - hi.astype(F32)).astype(BF)
            l = _dot(jnp.ones((16, 2 * TQ), BF),
                     jnp.concatenate([hi, lo], axis=1), NT)[0:1, :]
            rinv[q] = _recip(l)
            return o

        def store_ctx(q, o):
            last["v"] = o
            i = q // 2
            if i // 2 < STO and not first and 2 * i + 1 < HYB:
                ov[q] = o
                if 2 * i in ov and 2 * i + 1 in ov:
                    oa, ob = ov.pop(2 * i), ov.pop(2 * i + 1)
                    put_terms(ct_s, i, _rhs_terms(oa[:, :TQ], ob[:, :TQ],
                                                  oa[:, TQ:], ob[:, TQ:]))
            else:
                _put_rows(ctx_s, TQ * q, TQ * (q + 1), o)

        def pv_done(i):
            if ("PS", i) in prog.get("done", ()) and ("PD", i) in prog.get("done", ()):
                c11, c12, c21, c22 = _combine(prog.pop(("P", i)))
                da, db = prog.pop(("PDv", i))
                lt = prog.pop(("L", i))
                w = TQ * i
                lf, dg = prog.pop(("Lf", i)), prog.pop(("D", i))
                for q, o, ln in ((2 * i, jnp.concatenate([c11, c12], axis=1) + da, 4),
                                 (2 * i + 1, jnp.concatenate([c21, c22], axis=1) + db, 1)):
                    pf, pb = pp.pop(q)
                    if LSRC == 3:
                        src = jnp.concatenate([lf[ln], pf[:, 2 * w:]], axis=1)
                    elif LSRC == 2:
                        src = jnp.concatenate([lt[ln], dg[q % 2]], axis=1).astype(F32)
                    elif LSRC == 1:
                        src = pb.astype(F32)
                    else:
                        src = pf
                    store_ctx(q, finish(q, o, src))

        for kind, i, cnt in order:
            r0, r1 = PB * i, PB * (i + 1)
            n0 = PR * i
            qa, qb = 2 * i, 2 * i + 1
            eo = [2 * j for j in range(i)] + [2 * j + 1 for j in range(i)]
            if kind == "T":
                _put_rows(x_s, r0, r1, _bf(xT_s[:, r0:r1]).T)
            elif kind == "XS":
                for j in range(0, HB, 16):
                    z = jnp.zeros((16, MP - M), F32)
                    at = jnp.concatenate([_rows(x_s, r0 + j, r0 + j + 16).astype(F32), z], axis=1)
                    ab = jnp.concatenate([_rows(x_s, r0 + HB + j, r0 + HB + j + 16).astype(F32), z], axis=1)
                    tt = _lhs_terms(at[:, :PR], at[:, PR:], ab[:, :PR], ab[:, PR:])
                    for n in range(7):
                        if n != 2:
                            xsum_s[n, (HB * i + j) // 2:(HB * i + j) // 2 + 8, :] = _u32(tt[n])
            elif kind == "XP":
                blk, part = i // 4, i % 4
                z0 = anchor() * 8
                for j in range(64 * part, 64 * part + 64, 16):
                    z = jnp.zeros((16, MP - M), F32)
                    ld = lambda r: jnp.concatenate([_bf(x_s[pl.ds(pl.multiple_of(
                        jnp.minimum(r // 2 + z0, S // 2 - 8), 8), 8), :]).astype(F32), z], axis=1)
                    at, ab = ld(PB * blk + j), ld(PB * blk + HB + j)
                    tt = _lhs_terms(at[:, :PR], at[:, PR:], ab[:, :PR], ab[:, PR:])
                    d0 = (HB * blk + j) // 2
                    for n in range(7):
                        if n != 2:
                            xsum_s[n, d0:d0 + 8, :] = _u32(tt[n])
            elif kind == "GB":
                route(r0, r1)
            elif kind == "G":
                route(TQ * i, TQ * (i + 1))
            elif kind in ("K", "V", "Q"):
                w0, w1 = HB * i // 2, HB * (i + 1) // 2
                if kind == "Q" and (first or not STQ):
                    if "q" not in cache:
                        cache["q"] = weight32(wq32).astype(BF)
                    res = _quads(_dot(_rows(x_s, r0, r1), cache["q"], NN))
                else:
                    def lhs(n):
                        if kind == "Q":
                            if n == 2:
                                return _bf(x_s[r0 // 2:(r0 + HB) // 2, :PR])
                            return _bf(xsum_s[n, w0:w1, :])
                        if n == 2:
                            return _bf(ckv_s[r0 // 2:(r0 + HB) // 2, :HC])
                        if n == 3:
                            return _bf(ckv_s[(r0 + HB) // 2:r1 // 2, HC:])
                        return _bf(asum_s[SUMS.index(n), w0:w1, :])
                    if not run((kind, i), cnt, lambda n: _dot(lhs(n), wterms(kind)[n], NN)):
                        continue
                    res = _combine(prog.pop((kind, i)))
                if kind == "Q":
                    res = [c * QSCALE for c in res]
                dst = {"K": k_s, "V": v_s, "Q": q_s}[kind]
                for j, (c0, c1) in ((2 * i, res[:2]), (2 * i + 1, res[2:])):
                    _put_rows(dst, PR * j, PR * (j + 1), jnp.concatenate([c0, c1], axis=1))
                    if kind == "V" and any(("PS", u) in kinds for u in range(j + 1, NP)):
                        put_terms(vt_s, j, _rhs_terms(c0[:TQ], c1[:TQ], c0[TQ:], c1[TQ:]))
                    if kind == "K" and any(("SS", u) in kinds for u in range(j + 1, NP)):
                        put_terms(kt_s, j, _rhs_terms(c0[:TQ], c0[TQ:], c1[:TQ], c1[TQ:]))
                    if kind == "Q" and ("SS", j) in kinds:
                        put_terms(qt_s, j, _lhs_terms(c0[:TQ], c1[:TQ], c0[TQ:], c1[TQ:]))
            elif kind in ("SA", "SB"):
                q = qa if kind == "SA" else qb
                set_scores(q, 0, _dot(_rows(q_s, TQ * q, TQ * (q + 1)),
                                      _rows(k_s, 0, TQ * (q + 1)), NT))
            elif kind == "SD":
                for q in (qa, qb):
                    set_scores(q, qa, _dot(_rows(q_s, TQ * q, TQ * (q + 1)),
                                           _rows(k_s, n0, TQ * (q + 1)), NT))
            elif kind == "SS":
                qts = [term(qt_s, n, i, i + 1) for n in range(7)]
                done = prog.setdefault(("SSj", i), [0])
                j_end = min(i, done[0] + cnt) if cnt else i
                for j0 in range(done[0], j_end, QKC):
                    j1 = min(j_end, j0 + QKC)
                    cs = _combine({n: _dot(qts[n], term(kt_s, n, j0, j1), NT)
                                   for n in ORD["S"]})
                    for j in range(j0, j1):
                        sl = slice(TQ * (j - j0), TQ * (j - j0 + 1))
                        st.setdefault(qa, {})[2 * j] = cs[0][:, sl]
                        st[qa][2 * j + 1] = cs[1][:, sl]
                        st.setdefault(qb, {})[2 * j] = cs[2][:, sl]
                        st[qb][2 * j + 1] = cs[3][:, sl]
                done[0] = j_end
            elif kind in ("PA", "PB"):
                q = qa if kind == "PA" else qb
                pf, pb = probs(q, range(q + 1))
                pp.pop(q)
                o = _dot(pb, _rows(v_s, 0, TQ * (q + 1)), NN)
                store_ctx(q, finish(q, o, pb.astype(F32) if LSRC in (1, 2) or (LSRC == 3 and PL) else pf))
            elif kind in ("PS", "PD"):
                w = TQ * i
                (paf, pab), (pbf, pbb) = probs(qa, eo + [qa]), probs(qb, eo + [qa, qb])
                if ("D", i) not in prog:
                    prog["D", i] = ((paf[:, 2 * w:].astype(BF), pbf[:, 2 * w:].astype(BF))
                                    if PFORM else (pab[:, 2 * w:], pbb[:, 2 * w:]))
                if kind == "PD":
                    prog["PDv", i] = (_dot(prog["D", i][0], _rows(v_s, n0, n0 + TQ), NN),
                                      _dot(prog["D", i][1], _rows(v_s, n0, n0 + PR), NN))
                else:
                    if ("L", i) not in prog:
                        lf = _lhs_terms(paf[:, :w], paf[:, w:2 * w],
                                        pbf[:, :w], pbf[:, w:2 * w])
                        lt = [t.astype(BF) for t in lf]
                        if not PFORM:
                            lt[2], lt[3] = pab[:, :w], pbb[:, w:2 * w]
                        prog["L", i], prog["Lf", i] = lt, lf
                    def pprod(n):
                        l_ = prog["L", i][n]
                        if not TVAL & 16:
                            return _dot(l_, term(vt_s, n, 0, i), NN)
                        parts = [_dot(l_[:, TQ * j:TQ * (j + 1)], term(vt_s, n, j, j + 1), NN)
                                 for j in range(i)]
                        tot = parts[0]
                        for x in parts[1:]:
                            tot = tot + x
                        return tot
                    if not run(("P", i), cnt, pprod):
                        continue
                prog.setdefault("done", set()).add((kind, i))
                pv_done(i)
            elif kind == "O":
                j0, j1 = 2 * i, 2 * i + 2
                js = max(j0, min(j1, HYB // 2)) if i < STO and not first else j0
                cols = []
                for j in range(j0, js, OC):
                    je = min(js, j + OC)
                    c11, c12, c21, c22 = _combine(
                        {n: _dot(wterms("O")[n], term(ct_s, n, j, je), NT) for n in ORD["O"]})
                    ca = jnp.concatenate([c11, c21], axis=0)
                    cb = jnp.concatenate([c12, c22], axis=0)
                    for t in range(je - j):
                        cols += [ca[:, TQ * t:TQ * (t + 1)], cb[:, TQ * t:TQ * (t + 1)]]
                if j1 > js:
                    cols.append(_dot(_bf(wo_s[h]), _rows(ctx_s, PR * js, PR * j1), NT))
                g = g_s[:, r0:r1]
                f = []
                for t in range(4):
                    gt, rt = g[:, TQ * t:TQ * (t + 1)], rinv.pop(4 * i + t)
                    f.append(gt if rt is None else gt * rt)
                a = _cat(cols, 1) * jnp.concatenate(f, axis=1)
                if first:
                    acc[:, r0:r1] = a + (1.0 - g) * _bf(xT_s[:, r0:r1]).astype(F32)
                else:
                    a = acc[:, r0:r1] + a
                    acc[:, r0:r1] = a
                    for c0, c1 in out_blocks(i):
                        out_s[:, c0:c1] = a[:, c0 - r0:c1 - r0].astype(BF)

                        @pl.when(h == H - 1)
                        def _():
                            cp_out(c0, c1).start()
            elif kind == "TOPK":
                r = r_s[...]
                lane = lax.broadcasted_iota(I32, (1, S), 1)
                m1 = jnp.max(r, axis=1, keepdims=True)
                i1 = jnp.min(jnp.where(r == m1, lane, S - 1))
                r2 = jnp.where(lane == i1, -jnp.inf, r)
                m2 = jnp.max(r2, axis=1, keepdims=True)
                i2 = jnp.min(jnp.where((r2 == m2) & (lane != i1), lane, S - 1))
                r8 = lax.broadcasted_iota(I32, (8, TQ), 0)
                sig_s[...] = jnp.where(r8 == 0, _sigmoid(m1), _sigmoid(m2))
                lane = lax.broadcasted_iota(I32, (1, TQ), 1)
                for t, idx in enumerate((i1, i2)):
                    idx_s[t] = idx
                    blk = pl.ds(pl.multiple_of(idx // TQ * TQ, TQ), TQ)
                    xb = _bf(xT_s[:, blk]).astype(F32)
                    xc = jnp.sum(jnp.where(lane == idx % TQ, xb, 0.0),
                                 axis=1, keepdims=True)
                    xcol_s[t] = jnp.broadcast_to(xc, (M, TQ))
                ypart_s[...] = jnp.zeros_like(ypart_s)
            elif kind == "FV":
                chunk = jnp.minimum(h - 1, NF - 1)
                c = pl.ds(pl.multiple_of(chunk * TQ, TQ), TQ)
                wg, wu, wd = (_bf(w[:, c]).astype(F32) for w in (wg_s, wu_s, wd_s))
                for t in range(2):
                    xc = xcol_s[t]
                    g = jnp.sum(xc * wg, axis=0, keepdims=True)
                    u = jnp.sum(xc * wu, axis=0, keepdims=True)
                    ypart_s[t] += wd * (g * _sigmoid(g) * u)
            elif kind in ("FG", "FU", "FD"):
                if "fc" not in cache:
                    chunk = jnp.minimum(h - 1, NF - 1)
                    cache["fc"] = pl.ds(pl.multiple_of(chunk * TQ, TQ), TQ)
                w = _bf({"FG": wg_s, "FU": wu_s, "FD": wd_s}[kind][:, cache["fc"]])
                w = w.astype(F32)
                if kind != "FD":
                    cache[kind] = [jnp.sum(xcol_s[t] * w, axis=0, keepdims=True)
                                   for t in range(2)]
                else:
                    for t in range(2):
                        g, u = cache["FG"][t], cache["FU"][t]
                        ypart_s[t] += w * (g * _sigmoid(g) * u)
            else:
                raise ValueError(kind)
        assert not st and not pp and not rinv and not ov, (st.keys(), pp.keys(), rinv.keys())

    for c in [cp_ckv(0), c_wk, c_wv] + [cp_ckv(i) for i in range(1, NPB)]:
        c.start()
    for c in head0 + head1 + bulk:
        c.start()

    def proj0(t, carry):
        which, blk = t % 2, t // 2
        base = pl.multiple_of(blk * (PB // 2), PB // 2)
        half = pl.multiple_of(blk * (HB // 2), HB // 2)

        @pl.when(which == 0)
        def _():
            cp_ckv(blk).wait()
            for j in range(0, HB // 2, 8):
                at = _bf(ckv_s[pl.ds(base + j, 8), :]).astype(F32)
                ab = _bf(ckv_s[pl.ds(base + HB // 2 + j, 8), :]).astype(F32)
                tt = _lhs_terms(at[:, :HC], at[:, HC:], ab[:, :HC], ab[:, HC:])
                for k, n in enumerate(SUMS):
                    asum_s[k, pl.ds(half + j, 8), :] = _u32(tt[n])

        @pl.when(t == 0)
        def _():
            c_wk.wait()

        @pl.when(t == 1)
        def _():
            c_wv.wait()

        top, bot = pl.ds(base, HB // 2), pl.ds(base + HB // 2, HB // 2)
        lhs = {n: _bf(asum_s[k, pl.ds(half, HB // 2), :]) for k, n in enumerate(SUMS)}
        lhs[2], lhs[3] = _bf(ckv_s[top, :HC]), _bf(ckv_s[bot, HC:])
        f = pltpu.bitcast(wkv32[which, 0] << 16, F32)
        rhs = [t_.astype(BF) for t_ in _rhs_terms(*_quads(f))]
        c11, c12, c21, c22 = _combine({n: _dot(lhs[n], rhs[n], NN) for n in ORD["K"]})
        kv_s[which, top, :] = _u32(jnp.concatenate([c11, c12], axis=1))
        kv_s[which, bot, :] = _u32(jnp.concatenate([c21, c22], axis=1))
        return carry

    lax.fori_loop(0, 2 * NPB, proj0, 0)
    for c in head0:
        c.wait()
    if ONLY != 'loop':
        head(0, _first_order(), first=True)
    for c in head1:
        c.wait()

    def step(h, carry):
        @pl.when(h == 2)
        def _():
            for c in bulk:
                c.wait()

        @pl.when((h == H - 1) if E('noupd') == '' else False)
        def _():
            lane = lax.broadcasted_iota(I32, (1, TQ), 1)
            for t in range(2):
                idx = idx_s[t]
                y = jnp.sum(ypart_s[t], axis=1, keepdims=True) * sig_s[t:t + 1, :]
                blk = pl.ds(pl.multiple_of(idx // TQ * TQ, TQ), TQ)
                old = acc[:, blk]
                acc[:, blk] = jnp.where(
                    lane == idx % TQ, old + (1.0 - g_s[:, blk]) * y, old)

        head(h, _loop_order())
        return carry

    if ONLY != 'first':
        lax.fori_loop(1, H, step, 0)
        for i in range(NPB):
            for c0, c1 in out_blocks(i):
                cp_out(c0, c1).wait()
    else:
        for c in bulk:
            c.wait()
        k = idx_s[0] & 7
        r = pl.ds(pl.multiple_of((idx_s[1] & 63) * 8, 8), 8)
        out_s[0:16, 0:PR] = _bf(xsum_s[jnp.minimum(k, 6), r, :]) + xcol_s[0, 0:16, 0:1].astype(BF) + \
            acc[pl.ds(pl.multiple_of(k * 16, 16), 16), 0:PR].astype(BF) + ypart_s[1, 0:16, 0:1].astype(BF)
        cp_out(0, PB).start()
        cp_out(0, PB).wait()


@jax.jit
def pallas_gated_mix__compressed_kv_cla__moe_arch_mod__prompt_kernel(
    A_x: jax.Array,
    A_c_kv: jax.Array,
    A_w_q: jax.Array,
    A_w_uk: jax.Array,
    A_w_uv: jax.Array,
    A_w_o: jax.Array,
    B_x: jax.Array,
    B_w_r: jax.Array,
    B_w_gate: jax.Array,
    B_w_up: jax.Array,
    B_w_down: jax.Array,
    gate_w: jax.Array,
):
    del B_x
    xT = A_x.reshape(S, M).T
    ckv = A_c_kv.reshape(S, C)
    woT = jnp.transpose(A_w_o, (0, 2, 1))
    wdT = B_w_down.T

    V = pltpu.VMEM
    scratch = [
        V((M // 2, S), U32),
        V((S // 2, M), U32),
        V((S // 2, C), U32),
        V((H // 2, M, D), U32),
        V((2, H // 2, C, D), U32),
        V((H, M // 2, D), U32),
        V((S // 2, D), U32),
        V((2, S // 2, D), U32),
        V((S // 2, D), U32),
        V((M, S), F32),
        V((1, S), F32),
        V((1, S), F32),
        V((M,), BF),
        V((M,), BF),
        V((M // 2, F), U32),
        V((M // 2, F), U32),
        V((M // 2, F), U32),
        V((8, TQ), F32),
        pltpu.SMEM((2,), I32),
        V((2, M, TQ), F32),
        V((2, M, TQ), F32),
        V((5, S // 4, HC), U32),
        V((7, S // 4, PR), U32),
        V((7, S // 4, TQ), U32),
        V((7, S // 4, TQ), U32),
        V((7, S // 4, TQ), U32),
        V((7, S // 4, TQ), U32),
        V((M, S), BF),
        pltpu.SemaphoreType.DMA((NSEM,)),
    ]
    outT = pl.pallas_call(
        _kernel,
        in_specs=[pl.BlockSpec(memory_space=pl.ANY)] * 11,
        out_specs=pl.BlockSpec(memory_space=pl.ANY),
        out_shape=jax.ShapeDtypeStruct((M, S), BF),
        scratch_shapes=scratch,
        compiler_params=pltpu.CompilerParams(
            vmem_limit_bytes=100 * 1024 * 1024,
            disable_bounds_checks=E('nochk') != '', disable_semaphore_checks=E('nochk') != ''),
    )(xT, ckv, A_w_q, A_w_uk, A_w_uv, woT, B_w_r, B_w_gate, B_w_up, wdT, gate_w)
    return outT.T.reshape(1, S, M)
```

```python
import math
import re
_CFG = {'loop': 'K0.4,K0.2,Q0,K0,V0,SD1,SB0,SS1,SA0,K1,V1.4,FV0,V1,PA0,Q1,SD2,SS2,PA1,PB1,K2.2,PB0,SD3,PD2,K2.2,V2.1,K2,SS3,V2.4,PS2,V2,Q2.3,O0,Q2,SS4.1,SS4,SS5.1,SS5.1,K3.1,SS5,SD4,PS3,SD5,K3.5,K3,PD3,PS4,PD4,Q3,SS6.4,PS5.5,V3,PS5.1,SS6,O1,PD5,SD6,SS7,PS6,PS5,PD6,SD7,O2,PS7.4,PS7.2,PD7,PS7,O3', 'oP': '2014653', 'oO': '0341625', 'oV': '4150623', 'oK': '1403625', 'oS': '0136425', 'qkc': '1', 'oQ': '2546301', 'hyb': '14', 'pform': '1', 'raw': '1', 'lsrc': '2', 'pl': '1', 'sto': '2', 'oc': '2', 'first': 'T0,T1,T2,GB0,GB1,Q0.1,T3,Q0,SB0,SA1,SA0,Q1,SB1,G8,PB0,PA0,SA2,PB1,G9,SB2,G10,PA1,G11,SD3,SS3,G12,PA2,O0,Q2,PB2,G13,G14,SS5.4,SD4,PB3,G15,SS4,PA3,SS5,PB4,O1,Q3,SD5,SS6.4,TOPK0,SS6,SD6,PD5,PA4,PS5,SA7,SB7,PA6,PB6,PA7,O2,PB7,O3', 'flsrc': '2', 'fQ': '3614025', 'fO': '4032615', 'fsto': '1', 'fhyb': '14', 'fP': '2014563'}


def E(k, d=''):
    return _CFG.get(k, d)

import jax
import jax.numpy as jnp
from jax import lax
import jax.experimental.pallas as pl
import jax.experimental.pallas.tpu as pltpu

S, M, C, H, D, F = 2048, 448, 1024, 16, 256, 1792
TQ = 128
NQ = S // TQ
PR = 2 * TQ
NP = S // PR
PB = 512
NPB = S // PB
NF = F // TQ
HB, HC, HM = PB // 2, C // 2, M // 2
MP = 512

BF, F32, U32, I32 = jnp.bfloat16, jnp.float32, jnp.uint32, jnp.int32
NN = (((1,), (0,)), ((), ()))
NT = (((1,), (1,)), ((), ()))
LOG2E = math.log2(math.e)
QSCALE = (D ** -0.5) * LOG2E
NEG = -1e9 * LOG2E
HI16 = 0xFFFF0000

S_WK, S_WV, S_HEAD0, S_HEAD1, S_BULK, S_OUT, S_CKV = range(7)
NSEM = S_CKV + NPB

HYB_ = int(E('hyb', 14))
STQ = int(E('stq', 1))
QK0 = int(E('qk0', 99))
PV0 = int(E('pv0', 1))
STO_ = int(E('sto', 0))
LSRC_ = int(E('lsrc', 2))
QKC = int(E('qkc', 1))
OC = int(E('oc', 1))
ORD = {k: [int(c) for c in E('o' + k, d)] for k, d in
       (('K', '3104625'), ('V', '3104625'), ('Q', '3104625'), ('S', '3104625'),
        ('P', '2304156'), ('O', '0346125'))}
FORD = {k: [int(c) for c in E('f' + k, d)] for k, d in
        (('Q', '2310456'), ('S', '0136425'), ('P', '2014653'), ('O', '0341625'))}
ONLY = E('only')
RAW = int(E('raw', 1))
PFORM = int(E('pform', 0))
PL = int(E('pl', 1))
TVAL = int(E('tval', 0))
ASJ = int(E('asj', 1))
FQ = int(E('fq', 1))
FST = int(E('fst', 1))


def _parse(txt):
    out = []
    for t in txt.split(','):
        m = re.match(r'([A-Z]+)(\d+)(?:\.(\d))?$', t)
        out.append((m.group(1), int(m.group(2)), int(m.group(3) or 0)))
    return out


def _dot(a, b, dn):
    return lax.dot_general(a, b, dn, preferred_element_type=F32)


def _cat(xs, axis):
    return xs[0] if len(xs) == 1 else jnp.concatenate(xs, axis=axis)


def _recip(l):
    r = pl.reciprocal(l, approx=True)
    return r * (2.0 - l * r)


def _sigmoid(z):
    return 1.0 / (1.0 + jnp.exp(-z))


def _bf(w):
    return pltpu.bitcast(w, BF)


def _u32(v):
    return pltpu.bitcast(v.astype(BF), U32)


def _rows(ref, r0, r1):
    return _bf(ref[r0 // 2:r1 // 2, :])


def _put_rows(ref, r0, r1, v):
    ref[r0 // 2:r1 // 2, :] = _u32(v)


def _lhs_terms(a11, a12, a21, a22):
    return [a11 + a22, a21 + a22, a11, a22, a11 + a12, a21 - a11, a12 - a22]


def _rhs_terms(b11, b12, b21, b22):
    return [b11 + b22, b11, b12 - b22, b21 - b11, b22, b11 + b12, b21 + b22]


def _quads(f):
    k, n = f.shape[0] // 2, f.shape[1] // 2
    return f[:k, :n], f[:k, n:], f[k:, :n], f[k:, n:]


def _combine(m):
    return (m[0] + m[3] - m[4] + m[6], m[2] + m[4],
            m[1] + m[3], m[0] - m[1] + m[2] + m[5])


SUMS = (0, 1, 4, 5, 6)


def _att(i, st):
    qk = [("SS", i, 0), ("SD", i, 0)] if st and i >= max(QK0, 1) else [("SA", i, 0), ("SB", i, 0)]
    pv = [("PS", i, 0), ("PD", i, 0)] if st and i >= max(PV0, 1) else [("PA", i, 0), ("PB", i, 0)]
    return qk, pv


def _order(st, proj):
    q = lambda b: [("Q", b, 0)]
    kv = lambda b: [("K", b, 0), ("V", b, 0)] if proj else []
    t = q(0) + kv(0) + _att(0, st)[0] + _att(1, st)[0] + kv(1) + _att(0, st)[1] + q(1)
    for i in range(1, NP + 1):
        if i + 1 < NP:
            if i % 2 == 1 and i > 1:
                t += kv((i + 1) // 2) + q((i + 1) // 2)
            t += _att(i + 1, st)[0]
        if i < NP:
            t += _att(i, st)[1]
        if i % 2 == 0:
            t.append(("O", i // 2 - 1, 0))
    return t


def _first_order():
    if E('first'):
        return _parse(E('first'))
    out = [("T", b, 0) for b in range(NPB)] + [("GB", 0, 0), ("GB", 1, 0)]
    g = 8
    for e in _order(bool(FST), False):
        out.append(e)
        if ("Q", 1, 0) in out and g < NQ and e[0] in ("Q", "SA", "SB", "SS", "SD"):
            out.append(("G", g, 0))
            g += 1
        if e == ("O", 1, 0):
            out.append(("TOPK", 0, 0))
    if FQ:
        pass
    elif STQ and E('xp', '0') == '0':
        out += [("XS", b, 0) for b in range(NPB)]
    elif STQ:
        k, res = 0, []
        for e in out:
            res.append(e)
            if e[0] in ("SA", "SB") and e[1] >= int(E('xp0', 0)) and k < 16:
                res.append(("XP", k, 0))
                k += 1
        out = res + [("XP", j, 0) for j in range(k, 16)]
    return out


def _loop_order():
    if E('loop'):
        return _parse(E('loop'))
    out = []
    for e in _order(True, True):
        out.append(e)
        if e == ("V", 0, 0):
            out.append(("FV", 0, 0))
    return out


def _kernel(xT_hbm, ckv_hbm, wq_hbm, wk_hbm, wv_hbm, wo_hbm, wr_hbm, wg_hbm,
            wu_hbm, wd_hbm, gw_hbm, out_hbm,
            xT_s, x_s, ckv_s, wq32, wkv32, wo_s, q_s, kv_s, ctx_s, acc,
            r_s, g_s, wr_s, gw_s, wg_s, wu_s, wd_s, sig_s, idx_s, xcol_s, ypart_s,
            asum_s, xsum_s, qt_s, kt_s, vt_s, ct_s, out_s, sem):
    wk32, wv32 = wkv32.at[0], wkv32.at[1]
    k_s, v_s = kv_s.at[0], kv_s.at[1]
    (xT_u, ckv_u, wq_u, wk_u, wv_u, wo_u, wg_u, wu_u, wd_u) = (
        r.bitcast(U32) for r in (xT_hbm, ckv_hbm, wq_hbm, wk_hbm, wv_hbm,
                                 wo_hbm, wg_hbm, wu_hbm, wd_hbm))

    def cp(src, dst, s):
        return pltpu.make_async_copy(src, dst, sem.at[s])

    def cp_pair(w_u, w_s, p, s):
        return cp(w_u.at[:, p, :], w_s.at[p], s)

    def cp_ckv(i):
        r = pl.ds(pl.multiple_of(PB // 2 * i, PB // 2), PB // 2)
        return cp(ckv_u.at[r, :], ckv_s.at[r, :], S_CKV + i)

    def cp_out(c0, c1):
        r = pl.ds(c0, c1 - c0)
        return cp(out_s.at[:, r], out_hbm.at[:, r], S_OUT)

    def out_blocks(i):
        r0, r1 = PB * i, PB * (i + 1)
        return [(r0, r1)] if i < NPB - 1 else [(r0, r0 + PR), (r0 + PR, r1)]

    c_wk, c_wv = cp_pair(wk_u, wk32, 0, S_WK), cp_pair(wv_u, wv32, 0, S_WV)
    head0 = [cp(xT_u, xT_s, S_HEAD0), cp_pair(wq_u, wq32, 0, S_HEAD0),
             cp(wr_hbm, wr_s, S_HEAD0), cp(gw_hbm, gw_s, S_HEAD0),
             cp(wo_u.at[0], wo_s.at[0], S_HEAD0)]
    head1 = [cp(wo_u.at[1], wo_s.at[1], S_HEAD1), cp(wg_u, wg_s, S_HEAD1),
             cp(wu_u, wu_s, S_HEAD1), cp(wd_u, wd_s, S_HEAD1)]
    rest = pl.ds(2, H - 2)
    bulk = [cp(wo_u.at[rest], wo_s.at[rest], S_BULK)]
    for p in range(1, H // 2):
        bulk += [cp_pair(wk_u, wk32, p, S_BULK), cp_pair(wv_u, wv32, p, S_BULK),
                 cp_pair(wq_u, wq32, p, S_BULK)]

    row = lax.broadcasted_iota(I32, (TQ, TQ), 0)
    col = lax.broadcasted_iota(I32, (TQ, TQ), 1)
    tri = col <= row

    W = TQ // 2

    def term(ref, n, j0, j1):
        raw = RAW and {id(qt_s): (q_s, 2, 3), id(kt_s): (k_s, 1, 4),
                       id(vt_s): (v_s, 1, 4)}.get(id(ref))
        if raw and n in raw[1:]:
            odd = int(n == raw[2])
            return _bf(_cat([raw[0][W * (2 * j + odd):W * (2 * j + odd + 1),
                                    TQ * odd:TQ * (odd + 1)]
                             for j in range(j0, j1)], 0))
        if mode["first"] and (ref is kt_s or ref is vt_s):
            for j in range(j0, j1):
                if (id(ref), n, j) not in held:
                    f = _rows(k_s if ref is kt_s else v_s, PR * j, PR * (j + 1)).astype(F32)
                    q11, q12, q21, q22 = _quads(f)
                    tt = _rhs_terms(q11, q21, q12, q22) if ref is kt_s else \
                        _rhs_terms(q11, q12, q21, q22)
                    for u in (0, 2, 3, 5, 6):
                        held[id(ref), u, j] = tt[u].astype(BF)
        if (id(ref), n, j0) in held:
            return _cat([held[id(ref), n, j] for j in range(j0, j1)], 0)
        return _bf(ref[n, W * j0:W * j1, :])

    held, mode = {}, {}

    def put_terms(ref, j, terms):
        skip = () if not RAW or ref is ct_s else (2, 3) if ref is qt_s else (1, 4)
        bit = {id(ct_s): 1, id(kt_s): 2, id(qt_s): 4, id(vt_s): 8}[id(ref)]
        for n, t in enumerate(terms):
            if n in skip:
                continue
            if TVAL & bit:
                held[id(ref), n, j] = t.astype(BF)
            else:
                ref[n, W * j:W * (j + 1), :] = _u32(t)

    def head(h, order, first=False):
        if isinstance(h, int):
            pair, shift = h // 2, jnp.uint32(16 * (1 - h % 2))
        else:
            pair = lax.shift_right_logical(h, 1)
            shift = (16 - 16 * (h & 1)).astype(U32)
        kinds = {(k, i) for k, i, _ in order}
        held.clear()
        mode["first"] = first
        STO = int(E('fsto', 0)) if first else STO_
        HYB = int(E('fhyb', 14)) if first else HYB_
        LSRC = int(E('flsrc', 2)) if first else LSRC_
        cache, prog = {}, {}

        def weight32(ref):
            return pltpu.bitcast((ref[pair] << shift) & jnp.uint32(HI16), F32)

        def wterms(name):
            if name not in cache:
                if name == "O":
                    f = _bf(wo_s[h]).astype(F32)
                    cache[name] = [t.astype(BF) for t in _lhs_terms(*_quads(f))]
                else:
                    f = weight32({"K": wk32, "V": wv32, "Q": wq32}[name])
                    if name == "Q":
                        f = jnp.concatenate([f, jnp.zeros((MP - M, D), F32)], axis=0)
                    cache[name] = [t.astype(BF) for t in _rhs_terms(*_quads(f))]
            return cache[name]

        def run(key, cnt, product):
            m = prog.setdefault(key, {})
            todo = [n for n in (FORD if first else ORD)[key[0]] if n not in m]
            for n in (todo[:cnt] if cnt else todo):
                m[n] = product(n)
            return len(m) == 7

        def route(c0, c1):
            if "rg" not in cache:
                r16 = lax.broadcasted_iota(I32, (16, M), 0)
                wr = wr_s[...].astype(F32).reshape(1, M)
                gw = gw_s[...].astype(F32).reshape(1, M)
                cache["rg"] = jnp.where(
                    r16 == 0, wr, jnp.where(r16 == 1, gw, 0.0)).astype(BF)
            rg = _dot(cache["rg"], _bf(xT_s[:, c0:c1]), NN)
            r_s[:, c0:c1] = rg[0:1, :].astype(BF).astype(F32)
            g_s[:, c0:c1] = _sigmoid(rg[1:2, :])

        st, pp, ov, rinv = {}, {}, {}, {}
        last = {}

        def anchor():
            u = pltpu.bitcast(last["v"][0:8, 0:TQ], I32)[0, 0]
            return lax.shift_right_logical(lax.shift_right_logical(u, 31), 1)

        def set_scores(q, s0, s):
            last["v"] = s
            for t in range(s.shape[1] // TQ):
                blk = s[:, TQ * t:TQ * (t + 1)]
                st.setdefault(q, {})[s0 + t] = jnp.where(tri, blk, NEG) if s0 + t == q else blk

        def probs(q, perm):
            if q not in pp:
                tiles = st.pop(q)
                s = _cat([tiles[t] for t in perm], 1)
                p = jnp.exp2(s - jnp.max(s, axis=1, keepdims=True))
                pp[q] = (p, p.astype(BF))
            return pp[q]

        def finish(q, o, src):
            if q < HYB:
                rinv[q] = None
                return o * _recip(jnp.sum(src, axis=1, keepdims=True))
            la = src[:, 0:TQ]
            for t in range(1, src.shape[1] // TQ):
                la = la + src[:, TQ * t:TQ * (t + 1)]
            hi = la.astype(BF)
            lo = (la - hi.astype(F32)).astype(BF)
            l = _dot(jnp.ones((16, 2 * TQ), BF),
                     jnp.concatenate([hi, lo], axis=1), NT)[0:1, :]
            rinv[q] = _recip(l)
            return o

        def store_ctx(q, o):
            last["v"] = o
            i = q // 2
            if i // 2 < STO and 2 * i + 1 < HYB:
                ov[q] = o
                if 2 * i in ov and 2 * i + 1 in ov:
                    oa, ob = ov.pop(2 * i), ov.pop(2 * i + 1)
                    put_terms(ct_s, i, _rhs_terms(oa[:, :TQ], ob[:, :TQ],
                                                  oa[:, TQ:], ob[:, TQ:]))
            else:
                _put_rows(ctx_s, TQ * q, TQ * (q + 1), o)

        def pv_done(i):
            if ("PS", i) in prog.get("done", ()) and ("PD", i) in prog.get("done", ()):
                c11, c12, c21, c22 = _combine(prog.pop(("P", i)))
                da, db = prog.pop(("PDv", i))
                lt = prog.pop(("L", i))
                w = TQ * i
                lf, dg = prog.pop(("Lf", i)), prog.pop(("D", i))
                for q, o, ln in ((2 * i, jnp.concatenate([c11, c12], axis=1) + da, 4),
                                 (2 * i + 1, jnp.concatenate([c21, c22], axis=1) + db, 1)):
                    pf, pb = pp.pop(q)
                    if LSRC == 3:
                        src = jnp.concatenate([lf[ln], pf[:, 2 * w:]], axis=1)
                    elif LSRC == 2:
                        src = jnp.concatenate([lt[ln], dg[q % 2]], axis=1).astype(F32)
                    elif LSRC == 1:
                        src = pb.astype(F32)
                    else:
                        src = pf
                    store_ctx(q, finish(q, o, src))

        for kind, i, cnt in order:
            r0, r1 = PB * i, PB * (i + 1)
            n0 = PR * i
            qa, qb = 2 * i, 2 * i + 1
            eo = [2 * j for j in range(i)] + [2 * j + 1 for j in range(i)]
            if kind == "T":
                _put_rows(x_s, r0, r1, _bf(xT_s[:, r0:r1]).T)
            elif kind == "XS":
                for j in range(0, HB, 16):
                    z = jnp.zeros((16, MP - M), F32)
                    at = jnp.concatenate([_rows(x_s, r0 + j, r0 + j + 16).astype(F32), z], axis=1)
                    ab = jnp.concatenate([_rows(x_s, r0 + HB + j, r0 + HB + j + 16).astype(F32), z], axis=1)
                    tt = _lhs_terms(at[:, :PR], at[:, PR:], ab[:, :PR], ab[:, PR:])
                    for n in range(7):
                        if n != 2:
                            xsum_s[n, (HB * i + j) // 2:(HB * i + j) // 2 + 8, :] = _u32(tt[n])
            elif kind == "XP":
                blk, part = i // 4, i % 4
                z0 = anchor() * 8
                for j in range(64 * part, 64 * part + 64, 16):
                    z = jnp.zeros((16, MP - M), F32)
                    ld = lambda r: jnp.concatenate([_bf(x_s[pl.ds(pl.multiple_of(
                        jnp.minimum(r // 2 + z0, S // 2 - 8), 8), 8), :]).astype(F32), z], axis=1)
                    at, ab = ld(PB * blk + j), ld(PB * blk + HB + j)
                    tt = _lhs_terms(at[:, :PR], at[:, PR:], ab[:, :PR], ab[:, PR:])
                    d0 = (HB * blk + j) // 2
                    for n in range(7):
                        if n != 2:
                            xsum_s[n, d0:d0 + 8, :] = _u32(tt[n])
            elif kind == "GB":
                route(r0, r1)
            elif kind == "G":
                route(TQ * i, TQ * (i + 1))
            elif kind in ("K", "V", "Q"):
                w0, w1 = HB * i // 2, HB * (i + 1) // 2
                if kind == "Q" and first and FQ and ("xt", i) not in cache:
                    z = jnp.zeros((HB, MP - M), F32)
                    at = jnp.concatenate([_rows(x_s, r0, r0 + HB).astype(F32), z], axis=1)
                    ab = jnp.concatenate([_rows(x_s, r0 + HB, r1).astype(F32), z], axis=1)
                    tt = _lhs_terms(at[:, :PR], at[:, PR:], ab[:, :PR], ab[:, PR:])
                    cache["xt", i] = {n: tt[n].astype(BF) for n in range(7) if n != 2}
                    for n, v in cache["xt", i].items():
                        xsum_s[n, w0:w1, :] = pltpu.bitcast(v, U32)
                if kind == "Q" and ((first and not FQ) or not STQ):
                    if "q" not in cache:
                        cache["q"] = weight32(wq32).astype(BF)
                    res = _quads(_dot(_rows(x_s, r0, r1), cache["q"], NN))
                else:
                    def lhs(n):
                        if kind == "Q":
                            if n == 2:
                                return _bf(x_s[r0 // 2:(r0 + HB) // 2, :PR])
                            if first:
                                return cache["xt", i][n]
                            return _bf(xsum_s[n, w0:w1, :])
                        if n == 2:
                            return _bf(ckv_s[r0 // 2:(r0 + HB) // 2, :HC])
                        if n == 3:
                            return _bf(ckv_s[(r0 + HB) // 2:r1 // 2, HC:])
                        return _bf(asum_s[SUMS.index(n), w0:w1, :])
                    if not run((kind, i), cnt, lambda n: _dot(lhs(n), wterms(kind)[n], NN)):
                        continue
                    res = _combine(prog.pop((kind, i)))
                if kind == "Q":
                    res = [c * QSCALE for c in res]
                dst = {"K": k_s, "V": v_s, "Q": q_s}[kind]
                for j, (c0, c1) in ((2 * i, res[:2]), (2 * i + 1, res[2:])):
                    _put_rows(dst, PR * j, PR * (j + 1), jnp.concatenate([c0, c1], axis=1))
                    if kind == "V" and any(("PS", u) in kinds for u in range(j + 1, NP)):
                        put_terms(vt_s, j, _rhs_terms(c0[:TQ], c1[:TQ], c0[TQ:], c1[TQ:]))
                    if kind == "K" and any(("SS", u) in kinds for u in range(j + 1, NP)):
                        put_terms(kt_s, j, _rhs_terms(c0[:TQ], c0[TQ:], c1[:TQ], c1[TQ:]))
                    if kind == "Q" and ("SS", j) in kinds:
                        put_terms(qt_s, j, _lhs_terms(c0[:TQ], c1[:TQ], c0[TQ:], c1[TQ:]))
            elif kind in ("SA", "SB"):
                q = qa if kind == "SA" else qb
                set_scores(q, 0, _dot(_rows(q_s, TQ * q, TQ * (q + 1)),
                                      _rows(k_s, 0, TQ * (q + 1)), NT))
            elif kind == "SD":
                for q in (qa, qb):
                    set_scores(q, qa, _dot(_rows(q_s, TQ * q, TQ * (q + 1)),
                                           _rows(k_s, n0, TQ * (q + 1)), NT))
            elif kind == "SS":
                qts = [term(qt_s, n, i, i + 1) for n in range(7)]
                done = prog.setdefault(("SSj", i), [0])
                j_end = min(i, done[0] + cnt) if cnt else i
                for j0 in range(done[0], j_end, QKC):
                    j1 = min(j_end, j0 + QKC)
                    cs = _combine({n: _dot(qts[n], term(kt_s, n, j0, j1), NT)
                                   for n in (FORD if first else ORD)["S"]})
                    for j in range(j0, j1):
                        sl = slice(TQ * (j - j0), TQ * (j - j0 + 1))
                        st.setdefault(qa, {})[2 * j] = cs[0][:, sl]
                        st[qa][2 * j + 1] = cs[1][:, sl]
                        st.setdefault(qb, {})[2 * j] = cs[2][:, sl]
                        st[qb][2 * j + 1] = cs[3][:, sl]
                done[0] = j_end
            elif kind in ("PA", "PB"):
                q = qa if kind == "PA" else qb
                pf, pb = probs(q, range(q + 1))
                pp.pop(q)
                o = _dot(pb, _rows(v_s, 0, TQ * (q + 1)), NN)
                store_ctx(q, finish(q, o, pb.astype(F32) if LSRC in (1, 2) or (LSRC == 3 and PL) else pf))
            elif kind in ("PS", "PD"):
                w = TQ * i
                (paf, pab), (pbf, pbb) = probs(qa, eo + [qa]), probs(qb, eo + [qa, qb])
                if ("D", i) not in prog:
                    prog["D", i] = ((paf[:, 2 * w:].astype(BF), pbf[:, 2 * w:].astype(BF))
                                    if PFORM else (pab[:, 2 * w:], pbb[:, 2 * w:]))
                if kind == "PD":
                    prog["PDv", i] = (_dot(prog["D", i][0], _rows(v_s, n0, n0 + TQ), NN),
                                      _dot(prog["D", i][1], _rows(v_s, n0, n0 + PR), NN))
                else:
                    if ("L", i) not in prog:
                        lf = _lhs_terms(paf[:, :w], paf[:, w:2 * w],
                                        pbf[:, :w], pbf[:, w:2 * w])
                        lt = [t.astype(BF) for t in lf]
                        if not PFORM:
                            lt[2], lt[3] = pab[:, :w], pbb[:, w:2 * w]
                        prog["L", i], prog["Lf", i] = lt, lf
                    def pprod(n):
                        l_ = prog["L", i][n]
                        if not TVAL & 16:
                            return _dot(l_, term(vt_s, n, 0, i), NN)
                        parts = [_dot(l_[:, TQ * j:TQ * (j + 1)], term(vt_s, n, j, j + 1), NN)
                                 for j in range(i)]
                        tot = parts[0]
                        for x in parts[1:]:
                            tot = tot + x
                        return tot
                    if not run(("P", i), cnt, pprod):
                        continue
                prog.setdefault("done", set()).add((kind, i))
                pv_done(i)
            elif kind == "O":
                j0, j1 = 2 * i, 2 * i + 2
                js = max(j0, min(j1, HYB // 2)) if i < STO else j0
                cols = []
                for j in range(j0, js, OC):
                    je = min(js, j + OC)
                    c11, c12, c21, c22 = _combine(
                        {n: _dot(wterms("O")[n], term(ct_s, n, j, je), NT) for n in (FORD if first else ORD)["O"]})
                    ca = jnp.concatenate([c11, c21], axis=0)
                    cb = jnp.concatenate([c12, c22], axis=0)
                    for t in range(je - j):
                        cols += [ca[:, TQ * t:TQ * (t + 1)], cb[:, TQ * t:TQ * (t + 1)]]
                if j1 > js:
                    cols.append(_dot(_bf(wo_s[h]), _rows(ctx_s, PR * js, PR * j1), NT))
                g = g_s[:, r0:r1]
                f = []
                for t in range(4):
                    gt, rt = g[:, TQ * t:TQ * (t + 1)], rinv.pop(4 * i + t)
                    f.append(gt if rt is None else gt * rt)
                a = _cat(cols, 1) * jnp.concatenate(f, axis=1)
                if first:
                    acc[:, r0:r1] = a + (1.0 - g) * _bf(xT_s[:, r0:r1]).astype(F32)
                else:
                    a = acc[:, r0:r1] + a
                    acc[:, r0:r1] = a
                    for c0, c1 in out_blocks(i):
                        out_s[:, c0:c1] = a[:, c0 - r0:c1 - r0].astype(BF)

                        @pl.when(h == H - 1)
                        def _():
                            cp_out(c0, c1).start()
            elif kind == "TOPK":
                r = r_s[...]
                lane = lax.broadcasted_iota(I32, (1, S), 1)
                m1 = jnp.max(r, axis=1, keepdims=True)
                i1 = jnp.min(jnp.where(r == m1, lane, S - 1))
                r2 = jnp.where(lane == i1, -jnp.inf, r)
                m2 = jnp.max(r2, axis=1, keepdims=True)
                i2 = jnp.min(jnp.where((r2 == m2) & (lane != i1), lane, S - 1))
                r8 = lax.broadcasted_iota(I32, (8, TQ), 0)
                sig_s[...] = jnp.where(r8 == 0, _sigmoid(m1), _sigmoid(m2))
                lane = lax.broadcasted_iota(I32, (1, TQ), 1)
                for t, idx in enumerate((i1, i2)):
                    idx_s[t] = idx
                    blk = pl.ds(pl.multiple_of(idx // TQ * TQ, TQ), TQ)
                    xb = _bf(xT_s[:, blk]).astype(F32)
                    xc = jnp.sum(jnp.where(lane == idx % TQ, xb, 0.0),
                                 axis=1, keepdims=True)
                    xcol_s[t] = jnp.broadcast_to(xc, (M, TQ))
                ypart_s[...] = jnp.zeros_like(ypart_s)
            elif kind == "FV":
                chunk = jnp.minimum(h - 1, NF - 1)
                c = pl.ds(pl.multiple_of(chunk * TQ, TQ), TQ)
                wg, wu, wd = (_bf(w[:, c]).astype(F32) for w in (wg_s, wu_s, wd_s))
                for t in range(2):
                    xc = xcol_s[t]
                    g = jnp.sum(xc * wg, axis=0, keepdims=True)
                    u = jnp.sum(xc * wu, axis=0, keepdims=True)
                    ypart_s[t] += wd * (g * _sigmoid(g) * u)
            elif kind in ("FG", "FU", "FD"):
                if "fc" not in cache:
                    chunk = jnp.minimum(h - 1, NF - 1)
                    cache["fc"] = pl.ds(pl.multiple_of(chunk * TQ, TQ), TQ)
                w = _bf({"FG": wg_s, "FU": wu_s, "FD": wd_s}[kind][:, cache["fc"]])
                w = w.astype(F32)
                if kind != "FD":
                    cache[kind] = [jnp.sum(xcol_s[t] * w, axis=0, keepdims=True)
                                   for t in range(2)]
                else:
                    for t in range(2):
                        g, u = cache["FG"][t], cache["FU"][t]
                        ypart_s[t] += w * (g * _sigmoid(g) * u)
            else:
                raise ValueError(kind)
        assert not st and not pp and not rinv and not ov, (st.keys(), pp.keys(), rinv.keys())

    for c in [cp_ckv(0), c_wk, c_wv] + [cp_ckv(i) for i in range(1, NPB)]:
        c.start()
    for c in head0 + head1 + bulk:
        c.start()

    def proj0(t, carry):
        which, blk = t % 2, t // 2
        base = pl.multiple_of(blk * (PB // 2), PB // 2)
        half = pl.multiple_of(blk * (HB // 2), HB // 2)

        @pl.when(which == 0)
        def _():
            cp_ckv(blk).wait()
            for j in range(0, HB // 2 if ASJ == 0 else 0, 8):
                at = _bf(ckv_s[pl.ds(base + j, 8), :]).astype(F32)
                ab = _bf(ckv_s[pl.ds(base + HB // 2 + j, 8), :]).astype(F32)
                tt = _lhs_terms(at[:, :HC], at[:, HC:], ab[:, :HC], ab[:, HC:])
                for k, n in enumerate(SUMS):
                    asum_s[k, pl.ds(half + j, 8), :] = _u32(tt[n])

        @pl.when(t == 0)
        def _():
            c_wk.wait()

        @pl.when(t == 1)
        def _():
            c_wv.wait()

        top, bot = pl.ds(base, HB // 2), pl.ds(base + HB // 2, HB // 2)
        if ASJ == 0:
            lhs = {n: _bf(asum_s[k, pl.ds(half, HB // 2), :]) for k, n in enumerate(SUMS)}
        else:
            at, ab = _bf(ckv_s[top, :]).astype(F32), _bf(ckv_s[bot, :]).astype(F32)
            tt = _lhs_terms(at[:, :HC], at[:, HC:], ab[:, :HC], ab[:, HC:])
            lhs = {n: tt[n].astype(BF) for n in SUMS}
            for k, n in enumerate(SUMS):
                asum_s[k, pl.ds(half, HB // 2), :] = pltpu.bitcast(lhs[n], U32)
        lhs[2], lhs[3] = _bf(ckv_s[top, :HC]), _bf(ckv_s[bot, HC:])
        f = pltpu.bitcast(wkv32[which, 0] << 16, F32)
        rhs = [t_.astype(BF) for t_ in _rhs_terms(*_quads(f))]
        c11, c12, c21, c22 = _combine({n: _dot(lhs[n], rhs[n], NN) for n in [int(c) for c in E("o0", "3614025")]})
        kv_s[which, top, :] = _u32(jnp.concatenate([c11, c12], axis=1))
        kv_s[which, bot, :] = _u32(jnp.concatenate([c21, c22], axis=1))
        return carry

    lax.fori_loop(0, 2 * NPB, proj0, 0)
    for c in head0:
        c.wait()
    if ONLY not in ('loop', 'proj0'):
        head(0, _first_order(), first=True)
    for c in head1:
        c.wait()

    def step(h, carry):
        @pl.when(h == 2)
        def _():
            for c in bulk:
                c.wait()

        @pl.when((h == H - 1) if E('noupd') == '' else False)
        def _():
            lane = lax.broadcasted_iota(I32, (1, TQ), 1)
            for t in range(2):
                idx = idx_s[t]
                y = jnp.sum(ypart_s[t], axis=1, keepdims=True) * sig_s[t:t + 1, :]
                blk = pl.ds(pl.multiple_of(idx // TQ * TQ, TQ), TQ)
                old = acc[:, blk]
                acc[:, blk] = jnp.where(
                    lane == idx % TQ, old + (1.0 - g_s[:, blk]) * y, old)

        head(h, _loop_order())
        return carry

    if ONLY == 'proj0':
        for c in bulk:
            c.wait()
        r = pl.ds(pl.multiple_of((idx_s[1] & 63) * 8, 8), 8)
        out_s[0:16, 0:PR] = _bf(asum_s[idx_s[0] & 3, r, 0:PR]) + _bf(kv_s[idx_s[0] & 1, r, :])
        cp_out(0, PB).start()
        cp_out(0, PB).wait()
    elif ONLY != 'first':
        lax.fori_loop(1, H, step, 0)
        for i in range(NPB):
            for c0, c1 in out_blocks(i):
                cp_out(c0, c1).wait()
    else:
        for c in bulk:
            c.wait()
        k = idx_s[0] & 7
        r = pl.ds(pl.multiple_of((idx_s[1] & 63) * 8, 8), 8)
        out_s[0:16, 0:PR] = _bf(xsum_s[jnp.minimum(k, 6), r, :]) + xcol_s[0, 0:16, 0:1].astype(BF) + \
            acc[pl.ds(pl.multiple_of(k * 16, 16), 16), 0:PR].astype(BF) + ypart_s[1, 0:16, 0:1].astype(BF)
        cp_out(0, PB).start()
        cp_out(0, PB).wait()


@jax.jit
def pallas_gated_mix__compressed_kv_cla__moe_arch_mod__prompt_kernel(
    A_x: jax.Array,
    A_c_kv: jax.Array,
    A_w_q: jax.Array,
    A_w_uk: jax.Array,
    A_w_uv: jax.Array,
    A_w_o: jax.Array,
    B_x: jax.Array,
    B_w_r: jax.Array,
    B_w_gate: jax.Array,
    B_w_up: jax.Array,
    B_w_down: jax.Array,
    gate_w: jax.Array,
):
    del B_x
    xT = A_x.reshape(S, M).T
    ckv = A_c_kv.reshape(S, C)
    woT = jnp.transpose(A_w_o, (0, 2, 1))
    wdT = B_w_down.T

    V = pltpu.VMEM
    scratch = [
        V((M // 2, S), U32),
        V((S // 2, M), U32),
        V((S // 2, C), U32),
        V((H // 2, M, D), U32),
        V((2, H // 2, C, D), U32),
        V((H, M // 2, D), U32),
        V((S // 2, D), U32),
        V((2, S // 2, D), U32),
        V((S // 2, D), U32),
        V((M, S), F32),
        V((1, S), F32),
        V((1, S), F32),
        V((M,), BF),
        V((M,), BF),
        V((M // 2, F), U32),
        V((M // 2, F), U32),
        V((M // 2, F), U32),
        V((8, TQ), F32),
        pltpu.SMEM((2,), I32),
        V((2, M, TQ), F32),
        V((2, M, TQ), F32),
        V((5, S // 4, HC), U32),
        V((7, S // 4, PR), U32),
        V((7, S // 4, TQ), U32),
        V((7, S // 4, TQ), U32),
        V((7, S // 4, TQ), U32),
        V((7, S // 4, TQ), U32),
        V((M, S), BF),
        pltpu.SemaphoreType.DMA((NSEM,)),
    ]
    outT = pl.pallas_call(
        _kernel,
        in_specs=[pl.BlockSpec(memory_space=pl.ANY)] * 11,
        out_specs=pl.BlockSpec(memory_space=pl.ANY),
        out_shape=jax.ShapeDtypeStruct((M, S), BF),
        scratch_shapes=scratch,
        compiler_params=pltpu.CompilerParams(
            vmem_limit_bytes=100 * 1024 * 1024,
            disable_bounds_checks=E('nochk') != '', disable_semaphore_checks=E('nochk') != ''),
    )(xT, ckv, A_w_q, A_w_uk, A_w_uv, woT, B_w_r, B_w_gate, B_w_up, wdT, gate_w)
    return outT.T.reshape(1, S, M)
```

```python
import math

import jax
import jax.numpy as jnp
from jax import lax
import jax.experimental.pallas as pl
import jax.experimental.pallas.tpu as pltpu

S, M, C, H, D, F = 2048, 448, 1024, 16, 256, 1792
TQ = 128
PR = 2 * TQ
NP = S // PR
PB = 512
NPB = S // PB
NF = F // TQ
HB, HC = PB // 2, C // 2
MP = 512
TW = TQ // 2

BF, F32, U32, I32 = jnp.bfloat16, jnp.float32, jnp.uint32, jnp.int32
NN = (((1,), (0,)), ((), ()))
NT = (((1,), (1,)), ((), ()))
LOG2E = math.log2(math.e)
QSCALE = (D ** -0.5) * LOG2E
NEG = -1e9 * LOG2E
HI16 = 0xFFFF0000

S_WK, S_WV, S_HEAD0, S_HEAD1, S_BULK, S_OUT, S_CKV = range(7)
NSEM = S_CKV + NPB

_PLAN = {
    "first": (
        "T0,T1,T2,GB1,GB0,T3,Q0.1,Q0,SB0,SA1,SA0,Q1,SB1,G8,"
        "PB0,PA0,SA2,PB1,G9,SB2,G10,PA1,G11,SS3.1,SD3,SS3,G12,"
        "PA2,O0,Q2,PB2,G13,G14,SS5.4,SD4,PB3,G15,SS4,PA3,SS5,"
        "PB4,SD5,O1,Q3,SS6.4,SS6.1,TOPK0,SS6,SD6,PD5,PA4,PS5,"
        "PA6,SA7,SB7,PB6,PA7,O2,PB7,O3"),
    "loop": (
        "K0.4,K0.2,Q0,K0,V0,SB0,SS1,SA0,SD1,K1,V1.4,FV0,V1,"
        "PA0,Q1,SD2,SS2,PA1,PB1,K2.2,PB0,SS3.1,PD2,SS3,SD3,"
        "K2.2,V2.1,K2,V2.4,PS2,V2,Q2.3,O0,Q2,SS4.1,SS4,SS5.1,"
        "SS5,SD4,PS3,SD5,K3.5,K3,PD3,PS4,PD4,Q3,SS6.4,PS5.5,V3,"
        "PS5.1,SS6,O1,PD5,SD6,SS7,PS6,PS5,PD6,SD7,O2,PS7.4,"
        "PS7.2,PD7,PS7,O3"),
    "o0": "3641025",
    "fQ": "3614025", "fS": "0136425", "fP": "2014563", "fO": "4032615",
    "oK": "1403625", "oV": "4150623", "oQ": "2546301", "oS": "0136425", "oP": "2014653",
    "oO": "0341625",
    "fhyb": 14, "hyb": 14, "fsto": 1, "sto": 2,
}


def _items(txt):
    out = []
    for t in txt.split(","):
        t, _, cnt = t.partition(".")
        kind = t.rstrip("0123456789")
        out.append((kind, int(t[len(kind):]), int(cnt or 0)))
    return out


def _digits(txt):
    return [int(c) for c in txt]


def _dot(a, b, dn):
    return lax.dot_general(a, b, dn, preferred_element_type=F32)


def _cat(xs, axis):
    return xs[0] if len(xs) == 1 else jnp.concatenate(xs, axis=axis)


def _recip(l):
    r = pl.reciprocal(l, approx=True)
    return r * (2.0 - l * r)


def _sigmoid(z):
    return 1.0 / (1.0 + jnp.exp(-z))


def _bf(w):
    return pltpu.bitcast(w, BF)


def _u32(v):
    return pltpu.bitcast(v.astype(BF), U32)


def _rows(ref, r0, r1):
    return _bf(ref[r0 // 2:r1 // 2, :])


def _put_rows(ref, r0, r1, v):
    ref[r0 // 2:r1 // 2, :] = _u32(v)


def _lhs_terms(a11, a12, a21, a22):
    return [a11 + a22, a21 + a22, a11, a22, a11 + a12, a21 - a11, a12 - a22]


def _rhs_terms(b11, b12, b21, b22):
    return [b11 + b22, b11, b12 - b22, b21 - b11, b22, b11 + b12, b21 + b22]


def _quads(f):
    k, n = f.shape[0] // 2, f.shape[1] // 2
    return f[:k, :n], f[:k, n:], f[k:, :n], f[k:, n:]


def _combine(m):
    return (m[0] + m[3] - m[4] + m[6], m[2] + m[4],
            m[1] + m[3], m[0] - m[1] + m[2] + m[5])


LSUMS = (0, 1, 4, 5, 6)
RSUMS = (0, 2, 3, 5, 6)


def _token_block(idx):
    start = jnp.clip(idx // TQ * TQ, 0, S - TQ)
    return pl.ds(pl.multiple_of(start, TQ), TQ)


def _kernel(xT_hbm, ckv_hbm, wq_hbm, wk_hbm, wv_hbm, wo_hbm, wr_hbm, wg_hbm,
            wu_hbm, wd_hbm, gw_hbm, out_hbm,
            xT_s, x_s, ckv_s, wq32, wkv32, wo_s, q_s, kv_s, ctx_s, acc,
            r_s, g_s, wr_s, gw_s, wg_s, wu_s, wd_s, sig_s, idx_s, xcol_s, ypart_s,
            asum_s, xsum_s, qt_s, kt_s, vt_s, ct_s, out_s, sem):
    wk32, wv32 = wkv32.at[0], wkv32.at[1]
    k_s, v_s = kv_s.at[0], kv_s.at[1]
    (xT_u, ckv_u, wq_u, wk_u, wv_u, wo_u, wg_u, wu_u, wd_u) = (
        r.bitcast(U32) for r in (xT_hbm, ckv_hbm, wq_hbm, wk_hbm, wv_hbm,
                                 wo_hbm, wg_hbm, wu_hbm, wd_hbm))

    def cp(src, dst, s):
        return pltpu.make_async_copy(src, dst, sem.at[s])

    def cp_pair(w_u, w_s, p, s):
        return cp(w_u.at[:, p, :], w_s.at[p], s)

    def cp_ckv(i):
        r = pl.ds(pl.multiple_of(PB // 2 * i, PB // 2), PB // 2)
        return cp(ckv_u.at[r, :], ckv_s.at[r, :], S_CKV + i)

    def cp_out(c0, c1):
        r = pl.ds(c0, c1 - c0)
        return cp(out_s.at[:, r], out_hbm.at[:, r], S_OUT)

    def out_blocks(i):
        r0, r1 = PB * i, PB * (i + 1)
        return [(r0, r1)] if i < NPB - 1 else [(r0, r0 + PR), (r0 + PR, r1)]

    c_wk, c_wv = cp_pair(wk_u, wk32, 0, S_WK), cp_pair(wv_u, wv32, 0, S_WV)
    head0 = [cp(xT_u, xT_s, S_HEAD0), cp_pair(wq_u, wq32, 0, S_HEAD0),
             cp(wr_hbm, wr_s, S_HEAD0), cp(gw_hbm, gw_s, S_HEAD0),
             cp(wo_u.at[0], wo_s.at[0], S_HEAD0)]
    head1 = [cp(wo_u.at[1], wo_s.at[1], S_HEAD1), cp(wg_u, wg_s, S_HEAD1),
             cp(wu_u, wu_s, S_HEAD1), cp(wd_u, wd_s, S_HEAD1)]
    rest = pl.ds(2, H - 2)
    bulk = [cp(wo_u.at[rest], wo_s.at[rest], S_BULK)]
    for p in range(1, H // 2):
        bulk += [cp_pair(wk_u, wk32, p, S_BULK), cp_pair(wv_u, wv32, p, S_BULK),
                 cp_pair(wq_u, wq32, p, S_BULK)]

    row = lax.broadcasted_iota(I32, (TQ, TQ), 0)
    col = lax.broadcasted_iota(I32, (TQ, TQ), 1)
    tri = col <= row

    def head(h, first):
        pre = "f" if first else "o"
        order = _items(_PLAN["first" if first else "loop"])
        kinds = {(k, i) for k, i, _ in order}
        hyb = _PLAN["fhyb" if first else "hyb"]
        sto = _PLAN["fsto" if first else "sto"]
        if first:
            pair, shift = 0, jnp.uint32(16)
        else:
            pair = lax.shift_right_logical(h, 1)
            shift = (16 - 16 * (h & 1)).astype(U32)
        cache, prog, held = {}, {}, {}
        scores, probs_of, ctx_of, rinv = {}, {}, {}, {}

        def wterms(name):
            if name not in cache:
                if name == "O":
                    f = _bf(wo_s[h]).astype(F32)
                    cache[name] = [t.astype(BF) for t in _lhs_terms(*_quads(f))]
                else:
                    ref = {"K": wk32, "V": wv32, "Q": wq32}[name]
                    f = pltpu.bitcast((ref[pair] << shift) & jnp.uint32(HI16), F32)
                    if name == "Q":
                        f = jnp.concatenate([f, jnp.zeros((MP - M, D), F32)], axis=0)
                    cache[name] = [t.astype(BF) for t in _rhs_terms(*_quads(f))]
            return cache[name]

        def term(name, n, j0, j1):
            ref, plain, raw = {"q": (qt_s, q_s, (2, 3)), "k": (kt_s, k_s, (1, 4)),
                               "v": (vt_s, v_s, (1, 4)), "c": (ct_s, None, ())}[name]
            if n in raw:
                odd = raw.index(n)
                return _bf(_cat([plain[TW * (2 * j + odd):TW * (2 * j + odd + 1),
                                       TQ * odd:TQ * (odd + 1)]
                                 for j in range(j0, j1)], 0))
            if first and name in "kv":
                for j in range(j0, j1):
                    if (name, n, j) not in held:
                        f = _rows(plain, PR * j, PR * (j + 1)).astype(F32)
                        f11, f12, f21, f22 = _quads(f)
                        tt = (_rhs_terms(f11, f21, f12, f22) if name == "k"
                              else _rhs_terms(f11, f12, f21, f22))
                        for u in RSUMS:
                            held[name, u, j] = tt[u].astype(BF)
                return _cat([held[name, n, j] for j in range(j0, j1)], 0)
            return _bf(ref[n, TW * j0:TW * j1, :])

        def put_terms(ref, j, terms, which):
            for n in which:
                ref[n, TW * j:TW * (j + 1), :] = _u32(terms[n])

        def run(key, cnt, product):
            m = prog.setdefault(key, {})
            todo = [n for n in _digits(_PLAN[pre + key[0]]) if n not in m]
            for n in (todo[:cnt] if cnt else todo):
                m[n] = product(n)
            return len(m) == 7

        def route(c0, c1):
            if "rg" not in cache:
                r16 = lax.broadcasted_iota(I32, (16, M), 0)
                wr = wr_s[...].astype(F32).reshape(1, M)
                gw = gw_s[...].astype(F32).reshape(1, M)
                cache["rg"] = jnp.where(
                    r16 == 0, wr, jnp.where(r16 == 1, gw, 0.0)).astype(BF)
            rg = _dot(cache["rg"], _bf(xT_s[:, c0:c1]), NN)
            r_s[:, c0:c1] = rg[0:1, :].astype(BF).astype(F32)
            g_s[:, c0:c1] = _sigmoid(rg[1:2, :])

        def set_scores(q, t0, s):
            for t in range(s.shape[1] // TQ):
                blk = s[:, TQ * t:TQ * (t + 1)]
                scores.setdefault(q, {})[t0 + t] = (
                    jnp.where(tri, blk, NEG) if t0 + t == q else blk)

        def probs(q, perm):
            if q not in probs_of:
                tiles = scores.pop(q)
                s = _cat([tiles[t] for t in perm], 1)
                probs_of[q] = jnp.exp2(s - jnp.max(s, axis=1, keepdims=True))
            return probs_of[q]

        def finish(q, o, src):
            if q < hyb:
                rinv[q] = None
                o = o * _recip(jnp.sum(src, axis=1, keepdims=True))
            else:
                la = src[:, 0:TQ]
                for t in range(1, src.shape[1] // TQ):
                    la = la + src[:, TQ * t:TQ * (t + 1)]
                hi = la.astype(BF)
                lo = (la - hi.astype(F32)).astype(BF)
                l = _dot(jnp.ones((16, 2 * TQ), BF),
                         jnp.concatenate([hi, lo], axis=1), NT)[0:1, :]
                rinv[q] = _recip(l)
            i = q // 2
            if i // 2 < sto and 2 * i + 1 < hyb:
                ctx_of[q] = o
                if 2 * i in ctx_of and 2 * i + 1 in ctx_of:
                    oa, ob = ctx_of.pop(2 * i), ctx_of.pop(2 * i + 1)
                    put_terms(ct_s, i, _rhs_terms(oa[:, :TQ], ob[:, :TQ],
                                                  oa[:, TQ:], ob[:, TQ:]), range(7))
            else:
                _put_rows(ctx_s, TQ * q, TQ * (q + 1), o)

        for kind, i, cnt in order:
            r0, r1 = PB * i, PB * (i + 1)
            n0 = PR * i
            qa, qb = 2 * i, 2 * i + 1
            if kind == "T":
                _put_rows(x_s, r0, r1, _bf(xT_s[:, r0:r1]).T)
            elif kind == "GB":
                route(r0, r1)
            elif kind == "G":
                route(TQ * i, TQ * (i + 1))
            elif kind in ("K", "V", "Q"):
                w0, w1 = HB * i // 2, HB * (i + 1) // 2
                if first and ("x", i) not in cache:
                    z = jnp.zeros((HB, MP - M), F32)
                    at = jnp.concatenate([_rows(x_s, r0, r0 + HB).astype(F32), z], axis=1)
                    ab = jnp.concatenate([_rows(x_s, r0 + HB, r1).astype(F32), z], axis=1)
                    tt = _lhs_terms(at[:, :PR], at[:, PR:], ab[:, :PR], ab[:, PR:])
                    cache["x", i] = {n: tt[n].astype(BF) for n in range(7) if n != 2}
                    for n, v in cache["x", i].items():
                        xsum_s[n, w0:w1, :] = pltpu.bitcast(v, U32)

                def lhs(n):
                    if kind == "Q":
                        if n == 2:
                            return _bf(x_s[r0 // 2:(r0 + HB) // 2, :PR])
                        return cache["x", i][n] if first else _bf(xsum_s[n, w0:w1, :])
                    if n == 2:
                        return _bf(ckv_s[r0 // 2:(r0 + HB) // 2, :HC])
                    if n == 3:
                        return _bf(ckv_s[(r0 + HB) // 2:r1 // 2, HC:])
                    return _bf(asum_s[LSUMS.index(n), w0:w1, :])
                if not run((kind, i), cnt, lambda n: _dot(lhs(n), wterms(kind)[n], NN)):
                    continue
                res = _combine(prog.pop((kind, i)))
                if kind == "Q":
                    res = [c * QSCALE for c in res]
                dst = {"K": k_s, "V": v_s, "Q": q_s}[kind]
                for j, (c0, c1) in ((2 * i, res[:2]), (2 * i + 1, res[2:])):
                    _put_rows(dst, PR * j, PR * (j + 1), jnp.concatenate([c0, c1], axis=1))
                    if kind == "V" and any(("PS", u) in kinds for u in range(j + 1, NP)):
                        put_terms(vt_s, j, _rhs_terms(c0[:TQ], c1[:TQ], c0[TQ:], c1[TQ:]), RSUMS)
                    if kind == "K" and any(("SS", u) in kinds for u in range(j + 1, NP)):
                        put_terms(kt_s, j, _rhs_terms(c0[:TQ], c0[TQ:], c1[:TQ], c1[TQ:]), RSUMS)
                    if kind == "Q" and ("SS", j) in kinds:
                        put_terms(qt_s, j, _lhs_terms(c0[:TQ], c1[:TQ], c0[TQ:], c1[TQ:]), LSUMS)
            elif kind in ("SA", "SB"):
                q = qa if kind == "SA" else qb
                set_scores(q, 0, _dot(_rows(q_s, TQ * q, TQ * (q + 1)),
                                      _rows(k_s, 0, TQ * (q + 1)), NT))
            elif kind == "SD":
                for q in (qa, qb):
                    set_scores(q, qa, _dot(_rows(q_s, TQ * q, TQ * (q + 1)),
                                           _rows(k_s, n0, TQ * (q + 1)), NT))
            elif kind == "SS":
                qts = [term("q", n, i, i + 1) for n in range(7)]
                j0 = prog.get(("SS", i), 0)
                prog["SS", i] = j1 = min(i, j0 + cnt) if cnt else i
                for j in range(j0, j1):
                    cs = _combine({n: _dot(qts[n], term("k", n, j, j + 1), NT)
                                   for n in _digits(_PLAN[pre + "S"])})
                    scores.setdefault(qa, {}).update({2 * j: cs[0], 2 * j + 1: cs[1]})
                    scores.setdefault(qb, {}).update({2 * j: cs[2], 2 * j + 1: cs[3]})
            elif kind in ("PA", "PB"):
                q = qa if kind == "PA" else qb
                p = probs(q, range(q + 1)).astype(BF)
                probs_of.pop(q)
                finish(q, _dot(p, _rows(v_s, 0, TQ * (q + 1)), NN), p.astype(F32))
            elif kind in ("PS", "PD"):
                w = TQ * i
                eo = list(range(0, qa, 2)) + list(range(1, qa, 2))
                pa, pb = probs(qa, eo + [qa]), probs(qb, eo + [qa, qb])
                if ("diag", i) not in prog:
                    prog["diag", i] = (pa[:, 2 * w:].astype(BF), pb[:, 2 * w:].astype(BF))
                da, db = prog["diag", i]
                if kind == "PD":
                    prog["PD", i] = (_dot(da, _rows(v_s, n0, n0 + TQ), NN),
                                     _dot(db, _rows(v_s, n0, n0 + PR), NN))
                else:
                    if ("L", i) not in prog:
                        prog["L", i] = [t.astype(BF) for t in _lhs_terms(
                            pa[:, :w], pa[:, w:2 * w], pb[:, :w], pb[:, w:2 * w])]
                    if not run(("P", i), cnt, lambda n: _dot(
                            prog["L", i][n], term("v", n, 0, i), NN)):
                        continue
                if ("PD", i) in prog and len(prog.get(("P", i), ())) == 7:
                    c11, c12, c21, c22 = _combine(prog.pop(("P", i)))
                    oa, ob = prog.pop(("PD", i))
                    lt = prog.pop(("L", i))
                    oa = jnp.concatenate([c11, c12], axis=1) + oa
                    ob = jnp.concatenate([c21, c22], axis=1) + ob
                    for q, o, lo_, d in ((qa, oa, lt[4], da), (qb, ob, lt[1], db)):
                        probs_of.pop(q)
                        finish(q, o, jnp.concatenate([lo_, d], axis=1).astype(F32))
            elif kind == "O":
                j0, j1 = 2 * i, 2 * i + 2
                js = max(j0, min(j1, hyb // 2)) if i < sto else j0
                cols = []
                if js > j0:
                    c11, c12, c21, c22 = _combine(
                        {n: _dot(wterms("O")[n], term("c", n, j0, js), NT)
                         for n in _digits(_PLAN[pre + "O"])})
                    ca = jnp.concatenate([c11, c21], axis=0)
                    cb = jnp.concatenate([c12, c22], axis=0)
                    for t in range(js - j0):
                        cols += [ca[:, TQ * t:TQ * (t + 1)], cb[:, TQ * t:TQ * (t + 1)]]
                if j1 > js:
                    cols.append(_dot(_bf(wo_s[h]), _rows(ctx_s, PR * js, PR * j1), NT))
                g = g_s[:, r0:r1]
                f = []
                for t in range(4):
                    gt, rt = g[:, TQ * t:TQ * (t + 1)], rinv.pop(4 * i + t)
                    f.append(gt if rt is None else gt * rt)
                a = _cat(cols, 1) * jnp.concatenate(f, axis=1)
                if first:
                    acc[:, r0:r1] = a + (1.0 - g) * _bf(xT_s[:, r0:r1]).astype(F32)
                else:
                    a = acc[:, r0:r1] + a
                    acc[:, r0:r1] = a
                    for c0, c1 in out_blocks(i):
                        out_s[:, c0:c1] = a[:, c0 - r0:c1 - r0].astype(BF)

                        @pl.when(h == H - 1)
                        def _():
                            cp_out(c0, c1).start()
            elif kind == "TOPK":
                r = r_s[...]
                lane = lax.broadcasted_iota(I32, (1, S), 1)
                m1 = jnp.max(r, axis=1, keepdims=True)
                i1 = jnp.min(jnp.where(r == m1, lane, S - 1))
                r2 = jnp.where(lane == i1, -jnp.inf, r)
                m2 = jnp.max(r2, axis=1, keepdims=True)
                i2 = jnp.min(jnp.where((r2 == m2) & (lane != i1), lane, S - 1))
                r8 = lax.broadcasted_iota(I32, (8, TQ), 0)
                sig_s[...] = jnp.where(r8 == 0, _sigmoid(m1), _sigmoid(m2))
                lane = lax.broadcasted_iota(I32, (1, TQ), 1)
                for t, idx in enumerate((i1, i2)):
                    idx_s[t] = idx
                    xb = _bf(xT_s[:, _token_block(idx)]).astype(F32)
                    xc = jnp.sum(jnp.where(lane == idx % TQ, xb, 0.0),
                                 axis=1, keepdims=True)
                    xcol_s[t] = jnp.broadcast_to(xc, (M, TQ))
                ypart_s[...] = jnp.zeros_like(ypart_s)
            elif kind == "FV":
                chunk = jnp.minimum(h - 1, NF - 1)
                c = pl.ds(pl.multiple_of(chunk * TQ, TQ), TQ)
                wg, wu, wd = (_bf(w[:, c]).astype(F32) for w in (wg_s, wu_s, wd_s))
                for t in range(2):
                    xc = xcol_s[t]
                    g = jnp.sum(xc * wg, axis=0, keepdims=True)
                    u = jnp.sum(xc * wu, axis=0, keepdims=True)
                    ypart_s[t] += wd * (g * _sigmoid(g) * u)
            else:
                raise ValueError(kind)
        assert not (scores or probs_of or ctx_of or rinv)

    for c in [cp_ckv(0), c_wk, c_wv] + [cp_ckv(i) for i in range(1, NPB)]:
        c.start()
    for c in head0 + head1 + bulk:
        c.start()

    def proj0(t, carry):
        which, blk = t % 2, t // 2
        base = pl.multiple_of(blk * (PB // 2), PB // 2)
        half = pl.multiple_of(blk * (HB // 2), HB // 2)

        @pl.when(which == 0)
        def _():
            cp_ckv(blk).wait()

        @pl.when(t == 0)
        def _():
            c_wk.wait()

        @pl.when(t == 1)
        def _():
            c_wv.wait()

        top, bot = pl.ds(base, HB // 2), pl.ds(base + HB // 2, HB // 2)
        at, ab = _bf(ckv_s[top, :]).astype(F32), _bf(ckv_s[bot, :]).astype(F32)
        tt = _lhs_terms(at[:, :HC], at[:, HC:], ab[:, :HC], ab[:, HC:])
        lhs = {n: tt[n].astype(BF) for n in LSUMS}
        for k, n in enumerate(LSUMS):
            asum_s[k, pl.ds(half, HB // 2), :] = pltpu.bitcast(lhs[n], U32)
        lhs[2], lhs[3] = _bf(ckv_s[top, :HC]), _bf(ckv_s[bot, HC:])
        f = pltpu.bitcast(wkv32[which, 0] << 16, F32)
        rhs = [u.astype(BF) for u in _rhs_terms(*_quads(f))]
        c11, c12, c21, c22 = _combine(
            {n: _dot(lhs[n], rhs[n], NN) for n in _digits(_PLAN["o0"])})
        kv_s[which, top, :] = _u32(jnp.concatenate([c11, c12], axis=1))
        kv_s[which, bot, :] = _u32(jnp.concatenate([c21, c22], axis=1))
        return carry

    def step(h, carry):
        @pl.when(h == 2)
        def _():
            for c in bulk:
                c.wait()

        @pl.when(h == H - 1)
        def _():
            lane = lax.broadcasted_iota(I32, (1, TQ), 1)
            for t in range(2):
                idx = idx_s[t]
                y = jnp.sum(ypart_s[t], axis=1, keepdims=True) * sig_s[t:t + 1, :]
                blk = _token_block(idx)
                old = acc[:, blk]
                acc[:, blk] = jnp.where(
                    lane == idx % TQ, old + (1.0 - g_s[:, blk]) * y, old)

        head(h, False)
        return carry

    lax.fori_loop(0, 2 * NPB, proj0, 0)
    for c in head0:
        c.wait()
    head(0, True)
    for c in head1:
        c.wait()
    lax.fori_loop(1, H, step, 0)
    for i in range(NPB):
        for c0, c1 in out_blocks(i):
            cp_out(c0, c1).wait()


@jax.jit
def pallas_gated_mix__compressed_kv_cla__moe_arch_mod__prompt_kernel(
    A_x: jax.Array,
    A_c_kv: jax.Array,
    A_w_q: jax.Array,
    A_w_uk: jax.Array,
    A_w_uv: jax.Array,
    A_w_o: jax.Array,
    B_x: jax.Array,
    B_w_r: jax.Array,
    B_w_gate: jax.Array,
    B_w_up: jax.Array,
    B_w_down: jax.Array,
    gate_w: jax.Array,
):
    del B_x
    xT = A_x.reshape(S, M).T
    ckv = A_c_kv.reshape(S, C)
    woT = jnp.transpose(A_w_o, (0, 2, 1))
    wdT = B_w_down.T

    V = pltpu.VMEM
    scratch = [
        V((M // 2, S), U32),
        V((S // 2, M), U32),
        V((S // 2, C), U32),
        V((H // 2, M, D), U32),
        V((2, H // 2, C, D), U32),
        V((H, M // 2, D), U32),
        V((S // 2, D), U32),
        V((2, S // 2, D), U32),
        V((S // 2, D), U32),
        V((M, S), F32),
        V((1, S), F32),
        V((1, S), F32),
        V((M,), BF),
        V((M,), BF),
        V((M // 2, F), U32),
        V((M // 2, F), U32),
        V((M // 2, F), U32),
        V((8, TQ), F32),
        pltpu.SMEM((2,), I32),
        V((2, M, TQ), F32),
        V((2, M, TQ), F32),
        V((5, S // 4, HC), U32),
        V((7, S // 4, PR), U32),
        V((7, S // 4, TQ), U32),
        V((7, S // 4, TQ), U32),
        V((7, S // 4, TQ), U32),
        V((7, S // 4, TQ), U32),
        V((M, S), BF),
        pltpu.SemaphoreType.DMA((NSEM,)),
    ]
    outT = pl.pallas_call(
        _kernel,
        in_specs=[pl.BlockSpec(memory_space=pl.ANY)] * 11,
        out_specs=pl.BlockSpec(memory_space=pl.ANY),
        out_shape=jax.ShapeDtypeStruct((M, S), BF),
        scratch_shapes=scratch,
        compiler_params=pltpu.CompilerParams(
            vmem_limit_bytes=100 * 1024 * 1024),
    )(xT, ckv, A_w_q, A_w_uk, A_w_uv, woT, B_w_r, B_w_gate, B_w_up, wdT, gate_w)
    return outT.T.reshape(1, S, M)
```

```python
import math

import jax
import jax.numpy as jnp
from jax import lax
import jax.experimental.pallas as pl
import jax.experimental.pallas.tpu as pltpu

S, M, C, H, D, F = 2048, 448, 1024, 16, 256, 1792
TQ = 128
PR = 2 * TQ
NP = S // PR
PB = 512
NPB = S // PB
NF = F // TQ
HB, HC = PB // 2, C // 2
MP = 512
TW = TQ // 2

BF, F32, U32, I32 = jnp.bfloat16, jnp.float32, jnp.uint32, jnp.int32
NN = (((1,), (0,)), ((), ()))
NT = (((1,), (1,)), ((), ()))
LOG2E = math.log2(math.e)
QSCALE = (D ** -0.5) * LOG2E
NEG = -1e9 * LOG2E
HI16 = 0xFFFF0000

S_WK, S_WV, S_HEAD0, S_HEAD1, S_BULK, S_OUT, S_CKV = range(7)
NSEM = S_CKV + NPB

_PLAN = {
    "first": (
        "T0,T1,T2,GB1,GB0,T3,Q0.1,Q0,SB0,SA1,SA0,Q1,SB1,G8,"
        "PB0,PA0,SA2,PB1,G9,SB2,G10,PA1,G11,SS3.1,SS3.1,SD3,"
        "SS3,G12,PA2,O0,Q2,PB2,G13,G14,SS5.4,SD4,PB3,G15,SS4,"
        "PA3,SS5,PB4,SD5,O1,Q3,SS6.4,SS6.1,TOPK0,SS6,SD6,PD5,"
        "PA4,PS5,PA6,SA7,SB7,PB6,PA7,O2,PB7,O3"),
    "loop": (
        "K0.4,K0.2,Q0,K0,V0,SB0,K1.3,SS1,SA0,SD1,K1,V1.4,FV0,"
        "V1,PA0,Q1,SD2,SS2,PA1,PB1,K2.2,PB0,SS3.1,PD2,SS3,SD3,"
        "V2.1,K2,V2.4,PS2,V2,Q2.3,O0,Q2,SS4.1,SS4,SS5.1,SS5,"
        "SD4,PS3,SD5,K3.1,K3.5,K3,PD3,PD4,Q3,SS6.4,PS5.5,PS4,"
        "V3,PS5.1,SS6,O1,PD5,SD6,SS7,PS6,PS5,PD6,SD7,O2,PS7.4,"
        "PS7.2,PD7,PS7,O3"),
    "o0": "3641025",
    "fQ": "3614025", "fS": "0136425", "fP": "2014365", "fO": "4032615",
    "oK": "4103625", "oV": "4150623", "oQ": "2546301", "oS": "0136425", "oP": "2014653",
    "oO": "0413625",
    "fhyb": 14, "hyb": 14, "fsto": 1, "sto": 2,
}


def _items(txt):
    out = []
    for t in txt.split(","):
        t, _, cnt = t.partition(".")
        kind = t.rstrip("0123456789")
        out.append((kind, int(t[len(kind):]), int(cnt or 0)))
    return out


def _digits(txt):
    return [int(c) for c in txt]


def _dot(a, b, dn):
    return lax.dot_general(a, b, dn, preferred_element_type=F32)


def _cat(xs, axis):
    return xs[0] if len(xs) == 1 else jnp.concatenate(xs, axis=axis)


def _recip(l):
    r = pl.reciprocal(l, approx=True)
    return r * (2.0 - l * r)


def _sigmoid(z):
    return 1.0 / (1.0 + jnp.exp(-z))


def _bf(w):
    return pltpu.bitcast(w, BF)


def _u32(v):
    return pltpu.bitcast(v.astype(BF), U32)


def _rows(ref, r0, r1):
    return _bf(ref[r0 // 2:r1 // 2, :])


def _put_rows(ref, r0, r1, v):
    ref[r0 // 2:r1 // 2, :] = _u32(v)


def _lhs_terms(a11, a12, a21, a22):
    return [a11 + a22, a21 + a22, a11, a22, a11 + a12, a21 - a11, a12 - a22]


def _rhs_terms(b11, b12, b21, b22):
    return [b11 + b22, b11, b12 - b22, b21 - b11, b22, b11 + b12, b21 + b22]


def _quads(f):
    k, n = f.shape[0] // 2, f.shape[1] // 2
    return f[:k, :n], f[:k, n:], f[k:, :n], f[k:, n:]


def _combine(m):
    return (m[0] + m[3] - m[4] + m[6], m[2] + m[4],
            m[1] + m[3], m[0] - m[1] + m[2] + m[5])


LSUMS = (0, 1, 4, 5, 6)
RSUMS = (0, 2, 3, 5, 6)


def _token_block(idx):
    start = jnp.clip(idx // TQ * TQ, 0, S - TQ)
    return pl.ds(pl.multiple_of(start, TQ), TQ)


def _kernel(xT_hbm, ckv_hbm, wq_hbm, wk_hbm, wv_hbm, wo_hbm, wr_hbm, wg_hbm,
            wu_hbm, wd_hbm, gw_hbm, out_hbm,
            xT_s, x_s, ckv_s, wq32, wkv32, wo_s, q_s, kv_s, ctx_s, acc,
            r_s, g_s, wr_s, gw_s, wg_s, wu_s, wd_s, sig_s, idx_s, xcol_s, ypart_s,
            asum_s, xsum_s, qt_s, kt_s, vt_s, ct_s, out_s, sem):
    wk32, wv32 = wkv32.at[0], wkv32.at[1]
    k_s, v_s = kv_s.at[0], kv_s.at[1]
    (xT_u, ckv_u, wq_u, wk_u, wv_u, wo_u, wg_u, wu_u, wd_u) = (
        r.bitcast(U32) for r in (xT_hbm, ckv_hbm, wq_hbm, wk_hbm, wv_hbm,
                                 wo_hbm, wg_hbm, wu_hbm, wd_hbm))

    def cp(src, dst, s):
        return pltpu.make_async_copy(src, dst, sem.at[s])

    def cp_pair(w_u, w_s, p, s):
        return cp(w_u.at[:, p, :], w_s.at[p], s)

    def cp_ckv(i):
        r = pl.ds(pl.multiple_of(PB // 2 * i, PB // 2), PB // 2)
        return cp(ckv_u.at[r, :], ckv_s.at[r, :], S_CKV + i)

    def cp_out(c0, c1):
        r = pl.ds(c0, c1 - c0)
        return cp(out_s.at[:, r], out_hbm.at[:, r], S_OUT)

    def out_blocks(i):
        r0, r1 = PB * i, PB * (i + 1)
        return [(r0, r1)] if i < NPB - 1 else [(r0, r0 + PR), (r0 + PR, r1)]

    c_wk, c_wv = cp_pair(wk_u, wk32, 0, S_WK), cp_pair(wv_u, wv32, 0, S_WV)
    head0 = [cp(xT_u, xT_s, S_HEAD0), cp_pair(wq_u, wq32, 0, S_HEAD0),
             cp(wr_hbm, wr_s, S_HEAD0), cp(gw_hbm, gw_s, S_HEAD0),
             cp(wo_u.at[0], wo_s.at[0], S_HEAD0)]
    head1 = [cp(wo_u.at[1], wo_s.at[1], S_HEAD1), cp(wg_u, wg_s, S_HEAD1),
             cp(wu_u, wu_s, S_HEAD1), cp(wd_u, wd_s, S_HEAD1)]
    rest = pl.ds(2, H - 2)
    bulk = [cp(wo_u.at[rest], wo_s.at[rest], S_BULK)]
    for p in range(1, H // 2):
        bulk += [cp_pair(wk_u, wk32, p, S_BULK), cp_pair(wv_u, wv32, p, S_BULK),
                 cp_pair(wq_u, wq32, p, S_BULK)]

    row = lax.broadcasted_iota(I32, (TQ, TQ), 0)
    col = lax.broadcasted_iota(I32, (TQ, TQ), 1)
    tri = col <= row

    def head(h, first):
        pre = "f" if first else "o"
        order = _items(_PLAN["first" if first else "loop"])
        kinds = {(k, i) for k, i, _ in order}
        hyb = _PLAN["fhyb" if first else "hyb"]
        sto = _PLAN["fsto" if first else "sto"]
        if first:
            pair, shift = 0, jnp.uint32(16)
        else:
            pair = lax.shift_right_logical(h, 1)
            shift = (16 - 16 * (h & 1)).astype(U32)
        cache, prog, held = {}, {}, {}
        scores, probs_of, ctx_of, rinv = {}, {}, {}, {}

        def wterms(name):
            if name not in cache:
                if name == "O":
                    f = _bf(wo_s[h]).astype(F32)
                    cache[name] = [t.astype(BF) for t in _lhs_terms(*_quads(f))]
                else:
                    ref = {"K": wk32, "V": wv32, "Q": wq32}[name]
                    f = pltpu.bitcast((ref[pair] << shift) & jnp.uint32(HI16), F32)
                    if name == "Q":
                        f = jnp.concatenate([f, jnp.zeros((MP - M, D), F32)], axis=0)
                    cache[name] = [t.astype(BF) for t in _rhs_terms(*_quads(f))]
            return cache[name]

        def term(name, n, j0, j1):
            ref, plain, raw = {"q": (qt_s, q_s, (2, 3)), "k": (kt_s, k_s, (1, 4)),
                               "v": (vt_s, v_s, (1, 4)), "c": (ct_s, None, ())}[name]
            if n in raw:
                odd = raw.index(n)
                return _bf(_cat([plain[TW * (2 * j + odd):TW * (2 * j + odd + 1),
                                       TQ * odd:TQ * (odd + 1)]
                                 for j in range(j0, j1)], 0))
            if first and name in "kv":
                for j in range(j0, j1):
                    if (name, n, j) not in held:
                        f = _rows(plain, PR * j, PR * (j + 1)).astype(F32)
                        f11, f12, f21, f22 = _quads(f)
                        tt = (_rhs_terms(f11, f21, f12, f22) if name == "k"
                              else _rhs_terms(f11, f12, f21, f22))
                        for u in RSUMS:
                            held[name, u, j] = tt[u].astype(BF)
                return _cat([held[name, n, j] for j in range(j0, j1)], 0)
            return _bf(ref[n, TW * j0:TW * j1, :])

        def put_terms(ref, j, terms, which):
            for n in which:
                ref[n, TW * j:TW * (j + 1), :] = _u32(terms[n])

        def run(key, cnt, product):
            m = prog.setdefault(key, {})
            todo = [n for n in _digits(_PLAN[pre + key[0]]) if n not in m]
            for n in (todo[:cnt] if cnt else todo):
                m[n] = product(n)
            return len(m) == 7

        def route(c0, c1):
            if "rg" not in cache:
                r16 = lax.broadcasted_iota(I32, (16, M), 0)
                wr = wr_s[...].astype(F32).reshape(1, M)
                gw = gw_s[...].astype(F32).reshape(1, M)
                cache["rg"] = jnp.where(
                    r16 == 0, wr, jnp.where(r16 == 1, gw, 0.0)).astype(BF)
            rg = _dot(cache["rg"], _bf(xT_s[:, c0:c1]), NN)
            r_s[:, c0:c1] = rg[0:1, :].astype(BF).astype(F32)
            g_s[:, c0:c1] = _sigmoid(rg[1:2, :])

        def set_scores(q, t0, s):
            for t in range(s.shape[1] // TQ):
                blk = s[:, TQ * t:TQ * (t + 1)]
                scores.setdefault(q, {})[t0 + t] = (
                    jnp.where(tri, blk, NEG) if t0 + t == q else blk)

        def probs(q, perm):
            if q not in probs_of:
                tiles = scores.pop(q)
                s = _cat([tiles[t] for t in perm], 1)
                probs_of[q] = jnp.exp2(s - jnp.max(s, axis=1, keepdims=True))
            return probs_of[q]

        def finish(q, o, src):
            if q < hyb:
                rinv[q] = None
                o = o * _recip(jnp.sum(src, axis=1, keepdims=True))
            else:
                la = src[:, 0:TQ]
                for t in range(1, src.shape[1] // TQ):
                    la = la + src[:, TQ * t:TQ * (t + 1)]
                hi = la.astype(BF)
                lo = (la - hi.astype(F32)).astype(BF)
                l = _dot(jnp.ones((16, 2 * TQ), BF),
                         jnp.concatenate([hi, lo], axis=1), NT)[0:1, :]
                rinv[q] = _recip(l)
            i = q // 2
            if i // 2 < sto and 2 * i + 1 < hyb:
                ctx_of[q] = o
                if 2 * i in ctx_of and 2 * i + 1 in ctx_of:
                    oa, ob = ctx_of.pop(2 * i), ctx_of.pop(2 * i + 1)
                    put_terms(ct_s, i, _rhs_terms(oa[:, :TQ], ob[:, :TQ],
                                                  oa[:, TQ:], ob[:, TQ:]), range(7))
            else:
                _put_rows(ctx_s, TQ * q, TQ * (q + 1), o)

        for kind, i, cnt in order:
            r0, r1 = PB * i, PB * (i + 1)
            n0 = PR * i
            qa, qb = 2 * i, 2 * i + 1
            if kind == "T":
                _put_rows(x_s, r0, r1, _bf(xT_s[:, r0:r1]).T)
            elif kind == "GB":
                route(r0, r1)
            elif kind == "G":
                route(TQ * i, TQ * (i + 1))
            elif kind in ("K", "V", "Q"):
                w0, w1 = HB * i // 2, HB * (i + 1) // 2
                if first and ("x", i) not in cache:
                    z = jnp.zeros((HB, MP - M), F32)
                    at = jnp.concatenate([_rows(x_s, r0, r0 + HB).astype(F32), z], axis=1)
                    ab = jnp.concatenate([_rows(x_s, r0 + HB, r1).astype(F32), z], axis=1)
                    tt = _lhs_terms(at[:, :PR], at[:, PR:], ab[:, :PR], ab[:, PR:])
                    cache["x", i] = {n: tt[n].astype(BF) for n in range(7) if n != 2}
                    for n, v in cache["x", i].items():
                        xsum_s[n, w0:w1, :] = pltpu.bitcast(v, U32)

                def lhs(n):
                    if kind == "Q":
                        if n == 2:
                            return _bf(x_s[r0 // 2:(r0 + HB) // 2, :PR])
                        return cache["x", i][n] if first else _bf(xsum_s[n, w0:w1, :])
                    if n == 2:
                        return _bf(ckv_s[r0 // 2:(r0 + HB) // 2, :HC])
                    if n == 3:
                        return _bf(ckv_s[(r0 + HB) // 2:r1 // 2, HC:])
                    return _bf(asum_s[LSUMS.index(n), w0:w1, :])
                if not run((kind, i), cnt, lambda n: _dot(lhs(n), wterms(kind)[n], NN)):
                    continue
                res = _combine(prog.pop((kind, i)))
                if kind == "Q":
                    res = [c * QSCALE for c in res]
                dst = {"K": k_s, "V": v_s, "Q": q_s}[kind]
                for j, (c0, c1) in ((2 * i, res[:2]), (2 * i + 1, res[2:])):
                    _put_rows(dst, PR * j, PR * (j + 1), jnp.concatenate([c0, c1], axis=1))
                    if kind == "V" and any(("PS", u) in kinds for u in range(j + 1, NP)):
                        put_terms(vt_s, j, _rhs_terms(c0[:TQ], c1[:TQ], c0[TQ:], c1[TQ:]), RSUMS)
                    if kind == "K" and any(("SS", u) in kinds for u in range(j + 1, NP)):
                        put_terms(kt_s, j, _rhs_terms(c0[:TQ], c0[TQ:], c1[:TQ], c1[TQ:]), RSUMS)
                    if kind == "Q" and ("SS", j) in kinds:
                        put_terms(qt_s, j, _lhs_terms(c0[:TQ], c1[:TQ], c0[TQ:], c1[TQ:]), LSUMS)
            elif kind in ("SA", "SB"):
                q = qa if kind == "SA" else qb
                set_scores(q, 0, _dot(_rows(q_s, TQ * q, TQ * (q + 1)),
                                      _rows(k_s, 0, TQ * (q + 1)), NT))
            elif kind == "SD":
                for q in (qa, qb):
                    set_scores(q, qa, _dot(_rows(q_s, TQ * q, TQ * (q + 1)),
                                           _rows(k_s, n0, TQ * (q + 1)), NT))
            elif kind == "SS":
                qts = [term("q", n, i, i + 1) for n in range(7)]
                j0 = prog.get(("SS", i), 0)
                prog["SS", i] = j1 = min(i, j0 + cnt) if cnt else i
                for j in range(j0, j1):
                    cs = _combine({n: _dot(qts[n], term("k", n, j, j + 1), NT)
                                   for n in _digits(_PLAN[pre + "S"])})
                    scores.setdefault(qa, {}).update({2 * j: cs[0], 2 * j + 1: cs[1]})
                    scores.setdefault(qb, {}).update({2 * j: cs[2], 2 * j + 1: cs[3]})
            elif kind in ("PA", "PB"):
                q = qa if kind == "PA" else qb
                p = probs(q, range(q + 1)).astype(BF)
                probs_of.pop(q)
                finish(q, _dot(p, _rows(v_s, 0, TQ * (q + 1)), NN), p.astype(F32))
            elif kind in ("PS", "PD"):
                w = TQ * i
                eo = list(range(0, qa, 2)) + list(range(1, qa, 2))
                pa, pb = probs(qa, eo + [qa]), probs(qb, eo + [qa, qb])
                if ("diag", i) not in prog:
                    prog["diag", i] = (pa[:, 2 * w:].astype(BF), pb[:, 2 * w:].astype(BF))
                da, db = prog["diag", i]
                if kind == "PD":
                    prog["PD", i] = (_dot(da, _rows(v_s, n0, n0 + TQ), NN),
                                     _dot(db, _rows(v_s, n0, n0 + PR), NN))
                else:
                    if ("L", i) not in prog:
                        prog["L", i] = [t.astype(BF) for t in _lhs_terms(
                            pa[:, :w], pa[:, w:2 * w], pb[:, :w], pb[:, w:2 * w])]
                    if not run(("P", i), cnt, lambda n: _dot(
                            prog["L", i][n], term("v", n, 0, i), NN)):
                        continue
                if ("PD", i) in prog and len(prog.get(("P", i), ())) == 7:
                    c11, c12, c21, c22 = _combine(prog.pop(("P", i)))
                    oa, ob = prog.pop(("PD", i))
                    lt = prog.pop(("L", i))
                    oa = jnp.concatenate([c11, c12], axis=1) + oa
                    ob = jnp.concatenate([c21, c22], axis=1) + ob
                    for q, o, lo_, d in ((qa, oa, lt[4], da), (qb, ob, lt[1], db)):
                        probs_of.pop(q)
                        finish(q, o, jnp.concatenate([lo_, d], axis=1).astype(F32))
            elif kind == "O":
                j0, j1 = 2 * i, 2 * i + 2
                js = max(j0, min(j1, hyb // 2)) if i < sto else j0
                cols = []
                if js > j0:
                    c11, c12, c21, c22 = _combine(
                        {n: _dot(wterms("O")[n], term("c", n, j0, js), NT)
                         for n in _digits(_PLAN[pre + "O"])})
                    ca = jnp.concatenate([c11, c21], axis=0)
                    cb = jnp.concatenate([c12, c22], axis=0)
                    for t in range(js - j0):
                        cols += [ca[:, TQ * t:TQ * (t + 1)], cb[:, TQ * t:TQ * (t + 1)]]
                if j1 > js:
                    cols.append(_dot(_bf(wo_s[h]), _rows(ctx_s, PR * js, PR * j1), NT))
                g = g_s[:, r0:r1]
                f = []
                for t in range(4):
                    gt, rt = g[:, TQ * t:TQ * (t + 1)], rinv.pop(4 * i + t)
                    f.append(gt if rt is None else gt * rt)
                a = _cat(cols, 1) * jnp.concatenate(f, axis=1)
                if first:
                    acc[:, r0:r1] = a + (1.0 - g) * _bf(xT_s[:, r0:r1]).astype(F32)
                else:
                    a = acc[:, r0:r1] + a
                    acc[:, r0:r1] = a
                    for c0, c1 in out_blocks(i):
                        out_s[:, c0:c1] = a[:, c0 - r0:c1 - r0].astype(BF)

                        @pl.when(h == H - 1)
                        def _():
                            cp_out(c0, c1).start()
            elif kind == "TOPK":
                r = r_s[...]
                lane = lax.broadcasted_iota(I32, (1, S), 1)
                m1 = jnp.max(r, axis=1, keepdims=True)
                i1 = jnp.min(jnp.where(r == m1, lane, S - 1))
                r2 = jnp.where(lane == i1, -jnp.inf, r)
                m2 = jnp.max(r2, axis=1, keepdims=True)
                i2 = jnp.min(jnp.where((r2 == m2) & (lane != i1), lane, S - 1))
                r8 = lax.broadcasted_iota(I32, (8, TQ), 0)
                sig_s[...] = jnp.where(r8 == 0, _sigmoid(m1), _sigmoid(m2))
                lane = lax.broadcasted_iota(I32, (1, TQ), 1)
                for t, idx in enumerate((i1, i2)):
                    idx_s[t] = idx
                    xb = _bf(xT_s[:, _token_block(idx)]).astype(F32)
                    xc = jnp.sum(jnp.where(lane == idx % TQ, xb, 0.0),
                                 axis=1, keepdims=True)
                    xcol_s[t] = jnp.broadcast_to(xc, (M, TQ))
                ypart_s[...] = jnp.zeros_like(ypart_s)
            elif kind == "FV":
                chunk = jnp.minimum(h - 1, NF - 1)
                c = pl.ds(pl.multiple_of(chunk * TQ, TQ), TQ)
                wg, wu, wd = (_bf(w[:, c]).astype(F32) for w in (wg_s, wu_s, wd_s))
                for t in range(2):
                    xc = xcol_s[t]
                    g = jnp.sum(xc * wg, axis=0, keepdims=True)
                    u = jnp.sum(xc * wu, axis=0, keepdims=True)
                    ypart_s[t] += wd * (g * _sigmoid(g) * u)
            else:
                raise ValueError(kind)
        assert not (scores or probs_of or ctx_of or rinv)

    for c in [cp_ckv(0), c_wk, c_wv] + [cp_ckv(i) for i in range(1, NPB)]:
        c.start()
    for c in head0 + head1 + bulk:
        c.start()

    def proj0(t, carry):
        which, blk = t % 2, t // 2
        base = pl.multiple_of(blk * (PB // 2), PB // 2)
        half = pl.multiple_of(blk * (HB // 2), HB // 2)

        @pl.when(which == 0)
        def _():
            cp_ckv(blk).wait()

        @pl.when(t == 0)
        def _():
            c_wk.wait()

        @pl.when(t == 1)
        def _():
            c_wv.wait()

        top, bot = pl.ds(base, HB // 2), pl.ds(base + HB // 2, HB // 2)
        at, ab = _bf(ckv_s[top, :]).astype(F32), _bf(ckv_s[bot, :]).astype(F32)
        tt = _lhs_terms(at[:, :HC], at[:, HC:], ab[:, :HC], ab[:, HC:])
        lhs = {n: tt[n].astype(BF) for n in LSUMS}
        for k, n in enumerate(LSUMS):
            asum_s[k, pl.ds(half, HB // 2), :] = pltpu.bitcast(lhs[n], U32)
        lhs[2], lhs[3] = _bf(ckv_s[top, :HC]), _bf(ckv_s[bot, HC:])
        f = pltpu.bitcast(wkv32[which, 0] << 16, F32)
        rhs = [u.astype(BF) for u in _rhs_terms(*_quads(f))]
        c11, c12, c21, c22 = _combine(
            {n: _dot(lhs[n], rhs[n], NN) for n in _digits(_PLAN["o0"])})
        kv_s[which, top, :] = _u32(jnp.concatenate([c11, c12], axis=1))
        kv_s[which, bot, :] = _u32(jnp.concatenate([c21, c22], axis=1))
        return carry

    def step(h, carry):
        @pl.when(h == 2)
        def _():
            for c in bulk:
                c.wait()

        @pl.when(h == H - 1)
        def _():
            lane = lax.broadcasted_iota(I32, (1, TQ), 1)
            for t in range(2):
                idx = idx_s[t]
                y = jnp.sum(ypart_s[t], axis=1, keepdims=True) * sig_s[t:t + 1, :]
                blk = _token_block(idx)
                old = acc[:, blk]
                acc[:, blk] = jnp.where(
                    lane == idx % TQ, old + (1.0 - g_s[:, blk]) * y, old)

        head(h, False)
        return carry

    lax.fori_loop(0, 2 * NPB, proj0, 0)
    for c in head0:
        c.wait()
    head(0, True)
    for c in head1:
        c.wait()
    lax.fori_loop(1, H, step, 0)
    for i in range(NPB):
        for c0, c1 in out_blocks(i):
            cp_out(c0, c1).wait()


@jax.jit
def pallas_gated_mix__compressed_kv_cla__moe_arch_mod__prompt_kernel(
    A_x: jax.Array,
    A_c_kv: jax.Array,
    A_w_q: jax.Array,
    A_w_uk: jax.Array,
    A_w_uv: jax.Array,
    A_w_o: jax.Array,
    B_x: jax.Array,
    B_w_r: jax.Array,
    B_w_gate: jax.Array,
    B_w_up: jax.Array,
    B_w_down: jax.Array,
    gate_w: jax.Array,
):
    del B_x
    xT = A_x.reshape(S, M).T
    ckv = A_c_kv.reshape(S, C)
    woT = jnp.transpose(A_w_o, (0, 2, 1))
    wdT = B_w_down.T

    V = pltpu.VMEM
    scratch = [
        V((M // 2, S), U32),
        V((S // 2, M), U32),
        V((S // 2, C), U32),
        V((H // 2, M, D), U32),
        V((2, H // 2, C, D), U32),
        V((H, M // 2, D), U32),
        V((S // 2, D), U32),
        V((2, S // 2, D), U32),
        V((S // 2, D), U32),
        V((M, S), F32),
        V((1, S), F32),
        V((1, S), F32),
        V((M,), BF),
        V((M,), BF),
        V((M // 2, F), U32),
        V((M // 2, F), U32),
        V((M // 2, F), U32),
        V((8, TQ), F32),
        pltpu.SMEM((2,), I32),
        V((2, M, TQ), F32),
        V((2, M, TQ), F32),
        V((5, S // 4, HC), U32),
        V((7, S // 4, PR), U32),
        V((7, S // 4, TQ), U32),
        V((7, S // 4, TQ), U32),
        V((7, S // 4, TQ), U32),
        V((7, S // 4, TQ), U32),
        V((M, S), BF),
        pltpu.SemaphoreType.DMA((NSEM,)),
    ]
    outT = pl.pallas_call(
        _kernel,
        in_specs=[pl.BlockSpec(memory_space=pl.ANY)] * 11,
        out_specs=pl.BlockSpec(memory_space=pl.ANY),
        out_shape=jax.ShapeDtypeStruct((M, S), BF),
        scratch_shapes=scratch,
        compiler_params=pltpu.CompilerParams(
            vmem_limit_bytes=100 * 1024 * 1024),
    )(xT, ckv, A_w_q, A_w_uk, A_w_uv, woT, B_w_r, B_w_gate, B_w_up, wdT, gate_w)
    return outT.T.reshape(1, S, M)
```

```python
import math

import jax
import jax.numpy as jnp
from jax import lax
import jax.experimental.pallas as pl
import jax.experimental.pallas.tpu as pltpu

S, M, C, H, D, F = 2048, 448, 1024, 16, 256, 1792
TQ = 128
PR = 2 * TQ
NP = S // PR
PB = 512
NPB = S // PB
NF = F // TQ
HB, HC = PB // 2, C // 2
MP = 512
TW = TQ // 2

BF, F32, U32, I32 = jnp.bfloat16, jnp.float32, jnp.uint32, jnp.int32
NN = (((1,), (0,)), ((), ()))
NT = (((1,), (1,)), ((), ()))
LOG2E = math.log2(math.e)
QSCALE = (D ** -0.5) * LOG2E
NEG = -1e9 * LOG2E
HI16 = 0xFFFF0000

S_WK, S_WV, S_HEAD0, S_HEAD1, S_BULK, S_OUT, S_CKV = range(7)
NSEM = S_CKV + NPB

_PLAN = {
    "first": (
        "T0,T1,T2,GB1,GB0,T3,Q0.1,Q0,SB0,SA1,SA0,Q1,SB1,G8,"
        "PB0,PA0,SA2,PB1,G9,SB2,G10,PA1,G11,SS3.1,SS3.1,SD3,"
        "SS3,G12,PA2,O0,Q2,PB2,G13,G14,SS5.4,SD4,PB3,G15,SS4,"
        "PA3,SS5,PB4,SD5,O1,Q3,SS6.4,SS6.1,TOPK0,SD6,PD5,SS6,"
        "PA4,PS5,V3.1,SS7,V3.4,SD7,V3,PS6,PD7,PD6,O2,PS7,O3"),
    "loop": (
        "K0.4,K0.2,Q0,K0,V0,SS1,SA0,K1.5,SD1,SB0,K1,V1.4,FV0,"
        "V1,PA0,Q1,SD2,PS1,SS2,PB0,K2.2,PD1,SS3.1,PD2,SS3,SD3,"
        "V2.1,K2,V2.4,V2.1,PS2,O0,V2,Q2.1,Q2.3,Q2,SS4.1,SS4,"
        "SS5,SD4,PS3,SD5,K3.1,V3.5,K3,PD3,PD4,Q3.5,Q3,SS6.4,"
        "PS4.1,PS5.5,PS4,PS5.1,SS6,O1,V3,PD5,SD6,SS7,PS6,PS5,"
        "PD6,SD7,O2,PS7.4,PS7.2,PD7,PS7,O3"),
    "o0": "3641025",
    "fK": "4103625", "fV": "4250613", "fQ": "3614025", "fS": "0136425", "fP": "2014356", "fO": "4032615",
    "oK": "4103625", "oV": "4061523", "oQ": "2465301", "oS": "0136425", "oP": "2054613",
    "oO": "0413625",
    "fhyb": 14, "hyb": 14, "fsto": 1, "sto": 2,
    "fhold": "", "hold": "ck",
}


def _items(txt):
    out = []
    for t in txt.split(","):
        t, _, cnt = t.partition(".")
        kind = t.rstrip("0123456789")
        out.append((kind, int(t[len(kind):]), int(cnt or 0)))
    return out


def _digits(txt):
    return [int(c) for c in txt]


def _dot(a, b, dn):
    return lax.dot_general(a, b, dn, preferred_element_type=F32)


def _cat(xs, axis):
    return xs[0] if len(xs) == 1 else jnp.concatenate(xs, axis=axis)


def _recip(l):
    r = pl.reciprocal(l, approx=True)
    return r * (2.0 - l * r)


def _sigmoid(z):
    return 1.0 / (1.0 + jnp.exp(-z))


def _bf(w):
    return pltpu.bitcast(w, BF)


def _u32(v):
    return pltpu.bitcast(v.astype(BF), U32)


def _rows(ref, r0, r1):
    return _bf(ref[r0 // 2:r1 // 2, :])


def _put_rows(ref, r0, r1, v):
    ref[r0 // 2:r1 // 2, :] = _u32(v)


def _lhs_terms(a11, a12, a21, a22):
    return [a11 + a22, a21 + a22, a11, a22, a11 + a12, a21 - a11, a12 - a22]


def _rhs_terms(b11, b12, b21, b22):
    return [b11 + b22, b11, b12 - b22, b21 - b11, b22, b11 + b12, b21 + b22]


def _quads(f):
    k, n = f.shape[0] // 2, f.shape[1] // 2
    return f[:k, :n], f[:k, n:], f[k:, :n], f[k:, n:]


def _combine(m):
    return (m[0] + m[3] - m[4] + m[6], m[2] + m[4],
            m[1] + m[3], m[0] - m[1] + m[2] + m[5])


LSUMS = (0, 1, 4, 5, 6)
RSUMS = (0, 2, 3, 5, 6)


def _token_block(idx):
    start = jnp.clip(idx // TQ * TQ, 0, S - TQ)
    return pl.ds(pl.multiple_of(start, TQ), TQ)


def _kernel(xT_hbm, ckv_hbm, wq_hbm, wk_hbm, wv_hbm, wo_hbm, wr_hbm, wg_hbm,
            wu_hbm, wd_hbm, gw_hbm, out_hbm,
            xT_s, x_s, ckv_s, wq32, wkv32, wo_s, q_s, kv_s, ctx_s, acc,
            r_s, g_s, wr_s, gw_s, wg_s, wu_s, wd_s, sig_s, idx_s, xcol_s, ypart_s,
            asum_s, xsum_s, qt_s, kt_s, vt_s, ct_s, out_s, sem):
    wk32, wv32 = wkv32.at[0], wkv32.at[1]
    k_s, v_s = kv_s.at[0], kv_s.at[1]
    (xT_u, ckv_u, wq_u, wk_u, wv_u, wo_u, wg_u, wu_u, wd_u) = (
        r.bitcast(U32) for r in (xT_hbm, ckv_hbm, wq_hbm, wk_hbm, wv_hbm,
                                 wo_hbm, wg_hbm, wu_hbm, wd_hbm))

    def cp(src, dst, s):
        return pltpu.make_async_copy(src, dst, sem.at[s])

    def cp_pair(w_u, w_s, p, s):
        return cp(w_u.at[:, p, :], w_s.at[p], s)

    def cp_ckv(i):
        r = pl.ds(pl.multiple_of(PB // 2 * i, PB // 2), PB // 2)
        return cp(ckv_u.at[r, :], ckv_s.at[r, :], S_CKV + i)

    def cp_out(c0, c1):
        r = pl.ds(c0, c1 - c0)
        return cp(out_s.at[:, r], out_hbm.at[:, r], S_OUT)

    def out_blocks(i):
        r0, r1 = PB * i, PB * (i + 1)
        return [(r0, r1)] if i < NPB - 1 else [(r0, r0 + PR), (r0 + PR, r1)]

    c_wk, c_wv = cp_pair(wk_u, wk32, 0, S_WK), cp_pair(wv_u, wv32, 0, S_WV)
    head0 = [cp(xT_u, xT_s, S_HEAD0), cp_pair(wq_u, wq32, 0, S_HEAD0),
             cp(wr_hbm, wr_s, S_HEAD0), cp(gw_hbm, gw_s, S_HEAD0),
             cp(wo_u.at[0], wo_s.at[0], S_HEAD0)]
    head1 = [cp(wo_u.at[1], wo_s.at[1], S_HEAD1), cp(wg_u, wg_s, S_HEAD1),
             cp(wu_u, wu_s, S_HEAD1), cp(wd_u, wd_s, S_HEAD1)]
    rest = pl.ds(2, H - 2)
    bulk = [cp(wo_u.at[rest], wo_s.at[rest], S_BULK)]
    for p in range(1, H // 2):
        bulk += [cp_pair(wk_u, wk32, p, S_BULK), cp_pair(wv_u, wv32, p, S_BULK),
                 cp_pair(wq_u, wq32, p, S_BULK)]

    row = lax.broadcasted_iota(I32, (TQ, TQ), 0)
    col = lax.broadcasted_iota(I32, (TQ, TQ), 1)
    tri = col <= row

    def head(h, first):
        pre = "f" if first else "o"
        order = _items(_PLAN["first" if first else "loop"])
        kinds = {(k, i) for k, i, _ in order}
        hyb = _PLAN["fhyb" if first else "hyb"]
        sto = _PLAN["fsto" if first else "sto"]
        hold = _PLAN["fhold" if first else "hold"]
        if first:
            pair, shift = 0, jnp.uint32(16)
        else:
            pair = lax.shift_right_logical(h, 1)
            shift = (16 - 16 * (h & 1)).astype(U32)
        cache, prog, held = {}, {}, {}
        scores, probs_of, ctx_of, rinv = {}, {}, {}, {}

        def wterms(name):
            if name not in cache:
                if name == "O":
                    f = _bf(wo_s[h]).astype(F32)
                    cache[name] = [t.astype(BF) for t in _lhs_terms(*_quads(f))]
                else:
                    ref = {"K": wk32, "V": wv32, "Q": wq32}[name]
                    f = pltpu.bitcast((ref[pair] << shift) & jnp.uint32(HI16), F32)
                    if name == "Q":
                        f = jnp.concatenate([f, jnp.zeros((MP - M, D), F32)], axis=0)
                    cache[name] = [t.astype(BF) for t in _rhs_terms(*_quads(f))]
            return cache[name]

        def term(name, n, j0, j1):
            ref, plain, raw = {"q": (qt_s, q_s, (2, 3)), "k": (kt_s, k_s, (1, 4)),
                               "v": (vt_s, v_s, (1, 4)), "c": (ct_s, None, ())}[name]
            if n in raw:
                odd = raw.index(n)
                return _bf(_cat([plain[TW * (2 * j + odd):TW * (2 * j + odd + 1),
                                       TQ * odd:TQ * (odd + 1)]
                                 for j in range(j0, j1)], 0))
            if first and name in "kv":
                for j in range(j0, j1):
                    if (name, n, j) not in held:
                        f = _rows(plain, PR * j, PR * (j + 1)).astype(F32)
                        f11, f12, f21, f22 = _quads(f)
                        tt = (_rhs_terms(f11, f21, f12, f22) if name == "k"
                              else _rhs_terms(f11, f12, f21, f22))
                        for u in RSUMS:
                            held[name, u, j] = tt[u].astype(BF)
            if (name, n, j0) in held:
                return _cat([held[name, n, j] for j in range(j0, j1)], 0)
            return _bf(ref[n, TW * j0:TW * j1, :])

        def put_terms(name, j, terms, which):
            ref = {"q": qt_s, "k": kt_s, "v": vt_s, "c": ct_s}[name]
            for n in which:
                if name in hold:
                    held[name, n, j] = terms[n].astype(BF)
                else:
                    ref[n, TW * j:TW * (j + 1), :] = _u32(terms[n])

        def run(key, cnt, product):
            m = prog.setdefault(key, {})
            todo = [n for n in _digits(_PLAN[pre + key[0]]) if n not in m]
            for n in (todo[:cnt] if cnt else todo):
                m[n] = product(n)
            return len(m) == 7

        def route(c0, c1):
            if "rg" not in cache:
                r16 = lax.broadcasted_iota(I32, (16, M), 0)
                wr = wr_s[...].astype(F32).reshape(1, M)
                gw = gw_s[...].astype(F32).reshape(1, M)
                cache["rg"] = jnp.where(
                    r16 == 0, wr, jnp.where(r16 == 1, gw, 0.0)).astype(BF)
            rg = _dot(cache["rg"], _bf(xT_s[:, c0:c1]), NN)
            r_s[:, c0:c1] = rg[0:1, :].astype(BF).astype(F32)
            g_s[:, c0:c1] = _sigmoid(rg[1:2, :])

        def set_scores(q, t0, s):
            for t in range(s.shape[1] // TQ):
                blk = s[:, TQ * t:TQ * (t + 1)]
                scores.setdefault(q, {})[t0 + t] = (
                    jnp.where(tri, blk, NEG) if t0 + t == q else blk)

        def probs(q, perm):
            if q not in probs_of:
                tiles = scores.pop(q)
                s = _cat([tiles[t] for t in perm], 1)
                probs_of[q] = jnp.exp2(s - jnp.max(s, axis=1, keepdims=True))
            return probs_of[q]

        def finish(q, o, src):
            if q < hyb:
                rinv[q] = None
                o = o * _recip(jnp.sum(src, axis=1, keepdims=True))
            else:
                la = src[:, 0:TQ]
                for t in range(1, src.shape[1] // TQ):
                    la = la + src[:, TQ * t:TQ * (t + 1)]
                hi = la.astype(BF)
                lo = (la - hi.astype(F32)).astype(BF)
                l = _dot(jnp.ones((16, 2 * TQ), BF),
                         jnp.concatenate([hi, lo], axis=1), NT)[0:1, :]
                rinv[q] = _recip(l)
            i = q // 2
            if i // 2 < sto and 2 * i + 1 < hyb:
                ctx_of[q] = o
                if 2 * i in ctx_of and 2 * i + 1 in ctx_of:
                    oa, ob = ctx_of.pop(2 * i), ctx_of.pop(2 * i + 1)
                    put_terms("c", i, _rhs_terms(oa[:, :TQ], ob[:, :TQ],
                                                 oa[:, TQ:], ob[:, TQ:]), range(7))
            else:
                _put_rows(ctx_s, TQ * q, TQ * (q + 1), o)

        for kind, i, cnt in order:
            r0, r1 = PB * i, PB * (i + 1)
            n0 = PR * i
            qa, qb = 2 * i, 2 * i + 1
            if kind == "T":
                _put_rows(x_s, r0, r1, _bf(xT_s[:, r0:r1]).T)
            elif kind == "GB":
                route(r0, r1)
            elif kind == "G":
                route(TQ * i, TQ * (i + 1))
            elif kind in ("K", "V", "Q"):
                w0, w1 = HB * i // 2, HB * (i + 1) // 2
                if first and kind == "Q" and ("x", i) not in cache:
                    z = jnp.zeros((HB, MP - M), F32)
                    at = jnp.concatenate([_rows(x_s, r0, r0 + HB).astype(F32), z], axis=1)
                    ab = jnp.concatenate([_rows(x_s, r0 + HB, r1).astype(F32), z], axis=1)
                    tt = _lhs_terms(at[:, :PR], at[:, PR:], ab[:, :PR], ab[:, PR:])
                    cache["x", i] = {n: tt[n].astype(BF) for n in range(7) if n != 2}
                    for n, v in cache["x", i].items():
                        xsum_s[n, w0:w1, :] = pltpu.bitcast(v, U32)

                def lhs(n):
                    if kind == "Q":
                        if n == 2:
                            return _bf(x_s[r0 // 2:(r0 + HB) // 2, :PR])
                        return cache["x", i][n] if first else _bf(xsum_s[n, w0:w1, :])
                    if n == 2:
                        return _bf(ckv_s[r0 // 2:(r0 + HB) // 2, :HC])
                    if n == 3:
                        return _bf(ckv_s[(r0 + HB) // 2:r1 // 2, HC:])
                    return _bf(asum_s[LSUMS.index(n), w0:w1, :])
                if not run((kind, i), cnt, lambda n: _dot(lhs(n), wterms(kind)[n], NN)):
                    continue
                res = _combine(prog.pop((kind, i)))
                if kind == "Q":
                    res = [c * QSCALE for c in res]
                dst = {"K": k_s, "V": v_s, "Q": q_s}[kind]
                for j, (c0, c1) in ((2 * i, res[:2]), (2 * i + 1, res[2:])):
                    _put_rows(dst, PR * j, PR * (j + 1), jnp.concatenate([c0, c1], axis=1))
                    later = range(j + 1, NP) if not first else ()
                    if kind == "V" and any(("PS", u) in kinds for u in later):
                        put_terms("v", j, _rhs_terms(c0[:TQ], c1[:TQ], c0[TQ:], c1[TQ:]), RSUMS)
                    if kind == "K" and any(("SS", u) in kinds for u in later):
                        put_terms("k", j, _rhs_terms(c0[:TQ], c0[TQ:], c1[:TQ], c1[TQ:]), RSUMS)
                    if kind == "Q" and ("SS", j) in kinds:
                        put_terms("q", j, _lhs_terms(c0[:TQ], c1[:TQ], c0[TQ:], c1[TQ:]), LSUMS)
            elif kind in ("SA", "SB"):
                q = qa if kind == "SA" else qb
                set_scores(q, 0, _dot(_rows(q_s, TQ * q, TQ * (q + 1)),
                                      _rows(k_s, 0, TQ * (q + 1)), NT))
            elif kind == "SD":
                for q in (qa, qb):
                    set_scores(q, qa, _dot(_rows(q_s, TQ * q, TQ * (q + 1)),
                                           _rows(k_s, n0, TQ * (q + 1)), NT))
            elif kind == "SS":
                qts = [term("q", n, i, i + 1) for n in range(7)]
                j0 = prog.get(("SS", i), 0)
                prog["SS", i] = j1 = min(i, j0 + cnt) if cnt else i
                for j in range(j0, j1):
                    cs = _combine({n: _dot(qts[n], term("k", n, j, j + 1), NT)
                                   for n in _digits(_PLAN[pre + "S"])})
                    scores.setdefault(qa, {}).update({2 * j: cs[0], 2 * j + 1: cs[1]})
                    scores.setdefault(qb, {}).update({2 * j: cs[2], 2 * j + 1: cs[3]})
            elif kind in ("PA", "PB"):
                q = qa if kind == "PA" else qb
                p = probs(q, range(q + 1)).astype(BF)
                probs_of.pop(q)
                finish(q, _dot(p, _rows(v_s, 0, TQ * (q + 1)), NN), p.astype(F32))
            elif kind in ("PS", "PD"):
                w = TQ * i
                eo = list(range(0, qa, 2)) + list(range(1, qa, 2))
                pa, pb = probs(qa, eo + [qa]), probs(qb, eo + [qa, qb])
                if ("diag", i) not in prog:
                    prog["diag", i] = (pa[:, 2 * w:].astype(BF), pb[:, 2 * w:].astype(BF))
                da, db = prog["diag", i]
                if kind == "PD":
                    prog["PD", i] = (_dot(da, _rows(v_s, n0, n0 + TQ), NN),
                                     _dot(db, _rows(v_s, n0, n0 + PR), NN))
                else:
                    if ("L", i) not in prog:
                        prog["L", i] = [t.astype(BF) for t in _lhs_terms(
                            pa[:, :w], pa[:, w:2 * w], pb[:, :w], pb[:, w:2 * w])]
                    if not run(("P", i), cnt, lambda n: _dot(
                            prog["L", i][n], term("v", n, 0, i), NN)):
                        continue
                if ("PD", i) in prog and len(prog.get(("P", i), ())) == 7:
                    c11, c12, c21, c22 = _combine(prog.pop(("P", i)))
                    oa, ob = prog.pop(("PD", i))
                    lt = prog.pop(("L", i))
                    oa = jnp.concatenate([c11, c12], axis=1) + oa
                    ob = jnp.concatenate([c21, c22], axis=1) + ob
                    for q, o, lo_, d in ((qa, oa, lt[4], da), (qb, ob, lt[1], db)):
                        probs_of.pop(q)
                        finish(q, o, jnp.concatenate([lo_, d], axis=1).astype(F32))
            elif kind == "O":
                j0, j1 = 2 * i, 2 * i + 2
                js = max(j0, min(j1, hyb // 2)) if i < sto else j0
                cols = []
                if js > j0:
                    c11, c12, c21, c22 = _combine(
                        {n: _dot(wterms("O")[n], term("c", n, j0, js), NT)
                         for n in _digits(_PLAN[pre + "O"])})
                    ca = jnp.concatenate([c11, c21], axis=0)
                    cb = jnp.concatenate([c12, c22], axis=0)
                    for t in range(js - j0):
                        cols += [ca[:, TQ * t:TQ * (t + 1)], cb[:, TQ * t:TQ * (t + 1)]]
                if j1 > js:
                    cols.append(_dot(_bf(wo_s[h]), _rows(ctx_s, PR * js, PR * j1), NT))
                g = g_s[:, r0:r1]
                f = []
                for t in range(4):
                    gt, rt = g[:, TQ * t:TQ * (t + 1)], rinv.pop(4 * i + t)
                    f.append(gt if rt is None else gt * rt)
                a = _cat(cols, 1) * jnp.concatenate(f, axis=1)
                if first:
                    acc[:, r0:r1] = a + (1.0 - g) * _bf(xT_s[:, r0:r1]).astype(F32)
                else:
                    a = acc[:, r0:r1] + a
                    acc[:, r0:r1] = a
                    for c0, c1 in out_blocks(i):
                        out_s[:, c0:c1] = a[:, c0 - r0:c1 - r0].astype(BF)

                        @pl.when(h == H - 1)
                        def _():
                            cp_out(c0, c1).start()
            elif kind == "TOPK":
                r = r_s[...]
                lane = lax.broadcasted_iota(I32, (1, S), 1)
                m1 = jnp.max(r, axis=1, keepdims=True)
                i1 = jnp.min(jnp.where(r == m1, lane, S - 1))
                r2 = jnp.where(lane == i1, -jnp.inf, r)
                m2 = jnp.max(r2, axis=1, keepdims=True)
                i2 = jnp.min(jnp.where((r2 == m2) & (lane != i1), lane, S - 1))
                r8 = lax.broadcasted_iota(I32, (8, TQ), 0)
                sig_s[...] = jnp.where(r8 == 0, _sigmoid(m1), _sigmoid(m2))
                lane = lax.broadcasted_iota(I32, (1, TQ), 1)
                for t, idx in enumerate((i1, i2)):
                    idx_s[t] = idx
                    xb = _bf(xT_s[:, _token_block(idx)]).astype(F32)
                    xc = jnp.sum(jnp.where(lane == idx % TQ, xb, 0.0),
                                 axis=1, keepdims=True)
                    xcol_s[t] = jnp.broadcast_to(xc, (M, TQ))
                ypart_s[...] = jnp.zeros_like(ypart_s)
            elif kind == "FV":
                chunk = jnp.minimum(h - 1, NF - 1)
                c = pl.ds(pl.multiple_of(chunk * TQ, TQ), TQ)
                wg, wu, wd = (_bf(w[:, c]).astype(F32) for w in (wg_s, wu_s, wd_s))
                for t in range(2):
                    xc = xcol_s[t]
                    g = jnp.sum(xc * wg, axis=0, keepdims=True)
                    u = jnp.sum(xc * wu, axis=0, keepdims=True)
                    ypart_s[t] += wd * (g * _sigmoid(g) * u)
            else:
                raise ValueError(kind)
        assert not (scores or probs_of or ctx_of or rinv)

    for c in [cp_ckv(0), c_wk, c_wv] + [cp_ckv(i) for i in range(1, NPB)]:
        c.start()
    for c in head0 + head1 + bulk:
        c.start()

    def proj0(t, carry):
        which, blk = t % 2, t // 2
        base = pl.multiple_of(blk * (PB // 2), PB // 2)
        half = pl.multiple_of(blk * (HB // 2), HB // 2)

        @pl.when(which == 0)
        def _():
            cp_ckv(blk).wait()

        @pl.when(t == 0)
        def _():
            c_wk.wait()

        @pl.when(t == 1)
        def _():
            c_wv.wait()

        top, bot = pl.ds(base, HB // 2), pl.ds(base + HB // 2, HB // 2)
        at, ab = _bf(ckv_s[top, :]).astype(F32), _bf(ckv_s[bot, :]).astype(F32)
        tt = _lhs_terms(at[:, :HC], at[:, HC:], ab[:, :HC], ab[:, HC:])
        lhs = {n: tt[n].astype(BF) for n in LSUMS}
        for k, n in enumerate(LSUMS):
            asum_s[k, pl.ds(half, HB // 2), :] = pltpu.bitcast(lhs[n], U32)
        lhs[2], lhs[3] = _bf(ckv_s[top, :HC]), _bf(ckv_s[bot, HC:])
        f = pltpu.bitcast(wkv32[which, 0] << 16, F32)
        rhs = [u.astype(BF) for u in _rhs_terms(*_quads(f))]
        c11, c12, c21, c22 = _combine(
            {n: _dot(lhs[n], rhs[n], NN) for n in _digits(_PLAN["o0"])})
        kv_s[which, top, :] = _u32(jnp.concatenate([c11, c12], axis=1))
        kv_s[which, bot, :] = _u32(jnp.concatenate([c21, c22], axis=1))
        return carry

    def step(h, carry):
        @pl.when(h == 2)
        def _():
            for c in bulk:
                c.wait()

        @pl.when(h == H - 1)
        def _():
            lane = lax.broadcasted_iota(I32, (1, TQ), 1)
            for t in range(2):
                idx = idx_s[t]
                y = jnp.sum(ypart_s[t], axis=1, keepdims=True) * sig_s[t:t + 1, :]
                blk = _token_block(idx)
                old = acc[:, blk]
                acc[:, blk] = jnp.where(
                    lane == idx % TQ, old + (1.0 - g_s[:, blk]) * y, old)

        head(h, False)
        return carry

    left = {(k, i) for k, i, _ in _items(_PLAN["first"]) if k in ("K", "V")}
    lax.fori_loop(0, 2 * NPB - len(left), proj0, 0)
    for c in head0:
        c.wait()
    head(0, True)
    for c in head1:
        c.wait()
    lax.fori_loop(1, H, step, 0)
    for i in range(NPB):
        for c0, c1 in out_blocks(i):
            cp_out(c0, c1).wait()


@jax.jit
def pallas_gated_mix__compressed_kv_cla__moe_arch_mod__prompt_kernel(
    A_x: jax.Array,
    A_c_kv: jax.Array,
    A_w_q: jax.Array,
    A_w_uk: jax.Array,
    A_w_uv: jax.Array,
    A_w_o: jax.Array,
    B_x: jax.Array,
    B_w_r: jax.Array,
    B_w_gate: jax.Array,
    B_w_up: jax.Array,
    B_w_down: jax.Array,
    gate_w: jax.Array,
):
    del B_x
    xT = A_x.reshape(S, M).T
    ckv = A_c_kv.reshape(S, C)
    woT = jnp.transpose(A_w_o, (0, 2, 1))
    wdT = B_w_down.T

    V = pltpu.VMEM
    scratch = [
        V((M // 2, S), U32),
        V((S // 2, M), U32),
        V((S // 2, C), U32),
        V((H // 2, M, D), U32),
        V((2, H // 2, C, D), U32),
        V((H, M // 2, D), U32),
        V((S // 2, D), U32),
        V((2, S // 2, D), U32),
        V((S // 2, D), U32),
        V((M, S), F32),
        V((1, S), F32),
        V((1, S), F32),
        V((M,), BF),
        V((M,), BF),
        V((M // 2, F), U32),
        V((M // 2, F), U32),
        V((M // 2, F), U32),
        V((8, TQ), F32),
        pltpu.SMEM((2,), I32),
        V((2, M, TQ), F32),
        V((2, M, TQ), F32),
        V((5, S // 4, HC), U32),
        V((7, S // 4, PR), U32),
        V((7, S // 4, TQ), U32),
        V((7, S // 4, TQ), U32),
        V((7, S // 4, TQ), U32),
        V((7, S // 4, TQ), U32),
        V((M, S), BF),
        pltpu.SemaphoreType.DMA((NSEM,)),
    ]
    outT = pl.pallas_call(
        _kernel,
        in_specs=[pl.BlockSpec(memory_space=pl.ANY)] * 11,
        out_specs=pl.BlockSpec(memory_space=pl.ANY),
        out_shape=jax.ShapeDtypeStruct((M, S), BF),
        scratch_shapes=scratch,
        compiler_params=pltpu.CompilerParams(
            vmem_limit_bytes=100 * 1024 * 1024),
    )(xT, ckv, A_w_q, A_w_uk, A_w_uv, woT, B_w_r, B_w_gate, B_w_up, wdT, gate_w)
    return outT.T.reshape(1, S, M)
```

```python
import math

import jax
import jax.numpy as jnp
from jax import lax
import jax.experimental.pallas as pl
import jax.experimental.pallas.tpu as pltpu

S, M, C, H, D, F = 2048, 448, 1024, 16, 256, 1792
TQ = 128
PR = 2 * TQ
NP = S // PR
PB = 512
NPB = S // PB
NF = F // TQ
HB, HC = PB // 2, C // 2
MP = 512
TW = TQ // 2

BF, F32, U32, I32 = jnp.bfloat16, jnp.float32, jnp.uint32, jnp.int32
NN = (((1,), (0,)), ((), ()))
NT = (((1,), (1,)), ((), ()))
LOG2E = math.log2(math.e)
QSCALE = (D ** -0.5) * LOG2E
NEG = -1e9 * LOG2E
HI16 = 0xFFFF0000

S_WK, S_WV, S_HEAD0, S_HEAD1, S_BULK, S_OUT, S_CKV = range(7)
NSEM = S_CKV + NPB

_PLAN = {
    "first": (
        "T2,T1,T3,T0,V3.2,GB1,GB0,Q0.1,Q0,SB0,SA1,SA0,Q1,SB1,"
        "PA0,PB0,SA2,G8,PB1,G9,SB2,G10,PA1,G11,SS3.1,SS3.1,SD3,"
        "SS3,G12,PA2,O0,Q2.2,Q2,PB2,G13,G14,SS5.4,SD4,PB3,G15,"
        "SS4,PA3,SS5,PB4,SD5,O1,Q3,SS6.1,TOPK0,SD6,PD5,SS6.4,"
        "SS6,V3.2,PA4,PS5,SS7.4,SS7.2,SS7,PS6.3,V3.1,SD7,V3,PS6,"
        "PD7,PD6,O2,PS7.6,PS7,O3"),
    "loop": (
        "K0.4,K0.2,Q0,K0,V0,SS1,SA0,K1.5,SD1,SB0,K1,V1.4,FV0,"
        "V1,PA0,Q1,SD2,PS1,SS2,PB0,K2.2,PD1,SS3.1,PD2,SS3,SD3,"
        "V2.1,K2,V2.4,V2.1,PS2,O0,V2,Q2.1,Q2.3,Q2,SS4.1,SS4,"
        "SS5,SD4,PS3,SD5,K3.1,V3.5,K3,PD3,PD4,Q3.5,Q3,SS6.4,"
        "PS4.1,PS5.5,PS4,PS5.1,SS6,O1,V3,PD5,SD6,SS7,PS6,PS5,"
        "PD6,SD7,O2,PS7.4,PS7.2,PD7,PS7,O3"),
    "o0": "3641025",
    "fK": "4103625", "fV": "4253610", "fQ": "3614025", "fS": "0136425", "fP": "2014653", "fO": "4132605",
    "oK": "4103625", "oV": "4061523", "oQ": "2465301", "oS": "0136425", "oP": "2054613",
    "oO": "0413625",
    "fhyb": 14, "hyb": 14, "fsto": 1, "sto": 2,
    "fhold": "", "hold": "ck",
}


def _items(txt):
    out = []
    for t in txt.split(","):
        t, _, cnt = t.partition(".")
        kind = t.rstrip("0123456789")
        out.append((kind, int(t[len(kind):]), int(cnt or 0)))
    return out


def _digits(txt):
    return [int(c) for c in txt]


def _dot(a, b, dn):
    return lax.dot_general(a, b, dn, preferred_element_type=F32)


def _cat(xs, axis):
    return xs[0] if len(xs) == 1 else jnp.concatenate(xs, axis=axis)


def _recip(l):
    r = pl.reciprocal(l, approx=True)
    return r * (2.0 - l * r)


def _sigmoid(z):
    return 1.0 / (1.0 + jnp.exp(-z))


def _bf(w):
    return pltpu.bitcast(w, BF)


def _u32(v):
    return pltpu.bitcast(v.astype(BF), U32)


def _rows(ref, r0, r1):
    return _bf(ref[r0 // 2:r1 // 2, :])


def _put_rows(ref, r0, r1, v):
    ref[r0 // 2:r1 // 2, :] = _u32(v)


def _lhs_terms(a11, a12, a21, a22):
    return [a11 + a22, a21 + a22, a11, a22, a11 + a12, a21 - a11, a12 - a22]


def _rhs_terms(b11, b12, b21, b22):
    return [b11 + b22, b11, b12 - b22, b21 - b11, b22, b11 + b12, b21 + b22]


def _quads(f):
    k, n = f.shape[0] // 2, f.shape[1] // 2
    return f[:k, :n], f[:k, n:], f[k:, :n], f[k:, n:]


def _combine(m):
    return (m[0] + m[3] - m[4] + m[6], m[2] + m[4],
            m[1] + m[3], m[0] - m[1] + m[2] + m[5])


LSUMS = (0, 1, 4, 5, 6)
RSUMS = (0, 2, 3, 5, 6)


def _token_block(idx):
    start = jnp.clip(idx // TQ * TQ, 0, S - TQ)
    return pl.ds(pl.multiple_of(start, TQ), TQ)


def _kernel(xT_hbm, ckv_hbm, wq_hbm, wk_hbm, wv_hbm, wo_hbm, wr_hbm, wg_hbm,
            wu_hbm, wd_hbm, gw_hbm, out_hbm,
            xT_s, x_s, ckv_s, wq32, wkv32, wo_s, q_s, kv_s, ctx_s, acc,
            r_s, g_s, wr_s, gw_s, wg_s, wu_s, wd_s, sig_s, idx_s, xcol_s, ypart_s,
            asum_s, xsum_s, qt_s, kt_s, vt_s, ct_s, out_s, sem):
    wk32, wv32 = wkv32.at[0], wkv32.at[1]
    k_s, v_s = kv_s.at[0], kv_s.at[1]
    (xT_u, ckv_u, wq_u, wk_u, wv_u, wo_u, wg_u, wu_u, wd_u) = (
        r.bitcast(U32) for r in (xT_hbm, ckv_hbm, wq_hbm, wk_hbm, wv_hbm,
                                 wo_hbm, wg_hbm, wu_hbm, wd_hbm))

    def cp(src, dst, s):
        return pltpu.make_async_copy(src, dst, sem.at[s])

    def cp_pair(w_u, w_s, p, s):
        return cp(w_u.at[:, p, :], w_s.at[p], s)

    def cp_ckv(i):
        r = pl.ds(pl.multiple_of(PB // 2 * i, PB // 2), PB // 2)
        return cp(ckv_u.at[r, :], ckv_s.at[r, :], S_CKV + i)

    def cp_out(c0, c1):
        r = pl.ds(c0, c1 - c0)
        return cp(out_s.at[:, r], out_hbm.at[:, r], S_OUT)

    def out_blocks(i):
        r0, r1 = PB * i, PB * (i + 1)
        return [(r0, r1)] if i < NPB - 1 else [(r0, r0 + PR), (r0 + PR, r1)]

    c_wk, c_wv = cp_pair(wk_u, wk32, 0, S_WK), cp_pair(wv_u, wv32, 0, S_WV)
    head0 = [cp(xT_u, xT_s, S_HEAD0), cp_pair(wq_u, wq32, 0, S_HEAD0),
             cp(wr_hbm, wr_s, S_HEAD0), cp(gw_hbm, gw_s, S_HEAD0),
             cp(wo_u.at[0], wo_s.at[0], S_HEAD0)]
    head1 = [cp(wo_u.at[1], wo_s.at[1], S_HEAD1), cp(wg_u, wg_s, S_HEAD1),
             cp(wu_u, wu_s, S_HEAD1), cp(wd_u, wd_s, S_HEAD1)]
    rest = pl.ds(2, H - 2)
    bulk = [cp(wo_u.at[rest], wo_s.at[rest], S_BULK)]
    for p in range(1, H // 2):
        bulk += [cp_pair(wk_u, wk32, p, S_BULK), cp_pair(wv_u, wv32, p, S_BULK),
                 cp_pair(wq_u, wq32, p, S_BULK)]

    row = lax.broadcasted_iota(I32, (TQ, TQ), 0)
    col = lax.broadcasted_iota(I32, (TQ, TQ), 1)
    tri = col <= row

    def head(h, first):
        pre = "f" if first else "o"
        order = _items(_PLAN["first" if first else "loop"])
        kinds = {(k, i) for k, i, _ in order}
        hyb = _PLAN["fhyb" if first else "hyb"]
        sto = _PLAN["fsto" if first else "sto"]
        hold = _PLAN["fhold" if first else "hold"]
        if first:
            pair, shift = 0, jnp.uint32(16)
        else:
            pair = lax.shift_right_logical(h, 1)
            shift = (16 - 16 * (h & 1)).astype(U32)
        cache, prog, held = {}, {}, {}
        scores, probs_of, ctx_of, rinv = {}, {}, {}, {}

        def wterms(name):
            if name not in cache:
                if name == "O":
                    f = _bf(wo_s[h]).astype(F32)
                    cache[name] = [t.astype(BF) for t in _lhs_terms(*_quads(f))]
                else:
                    ref = {"K": wk32, "V": wv32, "Q": wq32}[name]
                    f = pltpu.bitcast((ref[pair] << shift) & jnp.uint32(HI16), F32)
                    if name == "Q":
                        f = jnp.concatenate([f, jnp.zeros((MP - M, D), F32)], axis=0)
                    cache[name] = [t.astype(BF) for t in _rhs_terms(*_quads(f))]
            return cache[name]

        def term(name, n, j0, j1):
            ref, plain, raw = {"q": (qt_s, q_s, (2, 3)), "k": (kt_s, k_s, (1, 4)),
                               "v": (vt_s, v_s, (1, 4)), "c": (ct_s, None, ())}[name]
            if n in raw:
                odd = raw.index(n)
                return _bf(_cat([plain[TW * (2 * j + odd):TW * (2 * j + odd + 1),
                                       TQ * odd:TQ * (odd + 1)]
                                 for j in range(j0, j1)], 0))
            if first and name in "kv":
                for j in range(j0, j1):
                    if (name, n, j) not in held:
                        f = _rows(plain, PR * j, PR * (j + 1)).astype(F32)
                        f11, f12, f21, f22 = _quads(f)
                        tt = (_rhs_terms(f11, f21, f12, f22) if name == "k"
                              else _rhs_terms(f11, f12, f21, f22))
                        for u in RSUMS:
                            held[name, u, j] = tt[u].astype(BF)
            if (name, n, j0) in held:
                return _cat([held[name, n, j] for j in range(j0, j1)], 0)
            return _bf(ref[n, TW * j0:TW * j1, :])

        def put_terms(name, j, terms, which):
            ref = {"q": qt_s, "k": kt_s, "v": vt_s, "c": ct_s}[name]
            for n in which:
                if name in hold:
                    held[name, n, j] = terms[n].astype(BF)
                else:
                    ref[n, TW * j:TW * (j + 1), :] = _u32(terms[n])

        def run(key, cnt, product):
            m = prog.setdefault(key, {})
            todo = [n for n in _digits(_PLAN[pre + key[0]]) if n not in m]
            for n in (todo[:cnt] if cnt else todo):
                m[n] = product(n)
            return len(m) == 7

        def route(c0, c1):
            if "rg" not in cache:
                r16 = lax.broadcasted_iota(I32, (16, M), 0)
                wr = wr_s[...].astype(F32).reshape(1, M)
                gw = gw_s[...].astype(F32).reshape(1, M)
                cache["rg"] = jnp.where(
                    r16 == 0, wr, jnp.where(r16 == 1, gw, 0.0)).astype(BF)
            rg = _dot(cache["rg"], _bf(xT_s[:, c0:c1]), NN)
            r_s[:, c0:c1] = rg[0:1, :].astype(BF).astype(F32)
            g_s[:, c0:c1] = _sigmoid(rg[1:2, :])

        def set_scores(q, t0, s):
            for t in range(s.shape[1] // TQ):
                blk = s[:, TQ * t:TQ * (t + 1)]
                scores.setdefault(q, {})[t0 + t] = (
                    jnp.where(tri, blk, NEG) if t0 + t == q else blk)

        def probs(q, perm):
            if q not in probs_of:
                tiles = scores.pop(q)
                s = _cat([tiles[t] for t in perm], 1)
                probs_of[q] = jnp.exp2(s - jnp.max(s, axis=1, keepdims=True))
            return probs_of[q]

        def finish(q, o, src):
            if q < hyb:
                rinv[q] = None
                o = o * _recip(jnp.sum(src, axis=1, keepdims=True))
            else:
                la = src[:, 0:TQ]
                for t in range(1, src.shape[1] // TQ):
                    la = la + src[:, TQ * t:TQ * (t + 1)]
                hi = la.astype(BF)
                lo = (la - hi.astype(F32)).astype(BF)
                l = _dot(jnp.ones((16, 2 * TQ), BF),
                         jnp.concatenate([hi, lo], axis=1), NT)[0:1, :]
                rinv[q] = _recip(l)
            i = q // 2
            if i // 2 < sto and 2 * i + 1 < hyb:
                ctx_of[q] = o
                if 2 * i in ctx_of and 2 * i + 1 in ctx_of:
                    oa, ob = ctx_of.pop(2 * i), ctx_of.pop(2 * i + 1)
                    put_terms("c", i, _rhs_terms(oa[:, :TQ], ob[:, :TQ],
                                                 oa[:, TQ:], ob[:, TQ:]), range(7))
            else:
                _put_rows(ctx_s, TQ * q, TQ * (q + 1), o)

        for kind, i, cnt in order:
            r0, r1 = PB * i, PB * (i + 1)
            n0 = PR * i
            qa, qb = 2 * i, 2 * i + 1
            if kind == "T":
                _put_rows(x_s, r0, r1, _bf(xT_s[:, r0:r1]).T)
            elif kind == "GB":
                route(r0, r1)
            elif kind == "G":
                route(TQ * i, TQ * (i + 1))
            elif kind in ("K", "V", "Q"):
                w0, w1 = HB * i // 2, HB * (i + 1) // 2
                if first and kind == "Q" and ("x", i) not in cache:
                    z = jnp.zeros((HB, MP - M), F32)
                    at = jnp.concatenate([_rows(x_s, r0, r0 + HB).astype(F32), z], axis=1)
                    ab = jnp.concatenate([_rows(x_s, r0 + HB, r1).astype(F32), z], axis=1)
                    tt = _lhs_terms(at[:, :PR], at[:, PR:], ab[:, :PR], ab[:, PR:])
                    cache["x", i] = {n: tt[n].astype(BF) for n in range(7) if n != 2}
                    for n, v in cache["x", i].items():
                        xsum_s[n, w0:w1, :] = pltpu.bitcast(v, U32)

                def lhs(n):
                    if kind == "Q":
                        if n == 2:
                            return _bf(x_s[r0 // 2:(r0 + HB) // 2, :PR])
                        return cache["x", i][n] if first else _bf(xsum_s[n, w0:w1, :])
                    if n == 2:
                        return _bf(ckv_s[r0 // 2:(r0 + HB) // 2, :HC])
                    if n == 3:
                        return _bf(ckv_s[(r0 + HB) // 2:r1 // 2, HC:])
                    return _bf(asum_s[LSUMS.index(n), w0:w1, :])
                if not run((kind, i), cnt, lambda n: _dot(lhs(n), wterms(kind)[n], NN)):
                    continue
                res = _combine(prog.pop((kind, i)))
                if kind == "Q":
                    res = [c * QSCALE for c in res]
                dst = {"K": k_s, "V": v_s, "Q": q_s}[kind]
                for j, (c0, c1) in ((2 * i, res[:2]), (2 * i + 1, res[2:])):
                    _put_rows(dst, PR * j, PR * (j + 1), jnp.concatenate([c0, c1], axis=1))
                    later = range(j + 1, NP) if not first else ()
                    if kind == "V" and any(("PS", u) in kinds for u in later):
                        put_terms("v", j, _rhs_terms(c0[:TQ], c1[:TQ], c0[TQ:], c1[TQ:]), RSUMS)
                    if kind == "K" and any(("SS", u) in kinds for u in later):
                        put_terms("k", j, _rhs_terms(c0[:TQ], c0[TQ:], c1[:TQ], c1[TQ:]), RSUMS)
                    if kind == "Q" and ("SS", j) in kinds:
                        put_terms("q", j, _lhs_terms(c0[:TQ], c1[:TQ], c0[TQ:], c1[TQ:]), LSUMS)
            elif kind in ("SA", "SB"):
                q = qa if kind == "SA" else qb
                set_scores(q, 0, _dot(_rows(q_s, TQ * q, TQ * (q + 1)),
                                      _rows(k_s, 0, TQ * (q + 1)), NT))
            elif kind == "SD":
                for q in (qa, qb):
                    set_scores(q, qa, _dot(_rows(q_s, TQ * q, TQ * (q + 1)),
                                           _rows(k_s, n0, TQ * (q + 1)), NT))
            elif kind == "SS":
                qts = [term("q", n, i, i + 1) for n in range(7)]
                j0 = prog.get(("SS", i), 0)
                prog["SS", i] = j1 = min(i, j0 + cnt) if cnt else i
                for j in range(j0, j1):
                    cs = _combine({n: _dot(qts[n], term("k", n, j, j + 1), NT)
                                   for n in _digits(_PLAN[pre + "S"])})
                    scores.setdefault(qa, {}).update({2 * j: cs[0], 2 * j + 1: cs[1]})
                    scores.setdefault(qb, {}).update({2 * j: cs[2], 2 * j + 1: cs[3]})
            elif kind in ("PA", "PB"):
                q = qa if kind == "PA" else qb
                p = probs(q, range(q + 1)).astype(BF)
                probs_of.pop(q)
                finish(q, _dot(p, _rows(v_s, 0, TQ * (q + 1)), NN), p.astype(F32))
            elif kind in ("PS", "PD"):
                w = TQ * i
                eo = list(range(0, qa, 2)) + list(range(1, qa, 2))
                pa, pb = probs(qa, eo + [qa]), probs(qb, eo + [qa, qb])
                if ("diag", i) not in prog:
                    prog["diag", i] = (pa[:, 2 * w:].astype(BF), pb[:, 2 * w:].astype(BF))
                da, db = prog["diag", i]
                if kind == "PD":
                    prog["PD", i] = (_dot(da, _rows(v_s, n0, n0 + TQ), NN),
                                     _dot(db, _rows(v_s, n0, n0 + PR), NN))
                else:
                    if ("L", i) not in prog:
                        prog["L", i] = [t.astype(BF) for t in _lhs_terms(
                            pa[:, :w], pa[:, w:2 * w], pb[:, :w], pb[:, w:2 * w])]
                    if not run(("P", i), cnt, lambda n: _dot(
                            prog["L", i][n], term("v", n, 0, i), NN)):
                        continue
                if ("PD", i) in prog and len(prog.get(("P", i), ())) == 7:
                    c11, c12, c21, c22 = _combine(prog.pop(("P", i)))
                    oa, ob = prog.pop(("PD", i))
                    lt = prog.pop(("L", i))
                    oa = jnp.concatenate([c11, c12], axis=1) + oa
                    ob = jnp.concatenate([c21, c22], axis=1) + ob
                    for q, o, lo_, d in ((qa, oa, lt[4], da), (qb, ob, lt[1], db)):
                        probs_of.pop(q)
                        finish(q, o, jnp.concatenate([lo_, d], axis=1).astype(F32))
            elif kind == "O":
                j0, j1 = 2 * i, 2 * i + 2
                js = max(j0, min(j1, hyb // 2)) if i < sto else j0
                cols = []
                if js > j0:
                    c11, c12, c21, c22 = _combine(
                        {n: _dot(wterms("O")[n], term("c", n, j0, js), NT)
                         for n in _digits(_PLAN[pre + "O"])})
                    ca = jnp.concatenate([c11, c21], axis=0)
                    cb = jnp.concatenate([c12, c22], axis=0)
                    for t in range(js - j0):
                        cols += [ca[:, TQ * t:TQ * (t + 1)], cb[:, TQ * t:TQ * (t + 1)]]
                if j1 > js:
                    cols.append(_dot(_bf(wo_s[h]), _rows(ctx_s, PR * js, PR * j1), NT))
                g = g_s[:, r0:r1]
                f = []
                for t in range(4):
                    gt, rt = g[:, TQ * t:TQ * (t + 1)], rinv.pop(4 * i + t)
                    f.append(gt if rt is None else gt * rt)
                a = _cat(cols, 1) * jnp.concatenate(f, axis=1)
                if first:
                    acc[:, r0:r1] = a + (1.0 - g) * _bf(xT_s[:, r0:r1]).astype(F32)
                else:
                    a = acc[:, r0:r1] + a
                    acc[:, r0:r1] = a
                    for c0, c1 in out_blocks(i):
                        out_s[:, c0:c1] = a[:, c0 - r0:c1 - r0].astype(BF)

                        @pl.when(h == H - 1)
                        def _():
                            cp_out(c0, c1).start()
            elif kind == "TOPK":
                r = r_s[...]
                lane = lax.broadcasted_iota(I32, (1, S), 1)
                m1 = jnp.max(r, axis=1, keepdims=True)
                i1 = jnp.min(jnp.where(r == m1, lane, S - 1))
                r2 = jnp.where(lane == i1, -jnp.inf, r)
                m2 = jnp.max(r2, axis=1, keepdims=True)
                i2 = jnp.min(jnp.where((r2 == m2) & (lane != i1), lane, S - 1))
                r8 = lax.broadcasted_iota(I32, (8, TQ), 0)
                sig_s[...] = jnp.where(r8 == 0, _sigmoid(m1), _sigmoid(m2))
                lane = lax.broadcasted_iota(I32, (1, TQ), 1)
                for t, idx in enumerate((i1, i2)):
                    idx_s[t] = idx
                    xb = _bf(xT_s[:, _token_block(idx)]).astype(F32)
                    xc = jnp.sum(jnp.where(lane == idx % TQ, xb, 0.0),
                                 axis=1, keepdims=True)
                    xcol_s[t] = jnp.broadcast_to(xc, (M, TQ))
                ypart_s[...] = jnp.zeros_like(ypart_s)
            elif kind == "FV":
                chunk = jnp.minimum(h - 1, NF - 1)
                c = pl.ds(pl.multiple_of(chunk * TQ, TQ), TQ)
                wg, wu, wd = (_bf(w[:, c]).astype(F32) for w in (wg_s, wu_s, wd_s))
                for t in range(2):
                    xc = xcol_s[t]
                    g = jnp.sum(xc * wg, axis=0, keepdims=True)
                    u = jnp.sum(xc * wu, axis=0, keepdims=True)
                    ypart_s[t] += wd * (g * _sigmoid(g) * u)
            else:
                raise ValueError(kind)
        assert not (scores or probs_of or ctx_of or rinv)

    for c in [cp_ckv(0), c_wk, c_wv] + [cp_ckv(i) for i in range(1, NPB)]:
        c.start()
    for c in head0 + head1 + bulk:
        c.start()

    def proj0(t, carry):
        which, blk = t % 2, t // 2
        base = pl.multiple_of(blk * (PB // 2), PB // 2)
        half = pl.multiple_of(blk * (HB // 2), HB // 2)

        @pl.when(which == 0)
        def _():
            cp_ckv(blk).wait()

        @pl.when(t == 0)
        def _():
            c_wk.wait()

        @pl.when(t == 1)
        def _():
            c_wv.wait()

        top, bot = pl.ds(base, HB // 2), pl.ds(base + HB // 2, HB // 2)
        at, ab = _bf(ckv_s[top, :]).astype(F32), _bf(ckv_s[bot, :]).astype(F32)
        tt = _lhs_terms(at[:, :HC], at[:, HC:], ab[:, :HC], ab[:, HC:])
        lhs = {n: tt[n].astype(BF) for n in LSUMS}
        for k, n in enumerate(LSUMS):
            asum_s[k, pl.ds(half, HB // 2), :] = pltpu.bitcast(lhs[n], U32)
        lhs[2], lhs[3] = _bf(ckv_s[top, :HC]), _bf(ckv_s[bot, HC:])
        f = pltpu.bitcast(wkv32[which, 0] << 16, F32)
        rhs = [u.astype(BF) for u in _rhs_terms(*_quads(f))]
        c11, c12, c21, c22 = _combine(
            {n: _dot(lhs[n], rhs[n], NN) for n in _digits(_PLAN["o0"])})
        kv_s[which, top, :] = _u32(jnp.concatenate([c11, c12], axis=1))
        kv_s[which, bot, :] = _u32(jnp.concatenate([c21, c22], axis=1))
        return carry

    def step(h, carry):
        @pl.when(h == 2)
        def _():
            for c in bulk:
                c.wait()

        @pl.when(h == H - 1)
        def _():
            lane = lax.broadcasted_iota(I32, (1, TQ), 1)
            for t in range(2):
                idx = idx_s[t]
                y = jnp.sum(ypart_s[t], axis=1, keepdims=True) * sig_s[t:t + 1, :]
                blk = _token_block(idx)
                old = acc[:, blk]
                acc[:, blk] = jnp.where(
                    lane == idx % TQ, old + (1.0 - g_s[:, blk]) * y, old)

        head(h, False)
        return carry

    left = {(k, i) for k, i, _ in _items(_PLAN["first"]) if k in ("K", "V")}
    assert left <= {("V", NPB - 1)}
    lax.fori_loop(0, 2 * NPB - len(left), proj0, 0)
    for c in head0:
        c.wait()
    head(0, True)
    for c in head1:
        c.wait()
    lax.fori_loop(1, H, step, 0)
    for i in range(NPB):
        for c0, c1 in out_blocks(i):
            cp_out(c0, c1).wait()


@jax.jit
def pallas_gated_mix__compressed_kv_cla__moe_arch_mod__prompt_kernel(
    A_x: jax.Array,
    A_c_kv: jax.Array,
    A_w_q: jax.Array,
    A_w_uk: jax.Array,
    A_w_uv: jax.Array,
    A_w_o: jax.Array,
    B_x: jax.Array,
    B_w_r: jax.Array,
    B_w_gate: jax.Array,
    B_w_up: jax.Array,
    B_w_down: jax.Array,
    gate_w: jax.Array,
):
    del B_x
    xT = A_x.reshape(S, M).T
    ckv = A_c_kv.reshape(S, C)
    woT = jnp.transpose(A_w_o, (0, 2, 1))
    wdT = B_w_down.T

    V = pltpu.VMEM
    scratch = [
        V((M // 2, S), U32),
        V((S // 2, M), U32),
        V((S // 2, C), U32),
        V((H // 2, M, D), U32),
        V((2, H // 2, C, D), U32),
        V((H, M // 2, D), U32),
        V((S // 2, D), U32),
        V((2, S // 2, D), U32),
        V((S // 2, D), U32),
        V((M, S), F32),
        V((1, S), F32),
        V((1, S), F32),
        V((M,), BF),
        V((M,), BF),
        V((M // 2, F), U32),
        V((M // 2, F), U32),
        V((M // 2, F), U32),
        V((8, TQ), F32),
        pltpu.SMEM((2,), I32),
        V((2, M, TQ), F32),
        V((2, M, TQ), F32),
        V((5, S // 4, HC), U32),
        V((7, S // 4, PR), U32),
        V((7, S // 4, TQ), U32),
        V((7, S // 4, TQ), U32),
        V((7, S // 4, TQ), U32),
        V((7, S // 4, TQ), U32),
        V((M, S), BF),
        pltpu.SemaphoreType.DMA((NSEM,)),
    ]
    outT = pl.pallas_call(
        _kernel,
        in_specs=[pl.BlockSpec(memory_space=pl.ANY)] * 11,
        out_specs=pl.BlockSpec(memory_space=pl.ANY),
        out_shape=jax.ShapeDtypeStruct((M, S), BF),
        scratch_shapes=scratch,
        compiler_params=pltpu.CompilerParams(
            vmem_limit_bytes=100 * 1024 * 1024),
    )(xT, ckv, A_w_q, A_w_uk, A_w_uv, woT, B_w_r, B_w_gate, B_w_up, wdT, gate_w)
    return outT.T.reshape(1, S, M)
```
